```python
import os as _os
_os.environ.setdefault('JAX_PLATFORMS', 'cpu')
import jax
import jax.numpy as jnp

def _softmax(x, axis=-1):
    return jax.nn.softmax(x, axis=axis)

def _gelu(x):
    return jax.nn.gelu(x, approximate=True)

def _silu(x):
    return jax.nn.silu(x)

def _sigmoid(x):
    return jax.nn.sigmoid(x)

def _layernorm(x, axis=-1, eps=1e-05):
    m = jnp.mean(x, axis=axis, keepdims=True)
    v = jnp.var(x, axis=axis, keepdims=True)
    return (x - m) / jnp.sqrt(v + eps)

def _scatter_add(tgt, idx, src, axis=0):
    return tgt.at[idx].add(src)

def _segment_sum(src, seg, n):
    return jax.ops.segment_sum(src, seg, n)

class _Rng:

    def __init__(self, key):
        self._k = key

    def _next(self):
        self._k, sub = jax.random.split(self._k)
        return sub

    def normal(self, shape):
        return jax.random.normal(self._next(), shape, dtype=jnp.bfloat16)

    def randint(self, lo, hi, shape):
        return jax.random.randint(self._next(), shape, lo, hi, dtype=jnp.int32)

    def uniform(self, shape, lo=0.0, hi=1.0):
        return jax.random.uniform(self._next(), shape, jnp.bfloat16, lo, hi)

    def permutation(self, n):
        return jax.random.permutation(self._next(), n)
kernel_name = 'concat_heads__spectral_gfnet__memory_aug_recurrent_mem_tr__prompt'

def setup_inputs():
    _rng = _Rng(jax.random.key(int.from_bytes(__import__("os").urandom(4), "little")))
    _w = lambda a: (lambda t: t.astype(jnp.bfloat16) if jnp.issubdtype(t.dtype, jnp.floating) else t)(jnp.asarray(a))

    def _A_setup():
        B, S, D = (1, 2048, 512)
        Df = D // 2 + 1
        return {'x': _w((lambda *s: _rng.normal(s) * 0.05)(B, S, D)), 'w_r': _w((lambda *s: _rng.normal(s) * 0.05)(S, Df) * 0.02), 'w_i': _w((lambda *s: _rng.normal(s) * 0.05)(S, Df) * 0.02)}
    _A_in = _A_setup()

    def _B_setup():
        B, S, Dm = (1, 2048, 512)
        H, Dh = (32, 128)
        M, seg = (8, 32)
        seg = min(seg, S)
        S = S // seg * seg
        return {'x': _w((lambda *s: _rng.normal(s) * 0.05)(B, S, Dm)), 'mem0': _w((lambda *s: _rng.normal(s) * 0.4)(B, M, Dm)), 'Wq': _w((lambda *s: _rng.normal(s) * 3.2)(Dm, H, Dh) * Dm ** (-0.5)), 'Wk': _w((lambda *s: _rng.normal(s) * 3.2)(Dm, H, Dh) * Dm ** (-0.5)), 'Wv': _w((lambda *s: _rng.normal(s) * 0.4)(Dm, H, Dh) * Dm ** (-0.5)), 'Wo': _w((lambda *s: _rng.normal(s) * 0.4)(H, Dh, Dm) * (H * Dh) ** (-0.5)), 'seg_len': seg}
    _B_in = _B_setup()
    return {'A_x': _A_in['x'], 'A_w_r': _A_in['w_r'], 'A_w_i': _A_in['w_i'], 'B_x': _B_in['x'], 'B_mem0': _B_in['mem0'], 'B_Wq': _B_in['Wq'], 'B_Wk': _B_in['Wk'], 'B_Wv': _B_in['Wv'], 'B_Wo': _B_in['Wo'], 'B_seg_len': _B_in['seg_len']}

def reference(A_x, A_w_r, A_w_i, B_x, B_mem0, B_Wq, B_Wk, B_Wv, B_Wo, B_seg_len):

    def _A_ref(x, w_r, w_i):
        B, S, D = x.shape
        X = (lambda x, axes=(-2, -1): jnp.fft.rfft2(x.astype(jnp.float32), axes=axes))(x, axes=(-2, -1))
        W = w_r + 1j * w_i
        X = X * W
        y = (lambda x, s, axes=(-2, -1): jnp.fft.irfft2(x, s=s, axes=axes).astype(jnp.bfloat16))(X, (S, D), axes=(-2, -1))
        return y

    def _B_ref(x, mem0, Wq, Wk, Wv, Wo, seg_len):
        B, S, Dm = x.shape
        H, Dh = (Wq.shape[1], Wq.shape[2])
        M = mem0.shape[1]
        scale = Dh ** (-0.5)
        n_seg = S // seg_len
        L = M + seg_len
        idx = jnp.arange(L)
        mask = (idx[:, None] < M) | (idx[:, None] >= idx[None, :])
        mem = mem0
        outs = []
        for s in range(n_seg):
            xs = x[:, s * seg_len:(s + 1) * seg_len, :].copy()
            h = jnp.concatenate([mem, xs], axis=1)
            q = jnp.einsum('btd,dhe->bhte', h, Wq)
            k = jnp.einsum('btd,dhe->bhte', h, Wk)
            v = jnp.einsum('btd,dhe->bhte', h, Wv)
            scores = jnp.einsum('bhqe,bhke->bhqk', q, k) * scale
            scores = jnp.where(mask[None, None], scores, -1000000000.0)
            p = _softmax(scores, axis=-1)
            o = jnp.einsum('bhqk,bhke->bhqe', p, v)
            o = jnp.einsum('bhte,hed->btd', o, Wo)
            mem = o[:, :M, :].copy()
            outs.append(o[:, M:, :])
        return jnp.concatenate(outs, axis=1)
    a = _A_ref(A_x, A_w_r, A_w_i)
    b = _B_ref(B_x, B_mem0, B_Wq, B_Wk, B_Wv, B_Wo, B_seg_len)
    return jnp.concatenate([a, b], axis=-1)
```

```python
import numpy as np
import jax
import jax.numpy as jnp
from jax import lax
import jax.experimental.pallas as pl
import jax.experimental.pallas.tpu as pltpu

S, DM, H, DH, MEM, SEG = 2048, 512, 32, 128, 8, 32
NSEG = S // SEG
NP = H // 2
N1, N2 = 32, 64
BF, F32, U32 = jnp.bfloat16, jnp.float32, jnp.uint32
EXP_C = float(DH ** -0.5 * np.log2(np.e))
WO_CH = 352
HI_MASK = 0xFFFF0000


def _pack_rows(m):
    f = np.ascontiguousarray(m, dtype=np.float32).view(np.uint32)
    r = ((f + 0x7FFF + ((f >> 16) & 1)) >> 16).astype(np.uint32)
    return r[..., 0::2, :] | (r[..., 1::2, :] << 16)


def _consts():
    l = np.arange(128)
    k_e = 2 * l
    k_o = 2 * l + 1
    d2 = np.arange(128)[:, None]
    lo = (l % 2) == 0
    a_re = 2 * np.pi * d2 * k_e[None, :] / DM
    a_im = 2 * np.pi * d2 * k_e[(l - 1) % 128][None, :] / DM
    m0 = np.where(lo[None, :], np.cos(a_re), -np.sin(a_im))
    m0[:, 1] = (-1.0) ** np.arange(128)
    m2 = np.where(lo[None, :], -np.sin(a_im), np.cos(a_re))
    a_o = 2 * np.pi * np.arange(256)[:, None] * k_o[None, :] / DM
    mo = np.concatenate([np.cos(a_o), -np.sin(a_o)], axis=1)
    sc = 2.0 / (S * DM)
    m0i = m0.T * sc
    m0i[0] /= 2
    m0i[1] /= 2
    dfw = np.concatenate([np.concatenate([m0, m2], axis=1), mo], axis=0)
    dinv = np.concatenate([np.concatenate([m0i, m2.T * sc], axis=1), mo.T * sc], axis=0)
    k1 = np.arange(N1)[:, None, None]
    k2 = np.arange(N2)[None, :, None]
    s2 = np.arange(N2)[None, None, :]
    th = 2 * np.pi * ((s2 * (k1 + N1 * k2)) % S) / S
    c, s = np.cos(th), np.sin(th)
    mf = np.concatenate([np.concatenate([c, s], 2), np.concatenate([-s, c], 2)], 1)
    dmat = _pack_rows(np.stack([dfw, dinv]))
    smat = _pack_rows(np.stack([mf, mf.transpose(0, 2, 1)]))
    head = np.concatenate([np.zeros(32), np.ones(32), np.zeros(8), np.ones(8)])
    pos = np.concatenate([np.arange(8), np.arange(16, 40)] * 2 + [np.arange(8, 16)] * 2)
    ok = (head[:, None] == head[None, :]) & ((pos[:, None] < MEM) | (pos[:, None] >= pos[None, :]))
    mask = np.where(ok, 0.0, -1e30).astype(np.float32)
    return dmat, smat, mask


def _cmul(z, ang):
    re, im = z
    c, s = float(np.cos(ang)), float(np.sin(ang))
    if abs(s) < 1e-12:
        return (re, im) if c > 0 else (-re, -im)
    if abs(abs(c) - abs(s)) < 1e-12:
        r = abs(c)
        p, m = (re + im) * r, (re - im) * r
        if c > 0 and s < 0:
            return p, -m
        if c > 0 and s > 0:
            return m, p
        if c < 0 and s < 0:
            return -m, -p
        return -p, m
    return re * c - im * s, re * s + im * c


def _fft(x, sign):
    n = len(x)
    if n == 1:
        return x
    if n == 2:
        (ar, ai), (br, bi) = x
        return [(ar + br, ai + bi), (ar - br, ai - bi)]
    ev, z1, z3 = _fft(x[0::2], sign), _fft(x[1::4], sign), _fft(x[3::4], sign)
    out = [None] * n
    q = n // 4
    for k in range(q):
        ar, ai = _cmul(z1[k], sign * 2 * np.pi * k / n)
        br, bi = _cmul(z3[k], sign * 2 * np.pi * 3 * k / n)
        sr, si, dr, di = ar + br, ai + bi, ar - br, ai - bi
        (er, ei), (fr, fi) = ev[k], ev[k + q]
        out[k] = (er + sr, ei + si)
        out[k + 2 * q] = (er - sr, ei - si)
        plus, minus = (fr - di, fi + dr), (fr + di, fi - dr)
        out[k + q], out[k + 3 * q] = (plus, minus) if sign > 0 else (minus, plus)
    return out


def _dot(a, b):
    return jnp.dot(a, b, preferred_element_type=F32)


def _bf(words):
    return pltpu.bitcast(words, BF)


def _kernel(ax_h, wr_h, wi_h, bx_h, mem_h, wq_h, wk_h, wv_h, wo_h, dmat_h, smat_h, mask_h,
            o_h,
            wraw, wtmp, w_s, woraw, wo_s, p_s, od_s, acc_s, x0raw, x0_s, xr_s, mem_s, mask_s,
            ax_s, fraw, f_s, u_s, dmat_s, smat_s, ce_s, oa_s, ob_s,
            sem_w, sem_wo, sem_m, sem_oa, sem_ob):
    w_h = (wk_h, wq_h, wv_h)

    def w_copy(t):
        return pltpu.make_async_copy(w_h[t // 4].at[:, pl.ds(8 * (t % 4), 8), :], wraw.at[t], sem_w.at[t])

    def wo_copy(t):
        n = min(WO_CH, H * DH - t * WO_CH)
        return pltpu.make_async_copy(wo_h.at[pl.ds(t * WO_CH, n)], woraw.at[pl.ds(t * WO_CH, n)], sem_wo.at[t])

    misc = [
        pltpu.make_async_copy(bx_h.at[:, pl.ds(0, 8), :], x0raw, sem_m.at[0]),
        pltpu.make_async_copy(bx_h.at[:, pl.ds(8, 24), :], xr_s, sem_m.at[1]),
        pltpu.make_async_copy(mem_h, mem_s, sem_m.at[2]),
        pltpu.make_async_copy(mask_h, mask_s, sem_m.at[3]),
        pltpu.make_async_copy(ax_h, ax_s, sem_m.at[4]),
        pltpu.make_async_copy(dmat_h, dmat_s, sem_m.at[5]),
        pltpu.make_async_copy(wr_h, fraw.at[0], sem_m.at[6]),
        pltpu.make_async_copy(wi_h, fraw.at[1], sem_m.at[7]),
        pltpu.make_async_copy(smat_h, smat_s, sem_m.at[8]),
    ]
    misc[0].start()
    w_copy(0).start()
    for t in range(1, 12):
        w_copy(t).start()
        wo_copy(t - 1).start()
    wo_copy(11).start()
    for c in misc[1:]:
        c.start()

    def relayout_a(t):
        for dc in range(8):
            v = wraw[t, dc * 64:(dc + 1) * 64]
            wtmp[dc * 256:(dc + 1) * 256, :] = pltpu.bitcast(v.reshape(512, 128), U32)

    def relayout_b(t, jj):
        a = wtmp[pl.ds(jj, 256, stride=8), :]
        b = wtmp[pl.ds(4 + jj, 256, stride=8), :]
        w_s[t * 8 + 2 * jj] = (a & 0xFFFF) | (b << 16)
        w_s[t * 8 + 2 * jj + 1] = (a >> 16) | (b & jnp.uint32(HI_MASK))

    misc[0].wait()
    x0_s[...] = pltpu.bitcast(x0raw[...].reshape(NSEG * 8, DM), U32)
    w_copy(0).wait()
    relayout_a(0)
    for jj in range(4):
        relayout_b(0, jj)

    def phase1(t, carry):
        tn = jnp.minimum(t + 1, 11)

        @pl.when(t < 11)
        def _():
            pltpu.make_async_copy(w_h[0].at[:, pl.ds(0, 8), :], wraw.at[tn], sem_w.at[tn]).wait()
            pltpu.make_async_copy(wo_h.at[pl.ds(0, WO_CH)], woraw.at[pl.ds(pl.multiple_of(t * WO_CH, 16), WO_CH)],
                                  sem_wo.at[t]).wait()

        @pl.when(t == 11)
        def _():
            wo_copy(11).wait()

        relayout_a(tn)
        r = pl.multiple_of(jnp.minimum(t * WO_CH, H * DH - WO_CH), 32)
        wo_s[pl.ds(pl.multiple_of(r // 2, 16), WO_CH // 2), :] = pltpu.bitcast(woraw[pl.ds(r, WO_CH), :], U32)
        for jj in range(4):
            x0 = _bf(x0_s[...])
            r1 = _dot(x0, _bf(w_s[t * 8 + 2 * jj]))
            r2 = _dot(x0, _bf(w_s[t * 8 + 2 * jj + 1]))
            p_s[t * 4 + jj] = jnp.concatenate([r1.reshape(NSEG, 8, 128), r2.reshape(NSEG, 8, 128)], axis=1)
            relayout_b(tn, jj)
        return carry

    lax.fori_loop(0, 12, phase1, 0)
    for c in misc[1:]:
        c.wait()

    lane = lax.broadcasted_iota(jnp.int32, (1, 128), 1)
    lane_lo = (lane & 1) == 0
    lane_0 = lane == 0

    def filt_prep(i):
        for h in range(2):
            col = pl.ds(pl.multiple_of((2 * i + h) * 128, 128), 128)
            nyq = [pltpu.bitcast(fraw[a, 256:257, col].astype(F32), U32) for a in range(2)]
            tiles = [pltpu.bitcast(fraw[a, 0:256, col], U32) for a in range(2)]
            tiles.append(jnp.broadcast_to((nyq[0] >> 16) | nyq[1], (128, 128)))
            for a in range(3):
                t = pltpu.bitcast(pltpu.bitcast(tiles[a], F32).T, U32)
                for q in range(16):
                    r = pl.multiple_of(((2 * i + h) * 4 + q // 4) * 8, 8)
                    f_s[a, q % 4, pl.ds(r, 8), :] = t[q * 8:(q + 1) * 8]

    def ax_blocks(c):
        v = ax_s[:, pl.ds(pl.multiple_of(c * 8, 8), 8), :].astype(F32).reshape(256, DM)
        return [v[:, i * 128:(i + 1) * 128] for i in range(4)]

    def split(re, im):
        return [(re[i * 8:(i + 1) * 8], im[i * 8:(i + 1) * 8]) for i in range(N1)]

    def put_u(c, blk, u):
        r = pl.multiple_of(c * 8, 8)
        for k in range(N1):
            u_s[k, blk, pl.ds(r, 8), :] = u[k][0]
            u_s[k, blk, pl.ds(64 + r, 8), :] = u[k][1]

    def get_u(c, blk):
        r = pl.multiple_of(c * 8, 8)
        return [(u_s[k, blk, pl.ds(r, 8), :], u_s[k, blk, pl.ds(64 + r, 8), :]) for k in range(N1)]

    def fwd_even(c):
        x0, x1, x2, x3 = ax_blocks(c)
        p, q = x0 + x2, x1 + x3
        t0 = _dot((p + q).astype(BF), _bf(dmat_s[0, 0:64, 0:128]))
        t2 = _dot((p - q).astype(BF), _bf(dmat_s[0, 0:64, 128:256]))
        re = jnp.where(lane_lo, t0, t2)
        im = pltpu.roll(jnp.where(lane_lo, t2, t0), 127, 1)
        u = _fft(split(re, im), -1)
        ue, un = [None] * N1, [None] * N1
        for k in range(N1 // 2 + 1):
            m = (N1 - k) % N1
            (ar, ai), (br, bi) = u[k], u[m]
            sr, si, dr, di = (ar + br) * 0.5, (ai + bi) * 0.5, (br - ar) * 0.5, (ai - bi) * 0.5
            ue[k] = (jnp.where(lane_0, sr, ar), jnp.where(lane_0, di, ai))
            un[k] = (si, dr)
            if m != k:
                ue[m] = (jnp.where(lane_0, sr, br), jnp.where(lane_0, -di, bi))
                un[m] = (si, -dr)
        put_u(c, 0, ue)
        put_u(c, 2, un)

    def fwd_odd(c):
        x0, x1, x2, x3 = ax_blocks(c)
        o = _dot(jnp.concatenate([x0 - x2, x1 - x3], axis=1).astype(BF), _bf(dmat_s[0, 64:192, :]))
        put_u(c, 1, _fft(split(o[:, 0:128], o[:, 128:256]), -1))

    def mid_a(i, u):
        k1 = 4 * i + u
        t = jnp.concatenate([u_s[k1, b] for b in range(3)], axis=1).astype(BF)
        z = _dot(_bf(smat_s[0, k1]), t)
        w = [jnp.where(i % 2 == 0, f_s[a, i // 2, pl.ds(u, 64, stride=8), :],
                       f_s[a, i // 2, pl.ds(4 + u, 64, stride=8), :]) for a in range(3)]
        lo = [pltpu.bitcast(v << 16, F32) for v in w]
        hi = [pltpu.bitcast(v & jnp.uint32(HI_MASK), F32) for v in w]
        wr = jnp.concatenate([lo[0], hi[0], lo[2]], axis=1)
        wi = jnp.concatenate([lo[1], hi[1], hi[2]], axis=1)
        zr, zi = z[0:64], z[64:128]
        return k1, jnp.concatenate([zr * wr - zi * wi, zr * wi + zi * wr], axis=0).astype(BF)

    def mid_b(k1, y):
        v = _dot(_bf(smat_s[1, k1]), y)
        for b in range(3):
            u_s[k1, b] = v[:, b * 128:(b + 1) * 128]

    def join(g):
        return jnp.concatenate([z[0] for z in g], axis=0), jnp.concatenate([z[1] for z in g], axis=0)

    def inv_even(c):
        v, vn = get_u(c, 0), get_u(c, 2)
        w = [None] * N1
        for k in range(N1 // 2 + 1):
            m = (N1 - k) % N1
            (ar, ai), (br, bi), (cr, ci), (er, ei) = v[k], v[m], vn[k], vn[m]
            sr, di, nr, ni = (ar + br) * 0.5, (ai - bi) * 0.5, (cr + er) * 0.5, (ci - ei) * 0.5
            w[k] = (jnp.where(lane_0, sr - ni, ar), jnp.where(lane_0, di + nr, ai))
            if m != k:
                w[m] = (jnp.where(lane_0, sr + ni, br), jnp.where(lane_0, nr - di, bi))
        re, im = join(_fft(w, 1))
        im = pltpu.roll(im, 1, 1)
        c0 = _dot(jnp.where(lane_lo, re, im).astype(BF), _bf(dmat_s[1, 0:64, 0:128]))
        c2 = _dot(jnp.where(lane_lo, im, re).astype(BF), _bf(dmat_s[1, 0:64, 128:256]))
        ce_s[0] = c0 + c2
        ce_s[1] = c0 - c2

    def inv_odd_a(c):
        re, im = join(_fft(get_u(c, 1), 1))
        return jnp.concatenate([re, im], axis=1).astype(BF)

    def inv_odd_b(c, g):
        pq = _dot(g, _bf(dmat_s[1, 64:192, :]))
        p, q = pq[:, 0:128], pq[:, 128:256]
        e, f = ce_s[0], ce_s[1]
        y = jnp.concatenate([e + p, f + q, e - p, f - q], axis=1)
        oa_s[:, pl.ds(pl.multiple_of(c * 8, 8), 8), :] = y.reshape(N1, 8, DM).astype(BF)

    def late_proj(g, c):
        a = od_s[c, pl.ds(pl.multiple_of(g * 128, 128), 128), :].astype(BF)
        w = _bf(wo_s[pl.ds(pl.multiple_of(c * 128, 128), 128), :])
        acc_s[...] += _dot(a, w)

    def step(s, mem, hooks):
        xr = xr_s[s]
        lhs = jnp.concatenate([mem, xr.astype(F32)], axis=0).astype(BF)
        r8 = pl.multiple_of(s * 8, 8)
        st = {}

        def proj(mi, j):
            y1 = _dot(lhs, _bf(w_s[mi * H + 2 * j]))
            y2 = _dot(lhs, _bf(w_s[mi * H + 2 * j + 1]))
            st[mi, j] = jnp.concatenate([y1, y2, p_s[mi * NP + j, s]], axis=0).astype(BF)

        def qk(j):
            sc = lax.dot_general(st.pop((1, j)), st.pop((0, j)), (((1,), (1,)), ((), ())),
                                 preferred_element_type=F32) + mask_s[...]
            p = jnp.exp2((sc - jnp.max(sc, axis=1, keepdims=True)) * EXP_C)
            st["p", j] = (p.astype(BF), pl.reciprocal(jnp.sum(p, axis=1, keepdims=True), approx=True))

        def pv(j):
            p, rl = st.pop(("p", j))
            o = _dot(p, st.pop((2, j))) * rl
            st["o", j] = jnp.concatenate([o[0:32], o[32:64]], axis=1).astype(BF)
            od_s[j, pl.ds(r8, 8), :] = jnp.concatenate([o[64:72], o[72:80]], axis=1)

        def op(js):
            oc = jnp.concatenate([st.pop(("o", j)) for j in js], axis=1)
            r = _dot(oc, _bf(wo_s[js[0] * 128:(js[-1] + 1) * 128, :]))
            st["acc"] = r if "acc" not in st else st["acc"] + r

        def hook(name):
            if name in hooks:
                hooks[name]()

        for j in range(NP):
            proj(0, j)
            if j >= 3:
                pv(j - 3)
            proj(1, j)
            if j >= 1:
                qk(j - 1)
            proj(2, j)
            hook(j)
        op([0, 1, 2])
        pv(13)
        qk(15)
        op([3, 4, 5])
        pv(14)
        op([6, 7, 8])
        pv(15)
        hook("op")
        op([9, 10, 11, 12])
        op([13, 14, 15])
        out = st["acc"]
        hook("end")
        ob_s[s // 2, pl.ds(pl.multiple_of((s % 2) * 32 + 8, 8), 24), :] = out[8:32].astype(BF)
        return out[0:8].astype(BF).astype(F32)

    def ob_copy(g):
        return pltpu.make_async_copy(ob_s.at[pl.ds(g * 8, 8)], o_h.at[pl.ds(g * 8, 8), :, pl.ds(DM, DM)],
                                     sem_ob.at[g])

    def finish(g):
        res = acc_s[...]
        for i in range(16):
            ob_s[g * 8 + i // 2, (i % 2) * 32:(i % 2) * 32 + 8, :] = res[i * 8:(i + 1) * 8].astype(BF)
        acc_s[...] = jnp.zeros_like(acc_s)
        ob_copy(g).start()

    acc_s[...] = jnp.zeros_like(acc_s)

    def loop1(i, mem):
        mem = step(2 * i, mem, {2: lambda: filt_prep(i), "end": lambda: fwd_odd(i)})
        return step(2 * i + 1, mem, {4: lambda: fwd_even(i)})

    mem = lax.fori_loop(0, 8, loop1, mem_s[...].astype(F32))

    def loop2(i, mem):
        g = i // 4
        for u in range(4):
            c = (i % 4) * 4 + u
            box = {}
            mem = step(16 + 4 * i + u, mem, {
                8: lambda: box.update(y=mid_a(i, u)),
                "op": lambda: mid_b(*box["y"]),
                "end": lambda: late_proj(g, c)})

        @pl.when(i % 4 == 3)
        def _():
            finish(g)

        return mem

    mem = lax.fori_loop(0, 8, loop2, mem)

    def oa_copy(c):
        return pltpu.make_async_copy(oa_s.at[:, pl.ds(c * 8, 8), :], o_h.at[:, pl.ds(c * 8, 8), pl.ds(0, DM)],
                                     sem_oa.at[c])

    def loop3(i, mem):
        box = {}
        mem = step(48 + 2 * i, mem, {"op": lambda: inv_even(i), "end": lambda: late_proj(2, 2 * i)})
        mem = step(49 + 2 * i, mem, {0: lambda: box.update(g=inv_odd_a(i)), 12: lambda: inv_odd_b(i, box["g"]),
                                     "end": lambda: late_proj(2, 2 * i + 1)})
        r = pl.multiple_of(i * 8, 8)
        pltpu.make_async_copy(oa_s.at[:, pl.ds(r, 8), :], o_h.at[:, pl.ds(r, 8), pl.ds(0, DM)], sem_oa.at[i]).start()
        return mem

    lax.fori_loop(0, 8, loop3, mem)
    finish(2)
    for c in range(16):
        late_proj(3, c)
    finish(3)
    for c in range(8):
        oa_copy(c).wait()
    for g in range(4):
        ob_copy(g).wait()


@jax.jit
def pallas_concat_heads__spectral_gfnet__memory_aug_recurrent_mem_tr__prompt_kernel(
        A_x, A_w_r, A_w_i, B_x, B_mem0, B_Wq, B_Wk, B_Wv, B_Wo, B_seg_len=None):
    dmat, smat, mask = _consts()
    vm = pltpu.VMEM
    out = pl.pallas_call(
        _kernel,
        out_shape=jax.ShapeDtypeStruct((N1, N2, 2 * DM), BF),
        in_specs=[pl.BlockSpec(memory_space=pl.ANY)] * 12,
        out_specs=pl.BlockSpec(memory_space=pl.ANY),
        scratch_shapes=[
            vm((12, DM, 8, DH), BF), vm((2048, 128), U32), vm((3 * H, DM // 2, DH), U32),
            vm((H * DH, DM), BF), vm((H * DH // 2, DM), U32),
            vm((3 * NP, NSEG, 16, DH), F32), vm((NP, NSEG * 8, 2 * DH), F32), vm((128, DM), F32),
            vm((NSEG, 8, DM), BF), vm((NSEG * 4, DM), U32), vm((NSEG, 24, DM), BF), vm((MEM, DM), BF),
            vm((80, 80), F32),
            vm((N1, N2, DM), BF), vm((2, 257, S), BF), vm((3, 4, 512, 128), U32),
            vm((N1, 3, 128, 128), F32), vm((2, 192, 256), U32), vm((2, N1, 64, 128), U32),
            vm((2, 256, 128), F32), vm((N1, N2, DM), BF), vm((N1, N2, DM), BF),
            pltpu.SemaphoreType.DMA((12,)), pltpu.SemaphoreType.DMA((12,)), pltpu.SemaphoreType.DMA((9,)),
            pltpu.SemaphoreType.DMA((8,)), pltpu.SemaphoreType.DMA((4,)),
        ],
        compiler_params=pltpu.CompilerParams(vmem_limit_bytes=120 * 1024 * 1024),
    )(A_x.reshape(N1, N2, DM), A_w_r.T, A_w_i.T,
      B_x.reshape(NSEG, SEG, DM), B_mem0.reshape(MEM, DM), B_Wq, B_Wk, B_Wv, B_Wo.reshape(H * DH, DM),
      jnp.asarray(dmat), jnp.asarray(smat), jnp.asarray(mask))
    return out.reshape(1, S, 2 * DM)
```

```python
import os
import numpy as np
import jax
import jax.numpy as jnp
from jax import lax
import jax.experimental.pallas as pl
import jax.experimental.pallas.tpu as pltpu

S, DM, H, DH, MEM, SEG = 2048, 512, 32, 128, 8, 32
NSEG = S // SEG
NP = H // 2
N1, N2 = 32, 64
BF, F32, U32 = jnp.bfloat16, jnp.float32, jnp.uint32
EXP_C = float(DH ** -0.5 * np.log2(np.e))
HI_MASK = 0xFFFF0000
UA = int(os.environ.get("UA", 4))
NOCHK = bool(int(os.environ.get("NOCHK", 1)))

P_OFF = 0
T_OFF = P_OFF + 3 * NP * NSEG * 16
L_OFF = T_OFF + 64 * 8
V_OFF = L_OFF + 4 * 256
X_OFF = V_OFF + (2 * N1 + 1) * 128
BIG_ROWS = X_OFF + 16
TK_OFF = 0
Z_OFF = TK_OFF + 16
TF_OFF = Z_OFF + 8
F_OFF = TF_OFF + 2 * 512 + 8
U_OFF = F_OFF + 8 * 512 + 96
PB_ROWS = U_OFF + (2 * N1 + 1) * 128
E = lambda k, d: int(os.environ.get(k, d))
QL, PL, SK = E("QL", 3), E("PL", 5), E("SK", 1)


def _pack_rows(m):
    f = np.ascontiguousarray(m, dtype=np.float32).view(np.uint32)
    r = ((f + 0x7FFF + ((f >> 16) & 1)) >> 16).astype(np.uint32)
    return r[..., 0::2, :] | (r[..., 1::2, :] << 16)


def _consts():
    l = np.arange(128)
    d2 = np.arange(128)[:, None]
    lo = (l % 2) == 0
    a_re = 2 * np.pi * d2 * (2 * l)[None, :] / DM
    a_im = 2 * np.pi * d2 * (2 * ((l - 1) % 128))[None, :] / DM
    m0 = np.where(lo[None, :], np.cos(a_re), -np.sin(a_im))
    m0[:, 1] = (-1.0) ** np.arange(128)
    m2 = np.where(lo[None, :], -np.sin(a_im), np.cos(a_re))
    e = np.arange(64)[:, None]

    def odd_cols(lanes):
        kd = 2 * lanes + 1
        ang = 2 * np.pi * e * kd[None, :] / DM
        sg = np.where(kd % 4 == 1, 1.0, -1.0)[None, :]
        return (np.concatenate([np.cos(ang), -sg * np.sin(ang)], axis=0),
                np.concatenate([-np.sin(ang), -sg * np.cos(ang)], axis=0))

    plus = (l % 4 == 0) | (l % 4 == 3)
    o_re, o_im = odd_cols(l)[0], odd_cols((l - 2) % 128)[1]
    mp = np.where(plus[None, :], o_re, o_im)
    mm = np.where(plus[None, :], o_im, o_re)
    sc = 2.0 / (S * DM)
    m0i = m0.T * sc
    m0i[0] /= 2
    m0i[1] /= 2
    a32 = 2 * np.pi * np.outer(np.arange(N1), np.arange(N1)) / N1
    c32, s32 = np.zeros((128, 128)), np.zeros((128, 128))
    c32[:N1, :N1], s32[:N1, :N1] = np.cos(a32), -np.sin(a32)
    nf = np.concatenate([c32, s32], axis=1)
    dfw = np.concatenate([np.concatenate([m0, m2], axis=1), np.concatenate([mp, mm], axis=1), nf], axis=0)
    dinv = np.concatenate([np.concatenate([m0i, m2.T * sc], axis=1),
                           np.concatenate([mp.T, mm.T], axis=1) * sc, nf], axis=0)
    k1 = np.arange(N1)[:, None, None]
    k2 = np.arange(N2)[None, :, None]
    s2 = np.arange(N2)[None, None, :]
    th = 2 * np.pi * ((s2 * (k1 + N1 * k2)) % S) / S
    rho = np.arange(N2)
    th = np.concatenate([th, th[:1, 4 * (rho % 16) + rho // 16]], axis=0)
    c, s = np.cos(th), np.sin(th)
    mf = np.concatenate([np.concatenate([c, s], 2), np.concatenate([-s, c], 2)], 1)
    dmat = _pack_rows(np.stack([dfw, dinv]))
    smat = _pack_rows(np.stack([mf, mf.transpose(0, 2, 1)], axis=1))
    head = np.concatenate([np.zeros(32), np.ones(32), np.zeros(8), np.ones(8)])
    pos = np.concatenate([np.arange(8), np.arange(16, 40)] * 2 + [np.arange(8, 16)] * 2)
    ok = (head[:, None] == head[None, :]) & ((pos[:, None] < MEM) | (pos[:, None] >= pos[None, :]))
    misc = np.zeros((80 + 2 * N2, 128), np.float32)
    misc[:80, :80] = np.where(ok, 0.0, -1e30)
    atw = 2 * np.pi * np.outer(np.arange(N2), np.arange(128) % N1) / S
    misc[80:80 + N2], misc[80 + N2:] = np.cos(atw), np.sin(atw)
    return dmat, smat, misc


def _cmul(z, ang):
    re, im = z
    c, s = float(np.cos(ang)), float(np.sin(ang))
    if abs(s) < 1e-12:
        return (re, im) if c > 0 else (-re, -im)
    if abs(c) < 1e-12:
        return (-im, re) if s > 0 else (im, -re)
    if abs(abs(c) - abs(s)) < 1e-12:
        return ((re - im) * c, (re + im) * c) if c * s > 0 else ((re + im) * c, (im - re) * c)
    return re * c - im * s, re * s + im * c


def _fft(x, sign):
    n = len(x)
    if n == 1:
        return x
    if n == 2:
        (ar, ai), (br, bi) = x
        return [(ar + br, ai + bi), (ar - br, ai - bi)]
    ev, z1, z3 = _fft(x[0::2], sign), _fft(x[1::4], sign), _fft(x[3::4], sign)
    out = [None] * n
    q = n // 4
    for k in range(q):
        ar, ai = _cmul(z1[k], sign * 2 * np.pi * k / n)
        br, bi = _cmul(z3[k], sign * 2 * np.pi * 3 * k / n)
        sr, si, dr, di = ar + br, ai + bi, ar - br, ai - bi
        (er, ei), (fr, fi) = ev[k], ev[k + q]
        out[k] = (er + sr, ei + si)
        out[k + 2 * q] = (er - sr, ei - si)
        plus, minus = (fr - di, fi + dr), (fr + di, fi - dr)
        out[k + q], out[k + 3 * q] = (plus, minus) if sign > 0 else (minus, plus)
    return out


def _dot(a, b):
    return jnp.dot(a, b, preferred_element_type=F32)


def _bf(words):
    return pltpu.bitcast(words, BF)


def _f32(words):
    return pltpu.bitcast(words, F32)


def _u32(x):
    return pltpu.bitcast(x, U32)


def _kernel(ax_h, wr_h, wi_h, bx_h, mem_h, wq_h, wk_h, wv_h, wo_h, dmat_h, smat_h, misc_h,
            o_h,
            wraw, pb, wtmp, w_s, wo_s, woraw, big, od_s, acc_s, x0raw, x0_s, xr_s, mem_s, misc_s,
            ax_s, fraw, dmat_s, smat_s, oa_s, ob_s,
            sem_w, sem_c, sem_m, sem_oa, sem_ob, sem_f):
    w_h = (wk_h, wq_h, wv_h)
    cp = pltpu.make_async_copy

    def w_copy(m, g):
        return cp(w_h[m].at[:, pl.ds(pl.multiple_of(8 * g, 8), 8), :], wraw.at[4 * m + g], sem_w.at[4 * m + g])

    def chunk_copies(i):
        rows = pl.ds(pl.multiple_of(i * 512, 512), 512)
        r8 = pl.ds(pl.multiple_of(i * 8, 8), 8)
        cols = pl.ds(pl.multiple_of(i * 256, 256), 256)
        return [cp(wo_h.at[rows], woraw.at[rows], sem_c.at[i]),
                cp(ax_h.at[:, r8, :], ax_s.at[:, r8, :], sem_c.at[i]),
                cp(wr_h.at[:, cols], fraw.at[0, :, cols], sem_c.at[i]),
                cp(wi_h.at[:, cols], fraw.at[1, :, cols], sem_c.at[i])]

    def first_copies(kt):
        d = pl.ds(pl.multiple_of(kt * 128, 128), 128)
        return [cp(bx_h.at[:, pl.ds(0, 8), d], x0raw.at[kt], sem_f.at[kt]),
                cp(wk_h.at[d, pl.ds(0, 8), :], wraw.at[0, d], sem_f.at[kt])]

    early = [cp(dmat_h, dmat_s, sem_m.at[1]), cp(misc_h, misc_s, sem_m.at[2]), cp(mem_h, mem_s, sem_m.at[3])]
    late = [cp(bx_h.at[:, pl.ds(8, 24), :], xr_s, sem_m.at[4]), cp(smat_h, smat_s, sem_m.at[5])]

    lane = lax.broadcasted_iota(jnp.int32, (1, 128), 1)
    lane_lo = (lane & 1) == 0
    lane_plus = ((lane + 1) & 2) == 0
    lane_half = lane < 64
    rt = float(np.sqrt(0.5))

    def wo_rows(j):
        r = pl.ds(pl.multiple_of((j % 2) * 128, 128), 128)
        return _bf(jnp.concatenate([wo_s[n * 8 + j // 2, r, :] for n in range(4)], axis=1))

    def rows8(off):
        return pl.ds(pl.multiple_of(off, 8), 8)

    def filt_prep(i, h, a):
        col = pl.ds(pl.multiple_of((2 * i + h) * 128, 128), 128)
        t = pltpu.bitcast(pltpu.bitcast(fraw[a, 0:256, col], F32).T, U32)
        for q in range(16):
            pb[rows8(F_OFF + (a * 4 + q % 4) * 512 + ((2 * i + h) * 4 + q // 4) * 8), :] = t[q * 8:(q + 1) * 8]

    order = [8 * a + b for b in range(8) for a in range(4)]

    def ax_blocks(c):
        v = jnp.concatenate([ax_s[s1, rows8(c * 8), :].astype(F32) for s1 in order], axis=0)
        return [v[:, i * 128:(i + 1) * 128] for i in range(4)]

    def t_rows(ka, b, part, off=T_OFF):
        return pl.ds(off + ((ka * 8 + b) * 2 + part) * 8, 8)

    def u_rows(k1, blk, part, c, off=0):
        return rows8(off + (k1 * 2 + blk) * 128 + part * 64 + c * 8)

    def tf_rows(c, blk, ka, b, part):
        return rows8(TF_OFF + (c % 2) * 8 + blk * 512 + ((ka * 8 + b) * 2 + part) * 8)

    def fwd_pass1(c, blk, re, im):
        for b in range(8):
            z = _fft([(re[(b * 4 + a) * 8:(b * 4 + a + 1) * 8], im[(b * 4 + a) * 8:(b * 4 + a + 1) * 8])
                      for a in range(4)], -1)
            for ka in range(4):
                zr, zi = _cmul(z[ka], -2 * np.pi * b * ka / N1)
                pb[tf_rows(c, blk, ka, b, 0), :] = _u32(zr)
                pb[tf_rows(c, blk, ka, b, 1), :] = _u32(zi)

    def fwd_pass2(c, blk, ka):
        z = _fft([(_f32(pb[tf_rows(c, blk, ka, b, 0), :]), _f32(pb[tf_rows(c, blk, ka, b, 1), :]))
                  for b in range(8)], -1)
        for kb in range(8):
            pb[u_rows(ka + 4 * kb, blk, 0, c, U_OFF), :] = _u32(z[kb][0])
            pb[u_rows(ka + 4 * kb, blk, 1, c, U_OFF), :] = _u32(z[kb][1])

    def fwd_even(c):
        x0, x1, x2, x3 = ax_blocks(c)
        p, q = x0 + x2, x1 + x3
        t0 = _dot((p + q).astype(BF), _bf(dmat_s[0, 0:64, 0:128]))
        t2 = _dot((p - q).astype(BF), _bf(dmat_s[0, 0:64, 128:256]))
        re = jnp.where(lane_lo, t0, t2)
        im = jnp.where(lane == 0, 0.0, pltpu.roll(jnp.where(lane_lo, t2, t0), 127, 1))
        n = jnp.zeros((8, 128), F32)
        for pos, s1 in enumerate(order):
            v = t0[pos * 8:(pos + 1) * 8]
            n = jnp.where(lane == s1, v if s1 == 1 else pltpu.roll(v, (s1 - 1) % 128, 1), n)
        return re, im, n

    def fwd_nyq(c, n):
        u = _dot(n.astype(BF), _bf(dmat_s[0, 128:192, :]))
        ur, ui = u[:, 0:128], u[:, 128:256]
        ct, st = misc_s[rows8(80 + c * 8), :], misc_s[rows8(80 + N2 + c * 8), :]
        return ur * ct + ui * st, ui * ct - ur * st

    def put_nyq(c, u):
        pb[u_rows(N1, 0, 0, c, U_OFF), :] = _u32(u[0])
        pb[u_rows(N1, 0, 1, c, U_OFF), :] = _u32(u[1])

    def fwd_odd(c):
        x0, x1, x2, x3 = ax_blocks(c)
        a, b = x0 - x2, x1 - x3
        r = pltpu.roll(jnp.where(lane_half, b, (a - b) * rt), 64, 1)
        p, q = jnp.where(lane_half, a, r), jnp.where(lane_half, r, (a + b) * rt)
        tp = _dot((p + q).astype(BF), _bf(dmat_s[0, 64:128, 0:128]))
        tm = _dot((p - q).astype(BF), _bf(dmat_s[0, 64:128, 128:256]))
        return jnp.where(lane_plus, tp, tm), pltpu.roll(jnp.where(lane_plus, tm, tp), 126, 1)

    def cfilter(z, wr, wi):
        zr, zi = z[0:64], z[64:128]
        return jnp.concatenate([zr * wr - zi * wi, zr * wi + zi * wr], axis=0).astype(BF)

    def tile_rows(k1, off=0):
        return pl.ds(pl.multiple_of(off + k1 * 256, 128), 256)

    def mid_a(k1):
        t = _f32(pb[tile_rows(k1, U_OFF), :])
        return _dot(_bf(smat_s[k1, 0]), jnp.concatenate([t[0:128], t[128:256]], axis=1).astype(BF))

    def mid_f(grp, low, z):
        w = [pb.at[pl.ds(pl.multiple_of(F_OFF + (a * 4 + grp) * 512, 8), 512)][pl.ds(low, 64, stride=8), :]
             for a in range(2)]
        wr, wi = [jnp.concatenate([_f32(v << 16), _f32(v & jnp.uint32(HI_MASK))], axis=1) for v in w]
        return cfilter(z, wr, wi)

    def mid_b(k1, y):
        v = _dot(_bf(smat_s[k1, 1]), y)
        big[tile_rows(k1, V_OFF), :] = jnp.concatenate([v[:, 0:128], v[:, 128:256]], axis=0)

    def nyq_a():
        z = _dot(_bf(smat_s[N1, 0]), _f32(pb[pl.ds(U_OFF + N1 * 256, 128), :]).astype(BF))
        w = []
        for a in range(2):
            g = jnp.concatenate([fraw[a, 256:257, t * 128:(t + 1) * 128].astype(F32) for t in range(16)], axis=0)
            w.append(jnp.concatenate([g] + [pltpu.roll(g, 128 - 32 * q, 1) for q in range(1, 4)], axis=0))
        return cfilter(z, *w)

    def nyq_b(y):
        big[pl.ds(V_OFF + N1 * 256, 128), :] = _dot(_bf(smat_s[N1, 1]), y)

    def inv_pass1(c, blk, ka):
        z = _fft([(big[u_rows(ka + 4 * kb, blk, 0, c, V_OFF), :], big[u_rows(ka + 4 * kb, blk, 1, c, V_OFF), :])
                  for kb in range(8)], 1)
        for b in range(8):
            zr, zi = _cmul(z[b], 2 * np.pi * b * ka / N1)
            big[t_rows(ka, b, 0), :] = zr
            big[t_rows(ka, b, 1), :] = zi

    def inv_nyq(c):
        vr, vi = big[u_rows(N1, 0, 0, c, V_OFF), :], big[u_rows(N1, 0, 1, c, V_OFF), :]
        ct, st = misc_s[rows8(80 + c * 8), :], misc_s[rows8(80 + N2 + c * 8), :]
        m = _bf(dmat_s[1, 128:192, :])
        return (_dot((vr * ct - vi * st).astype(BF), m[:, 0:128])
                + _dot((vi * ct + vr * st).astype(BF), m[:, 128:256]))

    def inv_pass2(blk, b, n):
        z = _fft([(big[t_rows(ka, b, 0), :], big[t_rows(ka, b, 1), :]) for ka in range(4)], 1)
        for a in range(4):
            re, im = z[a]
            s1 = 8 * a + b
            if blk == 0:
                im = pltpu.roll(im, 1, 1)
                nv = n if s1 == 1 else pltpu.roll(n, (1 - s1) % 128, 1)
                re, im = jnp.where(lane == 1, nv, jnp.where(lane_lo, re, im)), jnp.where(lane_lo, im, re)
            else:
                im = pltpu.roll(im, 2, 1)
                re, im = jnp.where(lane_plus, re, im), jnp.where(lane_plus, im, re)
            big[pl.ds(L_OFF + (2 * blk) * 256 + s1 * 8, 8), :] = re
            big[pl.ds(L_OFF + (2 * blk + 1) * 256 + s1 * 8, 8), :] = im

    def inv_out(c):
        lhs = [big[pl.ds(L_OFF + i * 256, 256), :] for i in range(4)]
        c0 = _dot(lhs[0].astype(BF), _bf(dmat_s[1, 0:64, 0:128]))
        c2 = _dot(lhs[1].astype(BF), _bf(dmat_s[1, 0:64, 128:256]))
        lp = _dot(lhs[2].astype(BF), _bf(dmat_s[1, 64:128, 0:128]))
        lm = _dot(lhs[3].astype(BF), _bf(dmat_s[1, 64:128, 128:256]))
        pp, qq = lp + lm, lp - lm
        r = pltpu.roll(jnp.where(lane_half, qq, pp), 64, 1)
        p, q = jnp.where(lane_half, pp, (r + qq) * rt), jnp.where(lane_half, r, (qq - r) * rt)
        e, f = c0 + c2, c0 - c2
        y = jnp.concatenate([e + p, f + q, e - p, f - q], axis=1)
        oa_s[:, rows8(c * 8), :] = y.reshape(N1, 8, DM).astype(BF)

    def head_words(hh, n):
        a = wtmp[pl.ds(hh // 2, n, stride=8), :]
        b = wtmp[pl.ds(4 + hh // 2, n, stride=8), :]
        return (a >> 16) | (b & jnp.uint32(HI_MASK)) if hh % 2 else (a & 0xFFFF) | (b << 16)

    def head_weights(t, hh):
        w = head_words(hh, 256)
        w_s[t * 8 + hh] = w
        return w

    def relayout_a(t):
        for dc in range(8):
            v = wraw[t, dc * 64:(dc + 1) * 64]
            wtmp[dc * 256:(dc + 1) * 256, :] = pltpu.bitcast(v.reshape(512, 128), U32)
        head_weights(t, 0)

    def early_proj(t, hooks):
        for jj in range(4):
            res = []
            for hh in (2 * jj, 2 * jj + 1):
                w = w_s[t * 8] if hh == 0 else head_weights(t, hh)
                r = _dot(_bf(jnp.concatenate([x0_s[k] for k in range(4)], axis=1)), _bf(w))
                res.append(r.reshape(NSEG, 8, 128))
                for tm, f, pinned in hooks:
                    if tm // 8 == hh:
                        if pinned:
                            pb[rows8(TK_OFF + (t % 2) * 8), :] = _u32(r[(tm % 8) * 64:(tm % 8) * 64 + 8])
                        f()
            big[pl.ds(pl.multiple_of(P_OFF + (t * 4 + jj) * 1024, 1024), 1024), :] = (
                jnp.concatenate(res, axis=1).reshape(1024, 128))

    ONLY = os.environ.get("ONLY", "")
    def phase_0(kt, carry):
        for c in first_copies(kt):
            c.wait()
        for dc in range(2):
            v = wraw[0, pl.ds(pl.multiple_of(kt * 128 + dc * 64, 64), 64)]
            wtmp[dc * 256:(dc + 1) * 256, :] = _u32(v.reshape(512, 128))
        xk = _u32(x0raw[kt].reshape(NSEG * 8, 128))
        x0_s[kt] = xk
        for jj in range(4):
            res = []
            for hh in (2 * jj, 2 * jj + 1):
                w = head_words(hh, 64)
                w_s[hh, pl.ds(pl.multiple_of(kt * 64, 64), 64), :] = w
                res.append(_dot(_bf(xk), _bf(w)).reshape(NSEG, 8, 128))
            rows = pl.ds(P_OFF + jj * 1024, 1024)
            big[rows, :] = jnp.where(kt > 0, big[rows, :], 0.0) + jnp.concatenate(res, axis=1).reshape(1024, 128)
        return carry

    with jax.named_scope("s_start"):
        for kt in range(4):
            for c in first_copies(kt):
                c.start()
        for g in range(1, 4):
            w_copy(0, g).start()
        lax.fori_loop(0, 4, phase_0, 0)
        w_copy(1, 0).start()
        for c in early + chunk_copies(0):
            c.start()

    def phase_a(t, carry):
        w_copy(1, t).start()
        for c in chunk_copies(t):
            c.start()

        @pl.when(t <= 2)
        def _():
            w_copy(0, t).wait()
            relayout_a(t)

        @pl.when(t >= 2)
        def _():
            cp(w_h[0].at[:, pl.ds(0, 8), :], wraw.at[t + 1], sem_w.at[t + 1]).wait()

        early_proj(t, [])
        relayout_a(jnp.where(t >= 2, t + 1, t))
        return carry

    with jax.named_scope("s_pa"):
        lax.fori_loop(1, 4, phase_a, 0) if ONLY in ('', 'pb') else None
    for c in early:
        c.wait()

    def phase_b(i, carry):
        t = i + 4
        tn = jnp.minimum(t + 1, 11)

        @pl.when(i < 4)
        def _():
            w_copy(2, i).start()
            for c in chunk_copies(i + 4):
                c.start()

        @pl.when(i == 4)
        def _():
            for c in late:
                c.start()

        @pl.when(i < 7)
        def _():
            cp(w_h[0].at[:, pl.ds(0, 8), :], wraw.at[tn], sem_w.at[tn]).wait()

        for c in chunk_copies(i):
            c.wait()

        def wo_retile(n):
            v = _u32(woraw[pl.ds(pl.multiple_of(i * 512, 512), 512), n * 128:(n + 1) * 128])
            wo_s[n * 8 + i] = v

        box = {}
        t_om, t_f, t_o1, t_o2, t_em, t_e1, t_n, t_e2, t_pn, dt = [
            int(v) for v in os.environ.get("PBS", "0,40,8,17,0,16,25,28,33,2").split(",")]
        hooks = [(t_f + dt * k, lambda k=k: filt_prep(i, k // 2, k % 2), False) for k in range(4)]
        hooks += [(t_om, lambda: box.update(o=fwd_odd(i)), False),
                  (t_o1, lambda: fwd_pass1(i, 1, *box["o"]), False),
                  (t_em, lambda: box.update(e=fwd_even(i)), False),
                  (t_e1, lambda: fwd_pass1(i, 0, *box["e"][:2]), False),
                  (t_n, lambda: box.update(n=fwd_nyq(i, box["e"][2])), False),
                  (t_pn, lambda: put_nyq(i, box["n"]), False)]
        hooks += [(t_o2 + dt * ka, lambda ka=ka: fwd_pass2(i, 1, ka), True) for ka in range(4)]
        hooks += [(t_e2 + dt * ka, lambda ka=ka: fwd_pass2(i, 0, ka), True) for ka in range(4)]
        hooks += [(0, lambda n=n: wo_retile(n), False) for n in range(4)]
        early_proj(t, sorted(hooks, key=lambda h: h[0]))
        relayout_a(tn)
        return carry

    with jax.named_scope("s_pb"):
        lax.fori_loop(0, 8, phase_b, 0) if ONLY in ('', 'pb') else None
    with jax.named_scope("s_nyq"):
        for c in late:
            c.wait()

    if os.environ.get("ONLY") == "pb":
        oa_s[0, 0:8, 0:128] = (big[0:8, :] + _f32(pb[U_OFF:U_OFF + 8, :]) + _f32(wo_s[0, 0:8, :]) + _f32(w_s[0, 0:8, :])).astype(BF)
        c = cp(oa_s, o_h.at[:, :, pl.ds(0, DM)], sem_oa.at[0])
        c.start()
        c.wait()
        return

    def put_late(g, res):
        for i in range(16):
            ob_s[g * 8 + i // 2, (i % 2) * 32:(i % 2) * 32 + 8, :] = res[i * 8:(i + 1) * 8].astype(BF)

    def late_proj(idx):
        g, c = idx // 16, idx % 16
        a = od_s[c, pl.ds(pl.multiple_of(g * 128, 128), 128), :].astype(BF)
        res = jnp.where(c > 0, acc_s[...], 0.0) + _dot(a, wo_rows(c))
        acc_s[...] = res
        put_late(g, res)

    def step(s, mem, hooks):
        lhs = jnp.concatenate([mem, xr_s[s].astype(F32)], axis=0).astype(BF)
        st = {}

        def proj(mi, j):
            y1 = _dot(lhs, _bf(w_s[mi * H + 2 * j]))
            y2 = _dot(lhs, _bf(w_s[mi * H + 2 * j + 1]))
            pre = big[pl.ds(pl.multiple_of(P_OFF + (mi * NP + j) * 1024 + s * 16, 16), 16), :]
            st[mi, j] = jnp.concatenate([y1, y2, pre], axis=0).astype(BF)
            st["last"] = y1[0:8]

        def pin():
            big[rows8(X_OFF + (s % 2) * 8), :] = st["last"]

        def pin2():
            pb[rows8(TK_OFF + (s % 2) * 8), :] = _u32(st["last"])

        def qk(j):
            sc = lax.dot_general(st.pop((1, j)), st.pop((0, j)), (((1,), (1,)), ((), ())),
                                 preferred_element_type=F32) + misc_s[0:80, 0:80]
            p = jnp.exp2((sc - jnp.max(sc, axis=1, keepdims=True)) * EXP_C)
            st["p", j] = (p.astype(BF), pl.reciprocal(jnp.sum(p, axis=1, keepdims=True), approx=True))

        def pv(j):
            p, rl = st.pop(("p", j))
            o = _dot(p, st.pop((2, j))) * rl
            st["o", j] = jnp.concatenate([o[0:32], o[32:64]], axis=1).astype(BF)
            od_s[j, rows8(s * 8), :] = jnp.concatenate([o[64:72], o[72:80]], axis=1)

        def op(j):
            r = _dot(st.pop(("o", j)), wo_rows(j))
            st["acc"] = r if "acc" not in st else st["acc"] + r

        units = []
        for j in range(-SK, NP):
            units += [(mi, j + SK) for mi in (0, 1) if j + SK < NP] + ([(2, j)] if j >= 0 else [])
        events = [(t, lambda mi=mi, j=j: proj(mi, j)) for t, (mi, j) in enumerate(units)]
        events += [(3 * NP + j, lambda j=j: op(j)) for j in range(NP)]
        for j in range(NP):
            tqk = units.index((1, j)) + 1 + QL
            events.append((tqk - 0.5, lambda j=j: qk(j)))
            events.append((max(tqk + PL, units.index((2, j)) + 1 + QL) - 0.4, lambda j=j: pv(j)))
        for t, fs in hooks.items():
            events += [(t - 0.3, {"pin": pin, "pin2": pin2}.get(f, f)) for f in fs]
        for _, f in sorted(events, key=lambda e: e[0]):
            f()
        out = st["acc"]
        ob_s[s // 2, pl.ds(pl.multiple_of((s % 2) * 32 + 8, 8), 24), :] = out[8:32].astype(BF)
        return out[0:8].astype(BF).astype(F32)

    def loop_a(i, mem):
        box = {}
        ha0, ha1, hf0, hf1, hn0, hn1, un, pf = [int(v) for v in os.environ.get("LAS", "10,36,0,0,27,38,3,0").split(",")]

        def stage_a(low):
            return lambda: box.update({("z", low): mid_a(8 * i + low)})

        def stage_f(low):
            return lambda: box.update({("y", low): mid_f(i, low, box["z", low])})

        def stage_b(low):
            return lambda: mid_b(8 * i + low, box["y", low])

        for u in range(4):
            hooks = {}

            def add(t, fs):
                hooks.setdefault(t, []).extend(fs)

            base = ha0 if u == 0 else 0
            if u == 0:
                add(ha0, [stage_a(0), stage_a(1)])
            add(base + hf0, ["pin2"] * pf + [stage_f(2 * u)])
            add(base + hf1, ["pin2"] * pf + [stage_f(2 * u + 1)])
            add(64 if u < 3 else ha1, [stage_b(2 * u), stage_b(2 * u + 1)])
            if u < 3:
                add(64, [stage_a(2 * u + 2), stage_a(2 * u + 3)])
            if u == un:
                add(hn0, [lambda: box.update(n=nyq_a())])
                add(hn1, [lambda: nyq_b(box["n"])])
            mem = step(4 * i + u, mem, hooks)
        return mem

    with jax.named_scope("s_la"):
        mem = lax.fori_loop(0, 16 // UA, loop_a, mem_s[...].astype(F32)) if ONLY in ('', 'la') else mem_s[...].astype(F32)

    def ob_copy(g):
        rows = pl.ds(pl.multiple_of(g * 8, 8), 8)
        return cp(ob_s.at[rows], o_h.at[rows, :, pl.ds(DM, DM)], sem_ob.at[g])

    def oa_copy(c):
        return cp(oa_s.at[:, rows8(c * 8), :], o_h.at[:, rows8(c * 8), pl.ds(0, DM)], sem_oa.at[c])

    def loop_b(i, mem):
        box = {}
        jobs = [{} for _ in range(6)]
        t1, d1, t2, d2, tn, to = [int(v) for v in os.environ.get("LBS", "7,10,2,3,39,275").split(",")]

        def add(t, fs):
            jobs[t // 64].setdefault(t % 64, []).extend(fs)

        for blk in range(2):
            for ka in range(4):
                add(128 * blk + t1 + d1 * ka, ["pin", lambda blk=blk, ka=ka: inv_pass1(i, blk, ka)])
            for b in range(8):
                add(128 * blk + 64 + t2 + d2 * b, ["pin", lambda blk=blk, b=b: inv_pass2(blk, b, box["n"])])
        add(tn, [lambda: box.update(n=inv_nyq(i))])
        add(to, [lambda: inv_out(i)])
        for u in range(6):
            jobs[u][64] = [lambda u=u: late_proj(6 * i + u)]
            mem = step(16 + 6 * i + u, mem, jobs[u])
        oa_copy(i).start()

        @pl.when((i == 2) | (i == 5))
        def _():
            ob_copy(i // 3).start()

        return mem

    with jax.named_scope("s_lb"):
        lax.fori_loop(0, 8, loop_b, mem) if ONLY in ('', 'lb') else None
    with jax.named_scope("s_tail"):
        ob_copy(2).start()
        last = [cp(ob_s.at[pl.ds(24, 8), pl.ds(r, n), :], o_h.at[pl.ds(24, 8), pl.ds(r, n), pl.ds(DM, DM)],
                   sem_ob.at[3 + k]) for k, (r, n) in enumerate([(8, 24), (40, 24), (0, 8), (32, 8)])]
        last[0].start()
        last[1].start()
        a = jnp.concatenate([od_s[c, 384:512, :] for c in range(16)], axis=1).astype(BF)
        put_late(3, _dot(a, jnp.concatenate([wo_rows(j) for j in range(NP)], axis=0)))
        last[2].start()
        last[3].start()
    with jax.named_scope("s_outwait"):
        for c in range(8):
            oa_copy(c).wait()
        for g in range(3):
            ob_copy(g).wait()
        for c in last:
            c.wait()


@jax.jit
def pallas_concat_heads__spectral_gfnet__memory_aug_recurrent_mem_tr__prompt_kernel(
        A_x, A_w_r, A_w_i, B_x, B_mem0, B_Wq, B_Wk, B_Wv, B_Wo, B_seg_len=None):
    dmat, smat, misc = _consts()
    vm = pltpu.VMEM
    out = pl.pallas_call(
        _kernel,
        out_shape=jax.ShapeDtypeStruct((N1, N2, 2 * DM), BF),
        in_specs=[pl.BlockSpec(memory_space=pl.ANY)] * 12,
        out_specs=pl.BlockSpec(memory_space=pl.ANY),
        scratch_shapes=[
            vm((12, DM, 8, DH), BF), vm((PB_ROWS, 128), U32), vm((2048, 128), U32), vm((3 * H, DM // 2, DH), U32), vm((H, DM // 2, DH), U32),
            vm((H * DH, DM), BF),
            vm((BIG_ROWS, 128), F32), vm((NP, NSEG * 8, 2 * DH), F32), vm((128, DM), F32),
            vm((4, NSEG, 8, 128), BF), vm((4, NSEG * 4, 128), U32), vm((NSEG, 24, DM), BF), vm((MEM, DM), BF),
            vm(misc.shape, F32),
            vm((N1, N2, DM), BF), vm((2, 257, S), BF),
            vm(dmat.shape, U32), vm(smat.shape, U32),
            vm((N1, N2, DM), BF), vm((N1, N2, DM), BF),
            pltpu.SemaphoreType.DMA((12,)), pltpu.SemaphoreType.DMA((8,)), pltpu.SemaphoreType.DMA((6,)),
            pltpu.SemaphoreType.DMA((8,)), pltpu.SemaphoreType.DMA((7,)), pltpu.SemaphoreType.DMA((4,)),
        ],
        compiler_params=pltpu.CompilerParams(vmem_limit_bytes=120 * 1024 * 1024, disable_bounds_checks=NOCHK,
                                             disable_semaphore_checks=NOCHK),
    )(A_x.reshape(N1, N2, DM), A_w_r.T, A_w_i.T,
      B_x.reshape(NSEG, SEG, DM), B_mem0.reshape(MEM, DM), B_Wq, B_Wk, B_Wv, B_Wo.reshape(H * DH, DM),
      jnp.asarray(dmat), jnp.asarray(smat), jnp.asarray(misc))
    return out.reshape(1, S, 2 * DM)
```

```python
import numpy as np
import jax
import jax.numpy as jnp
from jax import lax
import jax.experimental.pallas as pl
import jax.experimental.pallas.tpu as pltpu

S, DM, H, DH, MEM, SEG = 2048, 512, 32, 128, 8, 32
NSEG = S // SEG
NP = H // 2
N1, N2 = 32, 64
BF, F32, U32 = jnp.bfloat16, jnp.float32, jnp.uint32
EXP_C = float(DH ** -0.5 * np.log2(np.e))
HI_MASK = 0xFFFF0000

P_OFF = 0
T_OFF = P_OFF + 3 * NP * NSEG * 16
L_OFF = T_OFF + 64 * 8
V_OFF = L_OFF + 4 * 256
X_OFF = V_OFF + (2 * N1 + 1) * 128
BIG_ROWS = X_OFF + 64
TK_OFF = 0
TF_OFF = TK_OFF + 24
F_OFF = TF_OFF + 2 * 512 + 8
U_OFF = F_OFF + 8 * 512 + 96
PB_ROWS = U_OFF + (2 * N1 + 1) * 128

STEP_A = (3, 6, 1)
STEP_B = (3, 5, 1)
SCHED_PB = (0, 40, 8, 17, 0, 16, 25, 28, 33, 2)
SCHED_LA = (16, 30, 16, 25, 3)
SCHED_LB = (8, 12, 11, 3, 5, 301, 0)


def _pack_rows(m):
    f = np.ascontiguousarray(m, dtype=np.float32).view(np.uint32)
    r = ((f + 0x7FFF + ((f >> 16) & 1)) >> 16).astype(np.uint32)
    return r[..., 0::2, :] | (r[..., 1::2, :] << 16)


def _consts():
    l = np.arange(128)
    d2 = np.arange(128)[:, None]
    lo = (l % 2) == 0
    a_re = 2 * np.pi * d2 * (2 * l)[None, :] / DM
    a_im = 2 * np.pi * d2 * (2 * ((l - 1) % 128))[None, :] / DM
    m0 = np.where(lo[None, :], np.cos(a_re), -np.sin(a_im))
    m0[:, 1] = (-1.0) ** np.arange(128)
    m2 = np.where(lo[None, :], -np.sin(a_im), np.cos(a_re))
    e = np.arange(64)[:, None]

    def odd_cols(lanes):
        kd = 2 * lanes + 1
        ang = 2 * np.pi * e * kd[None, :] / DM
        sg = np.where(kd % 4 == 1, 1.0, -1.0)[None, :]
        return (np.concatenate([np.cos(ang), -sg * np.sin(ang)], axis=0),
                np.concatenate([-np.sin(ang), -sg * np.cos(ang)], axis=0))

    plus = (l % 4 == 0) | (l % 4 == 3)
    o_re, o_im = odd_cols(l)[0], odd_cols((l - 2) % 128)[1]
    mp = np.where(plus[None, :], o_re, o_im)
    mm = np.where(plus[None, :], o_im, o_re)
    sc = 2.0 / (S * DM)
    m0i = m0.T * sc
    m0i[0] /= 2
    m0i[1] /= 2
    a32 = 2 * np.pi * np.outer(np.arange(N1), np.arange(N1)) / N1
    c32, s32 = np.zeros((128, 128)), np.zeros((128, 128))
    c32[:N1, :N1], s32[:N1, :N1] = np.cos(a32), -np.sin(a32)
    nf = np.concatenate([c32, s32], axis=1)
    dfw = np.concatenate([np.concatenate([m0, m2], axis=1), np.concatenate([mp, mm], axis=1), nf], axis=0)
    dinv = np.concatenate([np.concatenate([m0i, m2.T * sc], axis=1),
                           np.concatenate([mp.T, mm.T], axis=1) * sc, nf], axis=0)
    k1 = np.arange(N1)[:, None, None]
    k2 = np.arange(N2)[None, :, None]
    s2 = np.arange(N2)[None, None, :]
    th = 2 * np.pi * ((s2 * (k1 + N1 * k2)) % S) / S
    rho = np.arange(N2)
    th = np.concatenate([th, th[:1, 4 * (rho % 16) + rho // 16]], axis=0)
    c, s = np.cos(th), np.sin(th)
    mf = np.concatenate([np.concatenate([c, s], 2), np.concatenate([-s, c], 2)], 1)
    dmat = _pack_rows(np.stack([dfw, dinv]))
    smat = _pack_rows(np.stack([mf, mf.transpose(0, 2, 1)], axis=1))
    head = np.concatenate([np.zeros(32), np.ones(32), np.zeros(8), np.ones(8)])
    pos = np.concatenate([np.arange(8), np.arange(16, 40)] * 2 + [np.arange(8, 16)] * 2)
    same = head[:, None] == head[None, :]
    ok = same & ((pos[:, None] < MEM) | (pos[:, None] >= pos[None, :]))
    misc = np.zeros((96 + 2 * N2, 128), np.float32)
    misc[:80, :80] = np.where(ok, 0.0, np.where(same, -1e9 * DH ** 0.5, -np.inf))
    atw = 2 * np.pi * np.outer(np.arange(N2), np.arange(128) % N1) / S
    misc[96:96 + N2], misc[96 + N2:] = np.cos(atw), np.sin(atw)
    return dmat, smat, misc


def _cmul(z, ang):
    re, im = z
    c, s = float(np.cos(ang)), float(np.sin(ang))
    if abs(s) < 1e-12:
        return (re, im) if c > 0 else (-re, -im)
    if abs(c) < 1e-12:
        return (-im, re) if s > 0 else (im, -re)
    if abs(abs(c) - abs(s)) < 1e-12:
        return ((re - im) * c, (re + im) * c) if c * s > 0 else ((re + im) * c, (im - re) * c)
    return re * c - im * s, re * s + im * c


def _fft(x, sign):
    n = len(x)
    if n == 1:
        return x
    if n == 2:
        (ar, ai), (br, bi) = x
        return [(ar + br, ai + bi), (ar - br, ai - bi)]
    ev, z1, z3 = _fft(x[0::2], sign), _fft(x[1::4], sign), _fft(x[3::4], sign)
    out = [None] * n
    q = n // 4
    for k in range(q):
        ar, ai = _cmul(z1[k], sign * 2 * np.pi * k / n)
        br, bi = _cmul(z3[k], sign * 2 * np.pi * 3 * k / n)
        sr, si, dr, di = ar + br, ai + bi, ar - br, ai - bi
        (er, ei), (fr, fi) = ev[k], ev[k + q]
        out[k] = (er + sr, ei + si)
        out[k + 2 * q] = (er - sr, ei - si)
        plus, minus = (fr - di, fi + dr), (fr + di, fi - dr)
        out[k + q], out[k + 3 * q] = (plus, minus) if sign > 0 else (minus, plus)
    return out


def _dot(a, b):
    return jnp.dot(a, b, preferred_element_type=F32)


def _bf(words):
    return pltpu.bitcast(words, BF)


def _f32(words):
    return pltpu.bitcast(words, F32)


def _u32(x):
    return pltpu.bitcast(x, U32)


def _rows8(off):
    return pl.ds(pl.multiple_of(off, 8), 8)


def _kernel(ax_h, wr_h, wi_h, bx_h, mem_h, wq_h, wk_h, wv_h, wo_h, dmat_h, smat_h, misc_h,
            o_h,
            wraw, pb, wtmp, w_s, wo_s, woraw, big, od_s, acc_s, x0raw, x0_s, xr_s, misc_s,
            ax_s, fraw, dmat_s, smat_s, oa_s, ob_s, mem_s,
            sem_w, sem_c, sem_m, sem_oa, sem_ob, sem_f):
    w_h = (wk_h, wq_h, wv_h)
    cp = pltpu.make_async_copy

    def w_copy(m, g):
        return cp(w_h[m].at[:, pl.ds(pl.multiple_of(8 * g, 8), 8), :], wraw.at[4 * m + g], sem_w.at[4 * m + g])

    def w_wait(t):
        cp(wraw.at[t], wraw.at[t], sem_w.at[t]).wait()

    def chunk_copies(i):
        rows = pl.ds(pl.multiple_of(i * 512, 512), 512)
        cols = pl.ds(pl.multiple_of(i * 256, 256), 256)
        return [cp(wo_h.at[rows], woraw.at[rows], sem_c.at[i]),
                cp(ax_h.at[:, _rows8(i * 8), :], ax_s.at[:, _rows8(i * 8), :], sem_c.at[i]),
                cp(wr_h.at[:, cols], fraw.at[0, :, cols], sem_c.at[i]),
                cp(wi_h.at[:, cols], fraw.at[1, :, cols], sem_c.at[i])]

    def first_copies(kt):
        d = pl.ds(pl.multiple_of(kt * 128, 128), 128)
        return [cp(bx_h.at[:, pl.ds(0, 8), d], x0raw.at[kt], sem_f.at[kt]),
                cp(wk_h.at[d, pl.ds(0, 8), :], wraw.at[0, d], sem_f.at[kt])]

    early = [cp(dmat_h, dmat_s, sem_m.at[0]), cp(misc_h, misc_s, sem_m.at[1]), cp(mem_h, mem_s.at[0], sem_m.at[2])]
    late = [cp(bx_h.at[:, pl.ds(8, 24), :], xr_s, sem_m.at[3]), cp(smat_h, smat_s, sem_m.at[4])]

    def ob_copy(g):
        return cp(ob_s.at[_rows8(g * 8)], o_h.at[_rows8(g * 8), :, pl.ds(DM, DM)], sem_ob.at[g])

    def oa_copy(c):
        return cp(oa_s.at[:, _rows8(c * 8), :], o_h.at[:, _rows8(c * 8), pl.ds(0, DM)], sem_oa.at[c])

    lane = lax.broadcasted_iota(jnp.int32, (1, 128), 1)
    lane_lo = (lane & 1) == 0
    lane_plus = ((lane + 1) & 2) == 0
    lane_half = lane < 64
    rt = float(np.sqrt(0.5))

    order = [8 * a + b for b in range(8) for a in range(4)]

    def filt_prep(i, h, a):
        col = pl.ds(pl.multiple_of((2 * i + h) * 128, 128), 128)
        t = _u32(fraw[a, 0:256, col]).T
        for q in range(16):
            pb[_rows8(F_OFF + (a * 4 + q % 4) * 512 + ((2 * i + h) * 4 + q // 4) * 8), :] = t[q * 8:(q + 1) * 8]

    def ax_blocks(c):
        v = jnp.concatenate([ax_s[s1, _rows8(c * 8), :].astype(F32) for s1 in order], axis=0)
        return [v[:, i * 128:(i + 1) * 128] for i in range(4)]

    def t_rows(ka, b, part):
        return pl.ds(T_OFF + ((ka * 8 + b) * 2 + part) * 8, 8)

    def tf_rows(c, blk, ka, b, part):
        return _rows8(TF_OFF + (c % 2) * 8 + blk * 512 + ((ka * 8 + b) * 2 + part) * 8)

    def u_rows(off, k1, blk, part, c):
        return _rows8(off + (k1 * 2 + blk) * 128 + part * 64 + c * 8)

    def tile_rows(off, k1):
        return pl.ds(pl.multiple_of(off + k1 * 256, 128), 256)

    def twiddles(c):
        return misc_s[_rows8(96 + c * 8), :], misc_s[_rows8(96 + N2 + c * 8), :]

    def fwd_even(c):
        x0, x1, x2, x3 = ax_blocks(c)
        p, q = x0 + x2, x1 + x3
        t0 = _dot((p + q).astype(BF), _bf(dmat_s[0, 0:64, 0:128]))
        t2 = _dot((p - q).astype(BF), _bf(dmat_s[0, 0:64, 128:256]))
        re = jnp.where(lane_lo, t0, t2)
        im = jnp.where(lane == 0, 0.0, pltpu.roll(jnp.where(lane_lo, t2, t0), 127, 1))
        n = jnp.zeros((8, 128), F32)
        for pos, s1 in enumerate(order):
            v = t0[pos * 8:(pos + 1) * 8]
            n = jnp.where(lane == s1, v if s1 == 1 else pltpu.roll(v, (s1 - 1) % 128, 1), n)
        return re, im, n

    def fwd_odd(c):
        x0, x1, x2, x3 = ax_blocks(c)
        a, b = x0 - x2, x1 - x3
        r = pltpu.roll(jnp.where(lane_half, b, (a - b) * rt), 64, 1)
        p, q = jnp.where(lane_half, a, r), jnp.where(lane_half, r, (a + b) * rt)
        tp = _dot((p + q).astype(BF), _bf(dmat_s[0, 64:128, 0:128]))
        tm = _dot((p - q).astype(BF), _bf(dmat_s[0, 64:128, 128:256]))
        return jnp.where(lane_plus, tp, tm), pltpu.roll(jnp.where(lane_plus, tm, tp), 126, 1)

    def fwd_pass1(c, blk, re, im):
        for b in range(8):
            z = _fft([(re[(b * 4 + a) * 8:(b * 4 + a + 1) * 8], im[(b * 4 + a) * 8:(b * 4 + a + 1) * 8])
                      for a in range(4)], -1)
            for ka in range(4):
                zr, zi = _cmul(z[ka], -2 * np.pi * b * ka / N1)
                pb[tf_rows(c, blk, ka, b, 0), :] = _u32(zr)
                pb[tf_rows(c, blk, ka, b, 1), :] = _u32(zi)

    def fwd_pass2(c, blk, ka):
        z = _fft([(_f32(pb[tf_rows(c, blk, ka, b, 0), :]), _f32(pb[tf_rows(c, blk, ka, b, 1), :]))
                  for b in range(8)], -1)
        for kb in range(8):
            pb[u_rows(U_OFF, ka + 4 * kb, blk, 0, c), :] = _u32(z[kb][0])
            pb[u_rows(U_OFF, ka + 4 * kb, blk, 1, c), :] = _u32(z[kb][1])

    def fwd_nyq(c, n):
        u = _dot(n.astype(BF), _bf(dmat_s[0, 128:192, :]))
        ur, ui = u[:, 0:128], u[:, 128:256]
        ct, st = twiddles(c)
        return ur * ct + ui * st, ui * ct - ur * st

    def put_nyq(c, u):
        pb[u_rows(U_OFF, N1, 0, 0, c), :] = _u32(u[0])
        pb[u_rows(U_OFF, N1, 0, 1, c), :] = _u32(u[1])

    def cfilter(z, wr, wi):
        zr, zi = z[0:64], z[64:128]
        return jnp.concatenate([zr * wr - zi * wi, zr * wi + zi * wr], axis=0).astype(BF)

    def mid_a(k1):
        t = _f32(pb[tile_rows(U_OFF, k1), :])
        return _dot(_bf(smat_s[k1, 0]), jnp.concatenate([t[0:128], t[128:256]], axis=1).astype(BF))

    def mid_f(grp, low, z):
        w = [pb.at[pl.ds(pl.multiple_of(F_OFF + (a * 4 + grp) * 512, 8), 520)][pl.ds(low, 64, stride=8), :]
             for a in range(2)]
        wr, wi = [jnp.concatenate([_f32(v << 16), _f32(v & jnp.uint32(HI_MASK))], axis=1) for v in w]
        return cfilter(z, wr, wi)

    def mid_b(k1, y):
        v = _dot(_bf(smat_s[k1, 1]), y)
        big[tile_rows(V_OFF, k1), :] = jnp.concatenate([v[:, 0:128], v[:, 128:256]], axis=0)

    def nyq_a():
        z = _dot(_bf(smat_s[N1, 0]), _f32(pb[pl.ds(U_OFF + N1 * 256, 128), :]).astype(BF))
        w = []
        for a in range(2):
            g = jnp.concatenate([fraw[a, 256:257, t * 128:(t + 1) * 128].astype(F32) for t in range(16)], axis=0)
            w.append(jnp.concatenate([g] + [pltpu.roll(g, 128 - 32 * q, 1) for q in range(1, 4)], axis=0))
        return cfilter(z, *w)

    def nyq_b(y):
        big[pl.ds(V_OFF + N1 * 256, 128), :] = _dot(_bf(smat_s[N1, 1]), y)

    def inv_pass1(c, blk, ka):
        z = _fft([(big[u_rows(V_OFF, ka + 4 * kb, blk, 0, c), :], big[u_rows(V_OFF, ka + 4 * kb, blk, 1, c), :])
                  for kb in range(8)], 1)
        for b in range(8):
            zr, zi = _cmul(z[b], 2 * np.pi * b * ka / N1)
            big[t_rows(ka, b, 0), :] = zr
            big[t_rows(ka, b, 1), :] = zi

    def inv_nyq(c):
        vr, vi = big[u_rows(V_OFF, N1, 0, 0, c), :], big[u_rows(V_OFF, N1, 0, 1, c), :]
        ct, st = twiddles(c)
        m = _bf(dmat_s[1, 128:192, :])
        return (_dot((vr * ct - vi * st).astype(BF), m[:, 0:128])
                + _dot((vi * ct + vr * st).astype(BF), m[:, 128:256]))

    def inv_pass2(blk, b, n):
        z = _fft([(big[t_rows(ka, b, 0), :], big[t_rows(ka, b, 1), :]) for ka in range(4)], 1)
        for a in range(4):
            re, im = z[a]
            s1 = 8 * a + b
            if blk == 0:
                im = pltpu.roll(im, 1, 1)
                nv = n if s1 == 1 else pltpu.roll(n, (1 - s1) % 128, 1)
                re, im = jnp.where(lane == 1, nv, jnp.where(lane_lo, re, im)), jnp.where(lane_lo, im, re)
            else:
                im = pltpu.roll(im, 2, 1)
                re, im = jnp.where(lane_plus, re, im), jnp.where(lane_plus, im, re)
            big[pl.ds(L_OFF + (2 * blk) * 256 + s1 * 8, 8), :] = re
            big[pl.ds(L_OFF + (2 * blk + 1) * 256 + s1 * 8, 8), :] = im

    def inv_out(c):
        lhs = [big[pl.ds(L_OFF + i * 256, 256), :] for i in range(4)]
        c0 = _dot(lhs[0].astype(BF), _bf(dmat_s[1, 0:64, 0:128]))
        c2 = _dot(lhs[1].astype(BF), _bf(dmat_s[1, 0:64, 128:256]))
        lp = _dot(lhs[2].astype(BF), _bf(dmat_s[1, 64:128, 0:128]))
        lm = _dot(lhs[3].astype(BF), _bf(dmat_s[1, 64:128, 128:256]))
        pp, qq = lp + lm, lp - lm
        r = pltpu.roll(jnp.where(lane_half, qq, pp), 64, 1)
        p, q = jnp.where(lane_half, pp, (r + qq) * rt), jnp.where(lane_half, r, (qq - r) * rt)
        e, f = c0 + c2, c0 - c2
        y = jnp.concatenate([e + p, f + q, e - p, f - q], axis=1)
        oa_s[:, _rows8(c * 8), :] = y.reshape(N1, 8, DM).astype(BF)

    def head_words(hh, n):
        a = wtmp[pl.ds(hh // 2, n, stride=8), :]
        b = wtmp[pl.ds(4 + hh // 2, n, stride=8), :]
        return (a >> 16) | (b & jnp.uint32(HI_MASK)) if hh % 2 else (a & 0xFFFF) | (b << 16)

    def head_weights(t, hh):
        w = head_words(hh, 256)
        w_s[t * 8 + hh] = w
        return w

    def stage_chunk(t):
        for dc in range(8):
            wtmp[dc * 256:(dc + 1) * 256, :] = _u32(wraw[t, dc * 64:(dc + 1) * 64].reshape(512, 128))
        head_weights(t, 0)

    def early_proj(t, hooks):
        for jj in range(4):
            res = []
            for hh in (2 * jj, 2 * jj + 1):
                w = w_s[t * 8] if hh == 0 else head_weights(t, hh)
                r = _dot(_bf(jnp.concatenate([x0_s[k] for k in range(4)], axis=1)), _bf(w))
                res.append(r.reshape(NSEG, 8, 128))
                for tm, f, pinned in hooks:
                    if tm // 8 == hh:
                        if pinned:
                            pb[_rows8(TK_OFF + (t % 2) * 8), :] = _u32(r[(tm % 8) * 64:(tm % 8) * 64 + 8])
                        f()
            big[pl.ds(pl.multiple_of(P_OFF + (t * 4 + jj) * 1024, 1024), 1024), :] = (
                jnp.concatenate(res, axis=1).reshape(1024, 128))

    def phase_0(kt, carry):
        for c in first_copies(kt):
            c.wait()
        for dc in range(2):
            v = wraw[0, pl.ds(pl.multiple_of(kt * 128 + dc * 64, 64), 64)]
            wtmp[dc * 256:(dc + 1) * 256, :] = _u32(v.reshape(512, 128))
        xk = _u32(x0raw[kt].reshape(NSEG * 8, 128))
        x0_s[kt] = xk
        for jj in range(4):
            res = []
            for hh in (2 * jj, 2 * jj + 1):
                w = head_words(hh, 64)
                w_s[hh, pl.ds(pl.multiple_of(kt * 64, 64), 64), :] = w
                res.append(_dot(_bf(xk), _bf(w)).reshape(NSEG, 8, 128))
            rows = pl.ds(P_OFF + jj * 1024, 1024)
            big[rows, :] = jnp.where(kt > 0, big[rows, :], 0.0) + jnp.concatenate(res, axis=1).reshape(1024, 128)
        return carry

    def phase_a(t, carry):
        w_copy(1, t).start()
        for c in chunk_copies(t):
            c.start()

        @pl.when(t <= 2)
        def _():
            w_wait(t)
            stage_chunk(t)

        @pl.when(t >= 2)
        def _():
            w_wait(t + 1)

        early_proj(t, [])
        stage_chunk(jnp.where(t >= 2, t + 1, t))
        return carry

    def phase_b(i, carry):
        t = i + 4
        tn = jnp.minimum(t + 1, 11)

        @pl.when(i < 4)
        def _():
            w_copy(2, i).start()
            for c in chunk_copies(i + 4):
                c.start()

        @pl.when(i == 4)
        def _():
            for c in late:
                c.start()

        @pl.when(i < 7)
        def _():
            w_wait(tn)

        for c in chunk_copies(i):
            c.wait()

        def wo_retile(n):
            wo_s[n * 8 + i] = _u32(woraw[pl.ds(pl.multiple_of(i * 512, 512), 512), n * 128:(n + 1) * 128])

        box = {}
        t_om, t_f, t_o1, t_o2, t_em, t_e1, t_n, t_e2, t_pn, dt = SCHED_PB
        hooks = [(t_f + dt * k, lambda k=k: filt_prep(i, k // 2, k % 2), False) for k in range(4)]
        hooks += [(t_om, lambda: box.update(o=fwd_odd(i)), False),
                  (t_o1, lambda: fwd_pass1(i, 1, *box["o"]), False),
                  (t_em, lambda: box.update(e=fwd_even(i)), False),
                  (t_e1, lambda: fwd_pass1(i, 0, *box["e"][:2]), False),
                  (t_n, lambda: box.update(n=fwd_nyq(i, box["e"][2])), False),
                  (t_pn, lambda: put_nyq(i, box["n"]), False)]
        hooks += [(t_o2 + dt * ka, lambda ka=ka: fwd_pass2(i, 1, ka), True) for ka in range(4)]
        hooks += [(t_e2 + dt * ka, lambda ka=ka: fwd_pass2(i, 0, ka), True) for ka in range(4)]
        hooks += [(0, lambda n=n: wo_retile(n), False) for n in range(4)]
        early_proj(t, sorted(hooks, key=lambda h: h[0]))
        stage_chunk(tn)
        return carry

    def wo_rows(j):
        r = pl.ds(pl.multiple_of((j % 2) * 128, 128), 128)
        return _bf(jnp.concatenate([wo_s[n * 8 + j // 2, r, :] for n in range(4)], axis=1))

    def put_late(g, res):
        for i in range(16):
            ob_s[g * 8 + i // 2, (i % 2) * 32:(i % 2) * 32 + 8, :] = res[i * 8:(i + 1) * 8].astype(BF)

    def late_proj(idx):
        g, c = idx // 16, idx % 16
        a = od_s[c, pl.ds(pl.multiple_of(g * 128, 128), 128), :].astype(BF)
        res = jnp.where(c > 0, acc_s[...], 0.0) + _dot(a, wo_rows(c))
        acc_s[...] = res
        put_late(g, res)

    def step(s0, u0, mem, hooks, lags):
        s = s0 + u0
        qk_lag, pv_lag, skew = lags
        lhs = jnp.concatenate([mem, xr_s[s].astype(F32)], axis=0).astype(BF)
        st = {}

        def proj(mi, j):
            y1 = _dot(lhs, _bf(w_s[mi * H + 2 * j]))
            y2 = _dot(lhs, _bf(w_s[mi * H + 2 * j + 1]))
            pre = big[pl.ds(pl.multiple_of(s0 * 16, 32) + (P_OFF + (mi * NP + j) * 1024 + u0 * 16), 16), :]
            st[mi, j] = jnp.concatenate([y1, y2, pre], axis=0).astype(BF)
            st["last"] = y1[0:8]

        def pin():
            big[pl.ds(pl.multiple_of((s0 % 4) * 16, 32) + X_OFF, 8), :] = st["last"]

        def qk(j):
            sc = lax.dot_general(st.pop((1, j)), st.pop((0, j)), (((1,), (1,)), ((), ())),
                                 preferred_element_type=F32)
            fill = misc_s[0:80, 0:80]
            sc = jnp.where(fill == 0.0, sc, fill)
            p = jnp.exp2((sc - jnp.max(sc, axis=1, keepdims=True)) * EXP_C)
            st["p", j] = (p.astype(BF), pl.reciprocal(jnp.sum(p, axis=1, keepdims=True), approx=True))

        def pv(j):
            p, rl = st.pop(("p", j))
            o = _dot(p, st.pop((2, j))) * rl
            st["o", j] = jnp.concatenate([o[0:32], o[32:64]], axis=1).astype(BF)
            od_s[j, pl.ds(pl.multiple_of(s0 * 8, 16) + u0 * 8, 8), :] = jnp.concatenate([o[64:72], o[72:80]], axis=1)

        def op(j):
            r = _dot(st.pop(("o", j)), wo_rows(j))
            st["acc"] = r if "acc" not in st else st["acc"] + r

        units = []
        for j in range(-skew, NP):
            units += [(mi, j + skew) for mi in (0, 1) if j + skew < NP] + ([(2, j)] if j >= 0 else [])
        events = [(t, lambda mi=mi, j=j: proj(mi, j)) for t, (mi, j) in enumerate(units)]
        events += [(3 * NP + j, lambda j=j: op(j)) for j in range(NP)]
        for j in range(NP):
            tqk = units.index((1, j)) + 1 + qk_lag
            events.append((tqk - 0.5, lambda j=j: qk(j)))
            events.append((max(tqk + pv_lag, units.index((2, j)) + 1 + qk_lag) - 0.4, lambda j=j: pv(j)))
        for t, fs in hooks.items():
            events += [(t - 0.3, pin if f is None else f) for f in fs]
        for _, f in sorted(events, key=lambda ev: ev[0]):
            f()
        out = st["acc"]
        ob_s[s0 // 2 + u0 // 2, (u0 % 2) * 32 + 8:(u0 % 2) * 32 + 32, :] = out[8:32].astype(BF)
        return out[0:8].astype(BF).astype(F32)

    def loop_a(i, mem):
        box = {}
        t_a, t_b, t_n0, t_n1, u_n = SCHED_LA

        def stage_a(low):
            return lambda: box.update({("z", low): mid_a(8 * i + low)})

        def stage_f(low):
            return lambda: box.update({("y", low): mid_f(i, low, box["z", low])})

        def stage_b(low):
            return lambda: mid_b(8 * i + low, box["y", low])

        for u in range(4):
            hooks = {}

            def add(t, fs):
                hooks.setdefault(t, []).extend(fs)

            if u == 0:
                add(t_a, [stage_a(0), stage_a(1)])
            add(t_a if u == 0 else 0, [stage_f(2 * u), stage_f(2 * u + 1)])
            add(64 if u < 3 else t_b, [stage_b(2 * u), stage_b(2 * u + 1)])
            if u < 3:
                add(64, [stage_a(2 * u + 2), stage_a(2 * u + 3)])
            if u == u_n:
                add(t_n0, [lambda: box.update(n=nyq_a())])
                add(t_n1, [lambda: nyq_b(box["n"])])
            mem = step(4 * i, u, mem, hooks, STEP_A)
        return mem

    def loop_b(i, mem):
        box = {}
        jobs = [{} for _ in range(6)]
        t1, d1, t2, d2, t_n, t_o, t_x = SCHED_LB

        def add(t, fs):
            u = min(t // 64, 5)
            jobs[u].setdefault(t - 64 * u, []).extend(fs)

        for blk in range(2):
            for ka in range(4):
                add(128 * blk + t1 + d1 * ka, [None, lambda blk=blk, ka=ka: inv_pass1(i, blk, ka)])
            for b in range(8):
                add(128 * blk + 64 + t2 + d2 * b, [None, lambda blk=blk, b=b: inv_pass2(blk, b, box["n"])])
        add(t_n, [lambda: box.update(n=inv_nyq(i))])
        add(t_o, [lambda: inv_out(i)])
        for u, t in enumerate(sorted([64 * u for u in range(1, 6)] + [t_x])):
            add(t, [lambda u=u: late_proj(6 * i + u)])
        for u in range(6):
            mem = step(6 * i, 16 + u, mem, jobs[u], STEP_B)
        oa_copy(i).start()

        @pl.when((i == 2) | (i == 5))
        def _():
            ob_copy(i // 3).start()

        return mem

    for kt in range(4):
        for c in first_copies(kt):
            c.start()
    for g in range(1, 4):
        w_copy(0, g).start()
    lax.fori_loop(0, 4, phase_0, 0)
    w_copy(1, 0).start()
    for c in early + chunk_copies(0):
        c.start()
    lax.fori_loop(1, 4, phase_a, 0)
    for c in early:
        c.wait()
    lax.fori_loop(0, 8, phase_b, 0)
    for c in late:
        c.wait()
    mem = mem_s[0].astype(F32)
    mem = lax.fori_loop(0, 4, loop_a, mem)
    lax.fori_loop(0, 8, loop_b, mem)
    ob_copy(2).start()
    last = [cp(ob_s.at[pl.ds(24, 8), pl.ds(r, n), :], o_h.at[pl.ds(24, 8), pl.ds(r, n), pl.ds(DM, DM)],
               sem_ob.at[3 + k]) for k, (r, n) in enumerate([(8, 24), (40, 24), (0, 8), (32, 8)])]
    last[0].start()
    last[1].start()
    a = jnp.concatenate([od_s[c, 384:512, :] for c in range(NP)], axis=1).astype(BF)
    put_late(3, _dot(a, jnp.concatenate([wo_rows(j) for j in range(NP)], axis=0)))
    last[2].start()
    last[3].start()
    for c in range(8):
        oa_copy(c).wait()
    for g in range(3):
        ob_copy(g).wait()
    for c in last:
        c.wait()


@jax.jit
def pallas_concat_heads__spectral_gfnet__memory_aug_recurrent_mem_tr__prompt_kernel(
        A_x, A_w_r, A_w_i, B_x, B_mem0, B_Wq, B_Wk, B_Wv, B_Wo, B_seg_len=None):
    dmat, smat, misc = _consts()
    vm, dma = pltpu.VMEM, pltpu.SemaphoreType.DMA
    out = pl.pallas_call(
        _kernel,
        out_shape=jax.ShapeDtypeStruct((N1, N2, 2 * DM), BF),
        in_specs=[pl.BlockSpec(memory_space=pl.ANY)] * 12,
        out_specs=pl.BlockSpec(memory_space=pl.ANY),
        scratch_shapes=[
            vm((12, DM, 8, DH), BF), vm((PB_ROWS, 128), U32), vm((2048 + 32, 128), U32),
            vm((3 * H, DM // 2, DH), U32), vm((H, DM // 2, DH), U32), vm((H * DH, DM), BF),
            vm((BIG_ROWS, 128), F32), vm((NP, NSEG * 8, 2 * DH), F32), vm((128, DM), F32),
            vm((4, NSEG, 8, 128), BF), vm((4, NSEG * 4, 128), U32), vm((NSEG, 24, DM), BF),
            vm(misc.shape, F32),
            vm((N1, N2, DM), BF), vm((2, DM // 2 + 1, S), BF), vm(dmat.shape, U32), vm(smat.shape, U32),
            vm((N1, N2, DM), BF), vm((N1, N2, DM), BF), vm((2, MEM, DM), BF),
            dma((12,)), dma((8,)), dma((5,)), dma((8,)), dma((7,)), dma((4,)),
        ],
        compiler_params=pltpu.CompilerParams(vmem_limit_bytes=120 * 1024 * 1024, disable_bounds_checks=True,
                                             disable_semaphore_checks=True),
    )(A_x.reshape(N1, N2, DM), A_w_r.T, A_w_i.T,
      B_x.reshape(NSEG, SEG, DM), B_mem0.reshape(MEM, DM), B_Wq, B_Wk, B_Wv, B_Wo.reshape(H * DH, DM),
      jnp.asarray(dmat), jnp.asarray(smat), jnp.asarray(misc))
    return out.reshape(1, S, 2 * DM)
```

```python
import numpy as np
import jax
import jax.numpy as jnp
from jax import lax
import jax.experimental.pallas as pl
import jax.experimental.pallas.tpu as pltpu

S, DM, H, DH, MEM, SEG = 2048, 512, 32, 128, 8, 32
NSEG = S // SEG
NP = H // 2
N1, N2 = 32, 64
BF, F32, U32 = jnp.bfloat16, jnp.float32, jnp.uint32
EXP_C = float(DH ** -0.5 * np.log2(np.e))
HI_MASK = 0xFFFF0000

P_OFF = 0
T_OFF = P_OFF + 3 * NP * NSEG * 16
L_OFF = T_OFF + 64 * 8
V_OFF = L_OFF + 4 * 256
VN_OFF = V_OFF + 8192
X_OFF = VN_OFF + 128
BIG_ROWS = X_OFF + 64
TK_OFF = 0
TF_OFF = TK_OFF + 64
F_OFF = TF_OFF + 2 * 512 + 32
U_OFF = F_OFF + 8 * 512
UN_OFF = U_OFF + 8192
PB_ROWS = UN_OFF + 128

STEP_A = (3, 5, 1)
STEP_B = (3, 5, 1)
SCHED_PB = (0, 52, 16, 28, 0, 16, 9, 20, 17, 2)
SCHED_LA = (3, 3, 25, 41, 15, 0)
SCHED_LB = (8, 12, 11, 3, 5, 301, 0)


def _pack_rows(m):
    f = np.ascontiguousarray(m, dtype=np.float32).view(np.uint32)
    r = ((f + 0x7FFF + ((f >> 16) & 1)) >> 16).astype(np.uint32)
    return r[..., 0::2, :] | (r[..., 1::2, :] << 16)


def _consts():
    l = np.arange(128)
    d2 = np.arange(128)[:, None]
    lo = (l % 2) == 0
    a_re = 2 * np.pi * d2 * (2 * l)[None, :] / DM
    a_im = 2 * np.pi * d2 * (2 * ((l - 1) % 128))[None, :] / DM
    m0 = np.where(lo[None, :], np.cos(a_re), -np.sin(a_im))
    m0[:, 1] = (-1.0) ** np.arange(128)
    m2 = np.where(lo[None, :], -np.sin(a_im), np.cos(a_re))
    e = np.arange(64)[:, None]

    def odd_cols(lanes):
        kd = 2 * lanes + 1
        ang = 2 * np.pi * e * kd[None, :] / DM
        sg = np.where(kd % 4 == 1, 1.0, -1.0)[None, :]
        return (np.concatenate([np.cos(ang), -sg * np.sin(ang)], axis=0),
                np.concatenate([-np.sin(ang), -sg * np.cos(ang)], axis=0))

    plus = (l % 4 == 0) | (l % 4 == 3)
    o_re, o_im = odd_cols(l)[0], odd_cols((l - 2) % 128)[1]
    mp = np.where(plus[None, :], o_re, o_im)
    mm = np.where(plus[None, :], o_im, o_re)
    sc = 2.0 / (S * DM)
    m0i = m0.T * sc
    m0i[0] /= 2
    m0i[1] /= 2
    a32 = 2 * np.pi * np.outer(np.arange(N1), np.arange(N1)) / N1
    c32, s32 = np.zeros((128, 128)), np.zeros((128, 128))
    c32[:N1, :N1], s32[:N1, :N1] = np.cos(a32), -np.sin(a32)
    nf = np.concatenate([c32, s32], axis=1)
    dfw = np.concatenate([np.concatenate([m0, m2], axis=1), np.concatenate([mp, mm], axis=1), nf], axis=0)
    dinv = np.concatenate([np.concatenate([m0i, m2.T * sc], axis=1),
                           np.concatenate([mp.T, mm.T], axis=1) * sc, nf], axis=0)
    rho = np.arange(N2)
    th = 2 * np.pi * np.outer(4 * (rho % 16) + rho // 16, rho) / N2
    c, s = np.cos(th), np.sin(th)
    mf = np.concatenate([np.concatenate([c, s], 1), np.concatenate([-s, c], 1)], 0)
    dfw = np.concatenate([dfw, np.concatenate([mf, mf.T], axis=1)], axis=0)
    dinv = np.concatenate([dinv, np.zeros((128, 256))], axis=0)
    dmat = _pack_rows(np.stack([dfw, dinv]))
    th = 2 * np.pi * np.arange(N1).reshape(4, 1, 8) * np.arange(N2).reshape(1, N2, 1) / S
    smat = np.broadcast_to(np.stack([np.cos(th), np.sin(th)], axis=2)[..., None], (4, N2, 2, 8, 128))
    smat = np.ascontiguousarray(smat, dtype=np.float32)
    head = np.concatenate([np.zeros(32), np.ones(32), np.zeros(8), np.ones(8)])
    pos = np.concatenate([np.arange(8), np.arange(16, 40)] * 2 + [np.arange(8, 16)] * 2)
    same = head[:, None] == head[None, :]
    ok = same & ((pos[:, None] < MEM) | (pos[:, None] >= pos[None, :]))
    misc = np.zeros((96 + 2 * N2, 128), np.float32)
    misc[:80, :80] = np.where(ok, 0.0, np.where(same, -1e9 * DH ** 0.5, -np.inf))
    atw = 2 * np.pi * np.outer(np.arange(N2), np.arange(128) % N1) / S
    misc[96:96 + N2], misc[96 + N2:] = np.cos(atw), np.sin(atw)
    return dmat, smat, misc


def _cmul(z, ang):
    re, im = z
    c, s = float(np.cos(ang)), float(np.sin(ang))
    if abs(s) < 1e-12:
        return (re, im) if c > 0 else (-re, -im)
    if abs(c) < 1e-12:
        return (-im, re) if s > 0 else (im, -re)
    if abs(abs(c) - abs(s)) < 1e-12:
        return ((re - im) * c, (re + im) * c) if c * s > 0 else ((re + im) * c, (im - re) * c)
    return re * c - im * s, re * s + im * c


def _fft(x, sign):
    n = len(x)
    if n == 1:
        return x
    if n == 2:
        (ar, ai), (br, bi) = x
        return [(ar + br, ai + bi), (ar - br, ai - bi)]
    ev, z1, z3 = _fft(x[0::2], sign), _fft(x[1::4], sign), _fft(x[3::4], sign)
    out = [None] * n
    q = n // 4
    for k in range(q):
        ar, ai = _cmul(z1[k], sign * 2 * np.pi * k / n)
        br, bi = _cmul(z3[k], sign * 2 * np.pi * 3 * k / n)
        sr, si, dr, di = ar + br, ai + bi, ar - br, ai - bi
        (er, ei), (fr, fi) = ev[k], ev[k + q]
        out[k] = (er + sr, ei + si)
        out[k + 2 * q] = (er - sr, ei - si)
        plus, minus = (fr - di, fi + dr), (fr + di, fi - dr)
        out[k + q], out[k + 3 * q] = (plus, minus) if sign > 0 else (minus, plus)
    return out


def _dot(a, b):
    return jnp.dot(a, b, preferred_element_type=F32)


def _bf(words):
    return pltpu.bitcast(words, BF)


def _f32(words):
    return pltpu.bitcast(words, F32)


def _u32(x):
    return pltpu.bitcast(x, U32)


def _rows8(off):
    return pl.ds(pl.multiple_of(off, 8), 8)


def _kernel(ax_h, wr_h, wi_h, bx_h, mem_h, wq_h, wk_h, wv_h, wo_h, dmat_h, smat_h, misc_h,
            o_h,
            wraw, pb, wtmp, w_s, wo_s, woraw, big, od_s, acc_s, x0raw, x0_s, xr_s, misc_s,
            ax_s, fraw, dmat_s, smat_s, oa_s, ob_s, mem_s,
            sem_w, sem_c, sem_m, sem_oa, sem_ob, sem_f):
    w_h = (wk_h, wq_h, wv_h)
    cp = pltpu.make_async_copy

    def w_copy(m, g):
        return cp(w_h[m].at[:, pl.ds(pl.multiple_of(8 * g, 8), 8), :], wraw.at[4 * m + g], sem_w.at[4 * m + g])

    def w_wait(t):
        cp(wraw.at[t], wraw.at[t], sem_w.at[t]).wait()

    def chunk_copies(i):
        rows = pl.ds(pl.multiple_of(i * 512, 512), 512)
        cols = pl.ds(pl.multiple_of(i * 256, 256), 256)
        return [cp(wo_h.at[rows], woraw.at[rows], sem_c.at[i]),
                cp(ax_h.at[:, _rows8(i * 8), :], ax_s.at[:, _rows8(i * 8), :], sem_c.at[i]),
                cp(wr_h.at[:, cols], fraw.at[0, :, cols], sem_c.at[i]),
                cp(wi_h.at[:, cols], fraw.at[1, :, cols], sem_c.at[i])]

    def first_copies(kt):
        d = pl.ds(pl.multiple_of(kt * 128, 128), 128)
        return [cp(bx_h.at[:, pl.ds(0, 8), d], x0raw.at[kt], sem_f.at[kt]),
                cp(wk_h.at[d, pl.ds(0, 8), :], wraw.at[0, d], sem_f.at[kt])]

    early = [cp(dmat_h, dmat_s, sem_m.at[0]), cp(misc_h, misc_s, sem_m.at[1]), cp(mem_h, mem_s.at[0], sem_m.at[2])]
    late = [cp(bx_h.at[:, pl.ds(8, 24), :], xr_s, sem_m.at[3]), cp(smat_h, smat_s, sem_m.at[4])]

    def ob_copy(g):
        return cp(ob_s.at[_rows8(g * 8)], o_h.at[_rows8(g * 8), :, pl.ds(DM, DM)], sem_ob.at[g])

    def oa_copy(c):
        return cp(oa_s.at[:, _rows8(c * 8), :], o_h.at[:, _rows8(c * 8), pl.ds(0, DM)], sem_oa.at[c])

    lane = lax.broadcasted_iota(jnp.int32, (1, 128), 1)
    lane_lo = (lane & 1) == 0
    lane_plus = ((lane + 1) & 2) == 0
    lane_half = lane < 64
    rt = float(np.sqrt(0.5))

    order = [8 * a + b for b in range(8) for a in range(4)]

    def filt_prep(i, h, a):
        col = pl.ds(pl.multiple_of((2 * i + h) * 128, 128), 128)
        t = _u32(fraw[a, 0:256, col]).T
        for q in range(16):
            pb[_rows8(F_OFF + (a * 4 + q % 4) * 512 + ((2 * i + h) * 4 + q // 4) * 8), :] = t[q * 8:(q + 1) * 8]

    def ax_blocks(c):
        v = jnp.concatenate([ax_s[s1, _rows8(c * 8), :].astype(F32) for s1 in order], axis=0)
        return [v[:, i * 128:(i + 1) * 128] for i in range(4)]

    def t_rows(ka, b, part):
        return pl.ds(T_OFF + ((ka * 8 + b) * 2 + part) * 8, 8)

    def tf_rows(c, blk, ka, b, part):
        return _rows8(TF_OFF + (c % 2) * 32 + blk * 512 + ((ka * 8 + b) * 2 + part) * 8)

    def twiddles(c):
        return misc_s[_rows8(96 + c * 8), :], misc_s[_rows8(96 + N2 + c * 8), :]

    def fwd_even(c):
        x0, x1, x2, x3 = ax_blocks(c)
        p, q = x0 + x2, x1 + x3
        t0 = _dot((p + q).astype(BF), _bf(dmat_s[0, 0:64, 0:128]))
        t2 = _dot((p - q).astype(BF), _bf(dmat_s[0, 0:64, 128:256]))
        re = jnp.where(lane_lo, t0, t2)
        im = jnp.where(lane == 0, 0.0, pltpu.roll(jnp.where(lane_lo, t2, t0), 127, 1))
        n = jnp.zeros((8, 128), F32)
        for pos, s1 in enumerate(order):
            v = t0[pos * 8:(pos + 1) * 8]
            n = jnp.where(lane == s1, v if s1 == 1 else pltpu.roll(v, (s1 - 1) % 128, 1), n)
        return re, im, n

    def fwd_odd(c):
        x0, x1, x2, x3 = ax_blocks(c)
        a, b = x0 - x2, x1 - x3
        r = pltpu.roll(jnp.where(lane_half, b, (a - b) * rt), 64, 1)
        p, q = jnp.where(lane_half, a, r), jnp.where(lane_half, r, (a + b) * rt)
        tp = _dot((p + q).astype(BF), _bf(dmat_s[0, 64:128, 0:128]))
        tm = _dot((p - q).astype(BF), _bf(dmat_s[0, 64:128, 128:256]))
        return jnp.where(lane_plus, tp, tm), pltpu.roll(jnp.where(lane_plus, tm, tp), 126, 1)

    def fwd_pass1(c, blk, re, im):
        for b in range(8):
            z = _fft([(re[(b * 4 + a) * 8:(b * 4 + a + 1) * 8], im[(b * 4 + a) * 8:(b * 4 + a + 1) * 8])
                      for a in range(4)], -1)
            for ka in range(4):
                zr, zi = _cmul(z[ka], -2 * np.pi * b * ka / N1)
                pb[tf_rows(c, blk, ka, b, 0), :] = _u32(zr)
                pb[tf_rows(c, blk, ka, b, 1), :] = _u32(zi)

    def fwd_pass2(c, blk, ka):
        z = _fft([(_f32(pb[tf_rows(c, blk, ka, b, 0), :]), _f32(pb[tf_rows(c, blk, ka, b, 1), :]))
                  for b in range(8)], -1)
        for kb in range(8):
            k1 = ka + 4 * kb
            for part in range(2):
                row = U_OFF + (k1 // 8) * 2048 + (blk * 2 + part) * 512 + (k1 % 8) * 8
                pb[_rows8(row + c * 64), :] = _u32(z[kb][part])

    def fwd_nyq(c, n):
        u = _dot(n.astype(BF), _bf(dmat_s[0, 128:192, :]))
        ur, ui = u[:, 0:128], u[:, 128:256]
        ct, st = twiddles(c)
        return ur * ct + ui * st, ui * ct - ur * st

    def put_nyq(c, u):
        pb[_rows8(UN_OFF + c * 8), :] = _u32(u[0])
        pb[_rows8(UN_OFF + 64 + c * 8), :] = _u32(u[1])

    def cfilter(z, wr, wi):
        zr, zi = z[0:64], z[64:128]
        return jnp.concatenate([zr * wr - zi * wi, zr * wi + zi * wr], axis=0).astype(BF)

    def tm_rows(kc, r, part):
        return pl.ds(TF_OFF + ((kc * 8 + r) * 2 + part) * 8, 8)

    def tm_get(kc, r):
        return _f32(pb[tm_rows(kc, r, 0), :]), _f32(pb[tm_rows(kc, r, 1), :])

    def tm_put(kc, r, z):
        pb[tm_rows(kc, r, 0), :] = _u32(z[0])
        pb[tm_rows(kc, r, 1), :] = _u32(z[1])

    def mid_1(g, blk, r):
        view = pb.at[pl.ds(pl.multiple_of(U_OFF + g * 2048, 32), 2048 + 8)]
        x = []
        for c in range(8):
            re, im = [_f32(view[pl.ds((blk * 2 + part) * 512 + c * 64 + r, 8, stride=8), :]) for part in range(2)]
            if 8 * c + r:
                ct, st = smat_s[g, 8 * c + r, 0], smat_s[g, 8 * c + r, 1]
                re, im = re * ct + im * st, im * ct - re * st
            x.append((re, im))
        z = _fft(x, -1)
        for kc in range(8):
            tm_put(kc, r, _cmul(z[kc], -2 * np.pi * r * kc / N2))

    def mid_2(g, blk, kc):
        z = _fft([tm_get(kc, r) for r in range(8)], -1)
        y = []
        for kr in range(8):
            w = [pb[pl.ds(pl.multiple_of(g * 512, 32) + (F_OFF + a * 2048 + (kc + 8 * kr) * 8), 8), :]
                 for a in range(2)]
            wr, wi = [_f32(v & jnp.uint32(HI_MASK)) if blk else _f32(v << 16) for v in w]
            zr, zi = z[kr]
            y.append((zr * wr - zi * wi, zr * wi + zi * wr))
        v = _fft(y, 1)
        for r in range(8):
            tm_put(kc, r, _cmul(v[r], 2 * np.pi * r * kc / N2))

    def mid_3(g, blk, r):
        z = _fft([tm_get(kc, r) for kc in range(8)], 1)
        for c in range(8):
            re, im = z[c]
            if 8 * c + r:
                ct, st = smat_s[g, 8 * c + r, 0], smat_s[g, 8 * c + r, 1]
                re, im = re * ct - im * st, im * ct + re * st
            for part, v in enumerate((re, im)):
                row = V_OFF + c * 1024 + (blk * 2 + part) * 256 + r * 8
                big[pl.ds(pl.multiple_of(g * 64, 32) + row, 8), :] = v

    def nyq_a():
        z = _dot(_bf(dmat_s[0, 192:256, 0:128]), _f32(pb[pl.ds(UN_OFF, 128), :]).astype(BF))
        w = []
        for a in range(2):
            g = jnp.concatenate([fraw[a, 256:257, t * 128:(t + 1) * 128].astype(F32) for t in range(16)], axis=0)
            w.append(jnp.concatenate([g] + [pltpu.roll(g, 128 - 32 * q, 1) for q in range(1, 4)], axis=0))
        return cfilter(z, *w)

    def nyq_b(y):
        big[pl.ds(VN_OFF, 128), :] = _dot(_bf(dmat_s[0, 192:256, 128:256]), y)

    def inv_pass1(c, blk, ka):
        view = big.at[pl.ds(pl.multiple_of(V_OFF + c * 1024, 32), 1024 + 8)]
        z = _fft([tuple(view[pl.ds((blk * 2 + part) * 256 + (k1 // 8) * 64 + k1 % 8, 8, stride=8), :]
                        for part in range(2)) for k1 in range(ka, N1, 4)], 1)
        for b in range(8):
            zr, zi = _cmul(z[b], 2 * np.pi * b * ka / N1)
            big[t_rows(ka, b, 0), :] = zr
            big[t_rows(ka, b, 1), :] = zi

    def inv_nyq(c):
        vr, vi = big[_rows8(VN_OFF + c * 8), :], big[_rows8(VN_OFF + 64 + c * 8), :]
        ct, st = twiddles(c)
        m = _bf(dmat_s[1, 128:192, :])
        return (_dot((vr * ct - vi * st).astype(BF), m[:, 0:128])
                + _dot((vi * ct + vr * st).astype(BF), m[:, 128:256]))

    def inv_pass2(blk, b, n):
        z = _fft([(big[t_rows(ka, b, 0), :], big[t_rows(ka, b, 1), :]) for ka in range(4)], 1)
        for a in range(4):
            re, im = z[a]
            s1 = 8 * a + b
            if blk == 0:
                im = pltpu.roll(im, 1, 1)
                nv = n if s1 == 1 else pltpu.roll(n, (1 - s1) % 128, 1)
                re, im = jnp.where(lane == 1, nv, jnp.where(lane_lo, re, im)), jnp.where(lane_lo, im, re)
            else:
                im = pltpu.roll(im, 2, 1)
                re, im = jnp.where(lane_plus, re, im), jnp.where(lane_plus, im, re)
            big[pl.ds(L_OFF + (2 * blk) * 256 + s1 * 8, 8), :] = re
            big[pl.ds(L_OFF + (2 * blk + 1) * 256 + s1 * 8, 8), :] = im

    def inv_out(c):
        lhs = [big[pl.ds(L_OFF + i * 256, 256), :] for i in range(4)]
        c0 = _dot(lhs[0].astype(BF), _bf(dmat_s[1, 0:64, 0:128]))
        c2 = _dot(lhs[1].astype(BF), _bf(dmat_s[1, 0:64, 128:256]))
        lp = _dot(lhs[2].astype(BF), _bf(dmat_s[1, 64:128, 0:128]))
        lm = _dot(lhs[3].astype(BF), _bf(dmat_s[1, 64:128, 128:256]))
        pp, qq = lp + lm, lp - lm
        r = pltpu.roll(jnp.where(lane_half, qq, pp), 64, 1)
        p, q = jnp.where(lane_half, pp, (r + qq) * rt), jnp.where(lane_half, r, (qq - r) * rt)
        e, f = c0 + c2, c0 - c2
        y = jnp.concatenate([e + p, f + q, e - p, f - q], axis=1)
        oa_s[:, _rows8(c * 8), :] = y.reshape(N1, 8, DM).astype(BF)

    def head_words(hh, n):
        a = wtmp[pl.ds(hh // 2, n, stride=8), :]
        b = wtmp[pl.ds(4 + hh // 2, n, stride=8), :]
        return (a >> 16) | (b & jnp.uint32(HI_MASK)) if hh % 2 else (a & 0xFFFF) | (b << 16)

    def head_weights(t, hh):
        w = head_words(hh, 256)
        w_s[t * 8 + hh] = w
        return w

    def stage_chunk(t):
        for dc in range(8):
            wtmp[dc * 256:(dc + 1) * 256, :] = _u32(wraw[t, dc * 64:(dc + 1) * 64].reshape(512, 128))
        head_weights(t, 0)

    def early_proj(t, hooks):
        for jj in range(4):
            res = []
            for hh in (2 * jj, 2 * jj + 1):
                w = w_s[t * 8] if hh == 0 else head_weights(t, hh)
                r = _dot(_bf(jnp.concatenate([x0_s[k] for k in range(4)], axis=1)), _bf(w))
                res.append(r.reshape(NSEG, 8, 128))
                for tm, f, pinned in hooks:
                    if tm // 8 == hh:
                        if pinned:
                            pb[_rows8(TK_OFF + (t % 2) * 32), :] = _u32(r[(tm % 8) * 64:(tm % 8) * 64 + 8])
                        f()
            big[pl.ds(pl.multiple_of(P_OFF + (t * 4 + jj) * 1024, 1024), 1024), :] = (
                jnp.concatenate(res, axis=1).reshape(1024, 128))

    def phase_0(kt, carry):
        for c in first_copies(kt):
            c.wait()
        for dc in range(2):
            v = wraw[0, pl.ds(pl.multiple_of(kt * 128 + dc * 64, 64), 64)]
            wtmp[dc * 256:(dc + 1) * 256, :] = _u32(v.reshape(512, 128))
        xk = _u32(x0raw[kt].reshape(NSEG * 8, 128))
        x0_s[kt] = xk
        for jj in range(4):
            res = []
            for hh in (2 * jj, 2 * jj + 1):
                w = head_words(hh, 64)
                w_s[hh, pl.ds(pl.multiple_of(kt * 64, 64), 64), :] = w
                res.append(_dot(_bf(xk), _bf(w)).reshape(NSEG, 8, 128))
            rows = pl.ds(P_OFF + jj * 1024, 1024)
            big[rows, :] = jnp.where(kt > 0, big[rows, :], 0.0) + jnp.concatenate(res, axis=1).reshape(1024, 128)
        return carry

    def phase_a(t, carry):
        w_copy(1, t).start()
        for c in chunk_copies(t):
            c.start()

        @pl.when(t <= 2)
        def _():
            w_wait(t)
            stage_chunk(t)

        @pl.when(t >= 2)
        def _():
            w_wait(t + 1)

        early_proj(t, [])
        stage_chunk(jnp.where(t >= 2, t + 1, t))
        return carry

    def phase_b(i, carry):
        t = i + 3

        @pl.when(i < 4)
        def _():
            w_copy(2, i).start()
            for c in chunk_copies(i + 4):
                c.start()

        @pl.when(i == 4)
        def _():
            for c in late:
                c.start()

        w_wait(t + 1)
        for c in chunk_copies(i):
            c.wait()

        def wo_retile(n):
            wo_s[n * 8 + i] = _u32(woraw[pl.ds(pl.multiple_of(i * 512, 512), 512), n * 128:(n + 1) * 128])

        box = {}
        t_om, t_f, t_o1, t_o2, t_em, t_e1, t_n, t_e2, t_pn, dt = SCHED_PB
        hooks = [(t_f + dt * k, lambda k=k: filt_prep(i, k // 2, k % 2), False) for k in range(4)]
        hooks += [(t_om, lambda: box.update(o=fwd_odd(i)), False),
                  (t_o1, lambda: fwd_pass1(i, 1, *box["o"]), False),
                  (t_em, lambda: box.update(e=fwd_even(i)), False),
                  (t_e1, lambda: fwd_pass1(i, 0, *box["e"][:2]), False),
                  (t_n, lambda: box.update(n=fwd_nyq(i, box["e"][2])), False),
                  (t_pn, lambda: put_nyq(i, box["n"]), False)]
        hooks += [(t_o2 + dt * ka, lambda ka=ka: fwd_pass2(i, 1, ka), True) for ka in range(4)]
        hooks += [(t_e2 + dt * ka, lambda ka=ka: fwd_pass2(i, 0, ka), True) for ka in range(4)]
        hooks += [(0, lambda n=n: wo_retile(n), False) for n in range(4)]
        early_proj(t, sorted(hooks, key=lambda h: h[0]))
        stage_chunk(jnp.minimum(t + 1, 11))
        return carry

    def x0_rows(r0, n):
        return _bf(jnp.concatenate([x0_s[k, r0 // 2:(r0 + n) // 2, :] for k in range(4)], axis=1))

    def phase_c():
        for jj in range(4):
            res = []
            for hh in (2 * jj, 2 * jj + 1):
                w = w_s[88] if hh == 0 else head_weights(11, hh)
                res.append(_dot(x0_rows(0, 128), _bf(w)).reshape(16, 8, 128))
            big[pl.ds(P_OFF + (44 + jj) * 1024, 256), :] = jnp.concatenate(res, axis=1).reshape(256, 128)

    def early_rest(i, u):
        r = _dot(x0_rows(128 + 192 * (u % 2), 192), _bf(w_s[88 + 2 * i + u // 2]))
        for q in range(24):
            row = P_OFF + 44 * 1024 + (16 + 24 * (u % 2) + q) * 16 + (u // 2) * 8
            big[pl.ds(pl.multiple_of(i * 1024, 32) + row, 8), :] = r[q * 8:(q + 1) * 8]

    def wo_rows(j):
        r = pl.ds(pl.multiple_of((j % 2) * 128, 128), 128)
        return _bf(jnp.concatenate([wo_s[n * 8 + j // 2, r, :] for n in range(4)], axis=1))

    def put_late(g, res):
        for i in range(16):
            ob_s[g * 8 + i // 2, (i % 2) * 32:(i % 2) * 32 + 8, :] = res[i * 8:(i + 1) * 8].astype(BF)

    def late_proj(idx):
        g, c = idx // 16, idx % 16
        a = od_s[c, pl.ds(pl.multiple_of(g * 128, 128), 128), :].astype(BF)
        res = jnp.where(c > 0, acc_s[...], 0.0) + _dot(a, wo_rows(c))
        acc_s[...] = res
        put_late(g, res)

    def step(s0, u0, mem, hooks, lags):
        s = s0 + u0
        qk_lag, pv_lag, skew = lags
        lhs = jnp.concatenate([mem, xr_s[s].astype(F32)], axis=0).astype(BF)
        st = {}

        def proj(mi, j):
            y1 = _dot(lhs, _bf(w_s[mi * H + 2 * j]))
            y2 = _dot(lhs, _bf(w_s[mi * H + 2 * j + 1]))
            pre = big[pl.ds(pl.multiple_of(s0 * 16, 32) + (P_OFF + (mi * NP + j) * 1024 + u0 * 16), 16), :]
            st[mi, j] = jnp.concatenate([y1, y2, pre], axis=0).astype(BF)
            st["last"] = y1[0:8]

        def pin():
            big[pl.ds(pl.multiple_of((s0 % 4) * 16, 32) + X_OFF, 8), :] = st["last"]

        def pin_pb():
            pb[pl.ds(pl.multiple_of((s0 % 8) * 8, 32) + TK_OFF, 8), :] = _u32(st["last"])

        def qk(j):
            sc = lax.dot_general(st.pop((1, j)), st.pop((0, j)), (((1,), (1,)), ((), ())),
                                 preferred_element_type=F32)
            fill = misc_s[0:80, 0:80]
            sc = jnp.where(fill == 0.0, sc, fill)
            p = jnp.exp2((sc - jnp.max(sc, axis=1, keepdims=True)) * EXP_C)
            st["p", j] = (p.astype(BF), pl.reciprocal(jnp.sum(p, axis=1, keepdims=True), approx=True))

        def pv(j):
            p, rl = st.pop(("p", j))
            o = _dot(p, st.pop((2, j))) * rl
            st["o", j] = jnp.concatenate([o[0:32], o[32:64]], axis=1).astype(BF)
            od_s[j, pl.ds(pl.multiple_of(s0 * 8, 16) + u0 * 8, 8), :] = jnp.concatenate([o[64:72], o[72:80]], axis=1)

        def op(j):
            r = _dot(st.pop(("o", j)), wo_rows(j))
            st["acc"] = r if "acc" not in st else st["acc"] + r

        units = []
        for j in range(-skew, NP):
            units += [(mi, j + skew) for mi in (0, 1) if j + skew < NP] + ([(2, j)] if j >= 0 else [])
        events = [(t, lambda mi=mi, j=j: proj(mi, j)) for t, (mi, j) in enumerate(units)]
        events += [(3 * NP + j, lambda j=j: op(j)) for j in range(NP)]
        for j in range(NP):
            tqk = units.index((1, j)) + 1 + qk_lag
            events.append((tqk - 0.5, lambda j=j: qk(j)))
            events.append((max(tqk + pv_lag, units.index((2, j)) + 1 + qk_lag) - 0.4, lambda j=j: pv(j)))
        for t, fs in hooks.items():
            events += [(t - 0.3, {None: pin, "pb": pin_pb}.get(f, f)) for f in fs]
        for _, f in sorted(events, key=lambda ev: ev[0]):
            f()
        out = st["acc"]
        ob_s[s0 // 2 + u0 // 2, (u0 % 2) * 32 + 8:(u0 % 2) * 32 + 32, :] = out[8:32].astype(BF)
        return out[0:8].astype(BF).astype(F32)

    def loop_a(i, mem):
        box = {}
        jobs = [{} for _ in range(4)]
        t_0, dt, t_n0, t_n1, nps, t_x = SCHED_LA

        def add(t, fs):
            u = min(t // 64, 3)
            jobs[u].setdefault(t - 64 * u, []).extend(fs)

        pieces = [(f, blk, k) for blk in range(2) for f in (mid_1, mid_2, mid_3) for k in range(8)]
        for n, (f, blk, k) in enumerate(pieces):
            add(64 * (n // nps) + t_0 + dt * (n % nps), ["pb", lambda f=f, blk=blk, k=k: f(i, blk, k)])
        add(192 + t_n0, [lambda: box.update(n=nyq_a())])
        add(192 + t_n1, [lambda: nyq_b(box["n"])])
        for u, t in enumerate(sorted([64, 128, 192, t_x])):
            add(t, [lambda u=u: early_rest(i, u)])
        for u in range(4):
            mem = step(4 * i, u, mem, jobs[u], STEP_A)
        return mem

    def loop_b(i, mem):
        box = {}
        jobs = [{} for _ in range(6)]
        t1, d1, t2, d2, t_n, t_o, t_x = SCHED_LB

        def add(t, fs):
            u = min(t // 64, 5)
            jobs[u].setdefault(t - 64 * u, []).extend(fs)

        for blk in range(2):
            for ka in range(4):
                add(128 * blk + t1 + d1 * ka, [None, lambda blk=blk, ka=ka: inv_pass1(i, blk, ka)])
            for b in range(8):
                add(128 * blk + 64 + t2 + d2 * b, [None, lambda blk=blk, b=b: inv_pass2(blk, b, box["n"])])
        add(t_n, [lambda: box.update(n=inv_nyq(i))])
        add(t_o, [lambda: inv_out(i)])
        for u, t in enumerate(sorted([64 * u for u in range(1, 6)] + [t_x])):
            add(t, [lambda u=u: late_proj(6 * i + u)])
        for u in range(6):
            mem = step(6 * i, 16 + u, mem, jobs[u], STEP_B)
        oa_copy(i).start()

        @pl.when((i == 2) | (i == 5))
        def _():
            ob_copy(i // 3).start()

        return mem

    for kt in range(4):
        for c in first_copies(kt):
            c.start()
    for g in range(1, 4):
        w_copy(0, g).start()
    lax.fori_loop(0, 4, phase_0, 0)
    w_copy(1, 0).start()
    for c in early + chunk_copies(0):
        c.start()
    lax.fori_loop(1, 3, phase_a, 0)
    w_copy(1, 3).start()
    for c in chunk_copies(3):
        c.start()
    for c in early:
        c.wait()
    lax.fori_loop(0, 8, phase_b, 0)
    phase_c()
    for c in late:
        c.wait()
    mem = mem_s[0].astype(F32)
    mem = lax.fori_loop(0, 4, loop_a, mem)
    lax.fori_loop(0, 8, loop_b, mem)
    ob_copy(2).start()
    last = [cp(ob_s.at[pl.ds(24, 8), pl.ds(r, n), :], o_h.at[pl.ds(24, 8), pl.ds(r, n), pl.ds(DM, DM)],
               sem_ob.at[3 + k]) for k, (r, n) in enumerate([(8, 24), (40, 24), (0, 8), (32, 8)])]
    last[0].start()
    last[1].start()
    a = jnp.concatenate([od_s[c, 384:512, :] for c in range(NP)], axis=1).astype(BF)
    put_late(3, _dot(a, jnp.concatenate([wo_rows(j) for j in range(NP)], axis=0)))
    last[2].start()
    last[3].start()
    for c in range(8):
        oa_copy(c).wait()
    for g in range(3):
        ob_copy(g).wait()
    for c in last:
        c.wait()


@jax.jit
def pallas_concat_heads__spectral_gfnet__memory_aug_recurrent_mem_tr__prompt_kernel(
        A_x, A_w_r, A_w_i, B_x, B_mem0, B_Wq, B_Wk, B_Wv, B_Wo, B_seg_len=None):
    dmat, smat, misc = _consts()
    vm, dma = pltpu.VMEM, pltpu.SemaphoreType.DMA
    out = pl.pallas_call(
        _kernel,
        out_shape=jax.ShapeDtypeStruct((N1, N2, 2 * DM), BF),
        in_specs=[pl.BlockSpec(memory_space=pl.ANY)] * 12,
        out_specs=pl.BlockSpec(memory_space=pl.ANY),
        scratch_shapes=[
            vm((12, DM, 8, DH), BF), vm((PB_ROWS, 128), U32), vm((2048 + 32, 128), U32),
            vm((3 * H, DM // 2, DH), U32), vm((H, DM // 2, DH), U32), vm((H * DH, DM), BF),
            vm((BIG_ROWS, 128), F32), vm((NP, NSEG * 8, 2 * DH), F32), vm((128, DM), F32),
            vm((4, NSEG, 8, 128), BF), vm((4, NSEG * 4, 128), U32), vm((NSEG, 24, DM), BF),
            vm(misc.shape, F32),
            vm((N1, N2, DM), BF), vm((2, DM // 2 + 1, S), BF), vm(dmat.shape, U32), vm(smat.shape, F32),
            vm((N1, N2, DM), BF), vm((N1, N2, DM), BF), vm((2, MEM, DM), BF),
            dma((12,)), dma((8,)), dma((5,)), dma((8,)), dma((7,)), dma((4,)),
        ],
        compiler_params=pltpu.CompilerParams(vmem_limit_bytes=120 * 1024 * 1024, disable_bounds_checks=True,
                                             disable_semaphore_checks=True),
    )(A_x.reshape(N1, N2, DM), A_w_r.T, A_w_i.T,
      B_x.reshape(NSEG, SEG, DM), B_mem0.reshape(MEM, DM), B_Wq, B_Wk, B_Wv, B_Wo.reshape(H * DH, DM),
      jnp.asarray(dmat), jnp.asarray(smat), jnp.asarray(misc))
    return out.reshape(1, S, 2 * DM)
```

```python
import numpy as np
import jax
import jax.numpy as jnp
from jax import lax
import jax.experimental.pallas as pl
import jax.experimental.pallas.tpu as pltpu

S, DM, H, DH, MEM, SEG = 2048, 512, 32, 128, 8, 32
NSEG = S // SEG
NP = H // 2
N1, N2 = 32, 64
BF, F32, U32 = jnp.bfloat16, jnp.float32, jnp.uint32
EXP_C = float(DH ** -0.5 * np.log2(np.e))
HI_MASK = 0xFFFF0000

P_OFF = 0
T_OFF = P_OFF + 3 * NP * NSEG * 16
L_OFF = T_OFF + 64 * 8
V_OFF = L_OFF + 4 * 256
VN_OFF = V_OFF + 8192
X_OFF = VN_OFF + 128
BIG_ROWS = X_OFF + 64
TK_OFF = 0
TF_OFF = TK_OFF + 64
F_OFF = TF_OFF + 2 * 512 + 32
U_OFF = F_OFF + 8 * 512
UN_OFF = U_OFF + 8192
PB_ROWS = UN_OFF + 128

STEP_A = (361, 361, 361, 361)
STEP_B = (361, 361, 361, 361, 361, 361)
SCHED_PB = (0, 52, 16, 28, 0, 16, 9, 20, 17, 2)
SCHED_LA = (9, 3, 31, 46, 14, 0)
SCHED_LB = (3, 7, 10, 4, 22, 285, 0)


def _pack_rows(m):
    f = np.ascontiguousarray(m, dtype=np.float32).view(np.uint32)
    r = ((f + 0x7FFF + ((f >> 16) & 1)) >> 16).astype(np.uint32)
    return r[..., 0::2, :] | (r[..., 1::2, :] << 16)


def _consts():
    l = np.arange(128)
    d2 = np.arange(128)[:, None]
    lo = (l % 2) == 0
    a_re = 2 * np.pi * d2 * (2 * l)[None, :] / DM
    a_im = 2 * np.pi * d2 * (2 * ((l - 1) % 128))[None, :] / DM
    m0 = np.where(lo[None, :], np.cos(a_re), -np.sin(a_im))
    m0[:, 1] = (-1.0) ** np.arange(128)
    m2 = np.where(lo[None, :], -np.sin(a_im), np.cos(a_re))
    e = np.arange(64)[:, None]

    def odd_cols(lanes):
        kd = 2 * lanes + 1
        ang = 2 * np.pi * e * kd[None, :] / DM
        sg = np.where(kd % 4 == 1, 1.0, -1.0)[None, :]
        return (np.concatenate([np.cos(ang), -sg * np.sin(ang)], axis=0),
                np.concatenate([-np.sin(ang), -sg * np.cos(ang)], axis=0))

    plus = (l % 4 == 0) | (l % 4 == 3)
    o_re, o_im = odd_cols(l)[0], odd_cols((l - 2) % 128)[1]
    mp = np.where(plus[None, :], o_re, o_im)
    mm = np.where(plus[None, :], o_im, o_re)
    sc = 2.0 / (S * DM)
    m0i = m0.T * sc
    m0i[0] /= 2
    m0i[1] /= 2
    a32 = 2 * np.pi * np.outer(np.arange(N1), np.arange(N1)) / N1
    c32, s32 = np.zeros((128, 128)), np.zeros((128, 128))
    c32[:N1, :N1], s32[:N1, :N1] = np.cos(a32), -np.sin(a32)
    nf = np.concatenate([c32, s32], axis=1)
    dfw = np.concatenate([np.concatenate([m0, m2], axis=1), np.concatenate([mp, mm], axis=1), nf], axis=0)
    dinv = np.concatenate([np.concatenate([m0i, m2.T * sc], axis=1),
                           np.concatenate([mp.T, mm.T], axis=1) * sc, nf], axis=0)
    rho = np.arange(N2)
    th = 2 * np.pi * np.outer(4 * (rho % 16) + rho // 16, rho) / N2
    c, s = np.cos(th), np.sin(th)
    mf = np.concatenate([np.concatenate([c, s], 1), np.concatenate([-s, c], 1)], 0)
    dfw = np.concatenate([dfw, np.concatenate([mf, mf.T], axis=1)], axis=0)
    dinv = np.concatenate([dinv, np.zeros((128, 256))], axis=0)
    dmat = _pack_rows(np.stack([dfw, dinv]))
    th = 2 * np.pi * np.arange(N1).reshape(4, 1, 8) * np.arange(N2).reshape(1, N2, 1) / S
    smat = np.broadcast_to(np.stack([np.cos(th), np.sin(th)], axis=2)[..., None], (4, N2, 2, 8, 128))
    smat = np.ascontiguousarray(smat, dtype=np.float32)
    head = np.concatenate([np.zeros(32), np.ones(32), np.zeros(8), np.ones(8)])
    pos = np.concatenate([np.arange(8), np.arange(16, 40)] * 2 + [np.arange(8, 16)] * 2)
    same = head[:, None] == head[None, :]
    ok = same & ((pos[:, None] < MEM) | (pos[:, None] >= pos[None, :]))
    misc = np.zeros((96 + 2 * N2, 128), np.float32)
    misc[:80, :80] = np.where(ok, 0.0, np.where(same, -1e9 * DH ** 0.5, -np.inf))
    atw = 2 * np.pi * np.outer(np.arange(N2), np.arange(128) % N1) / S
    misc[96:96 + N2], misc[96 + N2:] = np.cos(atw), np.sin(atw)
    return dmat, smat, misc


def _cmul(z, ang):
    re, im = z
    c, s = float(np.cos(ang)), float(np.sin(ang))
    if abs(s) < 1e-12:
        return (re, im) if c > 0 else (-re, -im)
    if abs(c) < 1e-12:
        return (-im, re) if s > 0 else (im, -re)
    if abs(abs(c) - abs(s)) < 1e-12:
        return ((re - im) * c, (re + im) * c) if c * s > 0 else ((re + im) * c, (im - re) * c)
    return re * c - im * s, re * s + im * c


def _fft(x, sign):
    n = len(x)
    if n == 1:
        return x
    if n == 2:
        (ar, ai), (br, bi) = x
        return [(ar + br, ai + bi), (ar - br, ai - bi)]
    ev, z1, z3 = _fft(x[0::2], sign), _fft(x[1::4], sign), _fft(x[3::4], sign)
    out = [None] * n
    q = n // 4
    for k in range(q):
        ar, ai = _cmul(z1[k], sign * 2 * np.pi * k / n)
        br, bi = _cmul(z3[k], sign * 2 * np.pi * 3 * k / n)
        sr, si, dr, di = ar + br, ai + bi, ar - br, ai - bi
        (er, ei), (fr, fi) = ev[k], ev[k + q]
        out[k] = (er + sr, ei + si)
        out[k + 2 * q] = (er - sr, ei - si)
        plus, minus = (fr - di, fi + dr), (fr + di, fi - dr)
        out[k + q], out[k + 3 * q] = (plus, minus) if sign > 0 else (minus, plus)
    return out


def _dot(a, b):
    return jnp.dot(a, b, preferred_element_type=F32)


def _bf(words):
    return pltpu.bitcast(words, BF)


def _f32(words):
    return pltpu.bitcast(words, F32)


def _u32(x):
    return pltpu.bitcast(x, U32)


def _rows8(off):
    return pl.ds(pl.multiple_of(off, 8), 8)


def _kernel(ax_h, wr_h, wi_h, bx_h, mem_h, wq_h, wk_h, wv_h, wo_h, dmat_h, smat_h, misc_h,
            o_h,
            wraw, pb, wtmp, w_s, wo_s, woraw, big, od_s, acc_s, x0raw, x0_s, xr_s, misc_s,
            ax_s, fraw, dmat_s, smat_s, oa_s, ob_s, mem_s,
            sem_w, sem_c, sem_m, sem_oa, sem_ob, sem_f):
    w_h = (wk_h, wq_h, wv_h)
    cp = pltpu.make_async_copy

    def w_copy(m, g):
        return cp(w_h[m].at[:, pl.ds(pl.multiple_of(8 * g, 8), 8), :], wraw.at[4 * m + g], sem_w.at[4 * m + g])

    def w_wait(t):
        cp(wraw.at[t], wraw.at[t], sem_w.at[t]).wait()

    def chunk_copies(i):
        rows = pl.ds(pl.multiple_of(i * 512, 512), 512)
        cols = pl.ds(pl.multiple_of(i * 256, 256), 256)
        return [cp(wo_h.at[rows], woraw.at[rows], sem_c.at[i]),
                cp(ax_h.at[:, _rows8(i * 8), :], ax_s.at[:, _rows8(i * 8), :], sem_c.at[i]),
                cp(wr_h.at[:, cols], fraw.at[0, :, cols], sem_c.at[i]),
                cp(wi_h.at[:, cols], fraw.at[1, :, cols], sem_c.at[i])]

    def first_copies(kt):
        d = pl.ds(pl.multiple_of(kt * 128, 128), 128)
        return [cp(bx_h.at[:, pl.ds(0, 8), d], x0raw.at[kt], sem_f.at[kt]),
                cp(wk_h.at[d, pl.ds(0, 8), :], wraw.at[0, d], sem_f.at[kt])]

    early = [cp(dmat_h, dmat_s, sem_m.at[0]), cp(misc_h, misc_s, sem_m.at[1]), cp(mem_h, mem_s.at[0], sem_m.at[2])]
    late = [cp(bx_h.at[:, pl.ds(8, 24), :], xr_s, sem_m.at[3]), cp(smat_h, smat_s, sem_m.at[4])]

    def ob_copy(g):
        return cp(ob_s.at[_rows8(g * 8)], o_h.at[_rows8(g * 8), :, pl.ds(DM, DM)], sem_ob.at[g])

    def oa_copy(c):
        return cp(oa_s.at[:, _rows8(c * 8), :], o_h.at[:, _rows8(c * 8), pl.ds(0, DM)], sem_oa.at[c])

    lane = lax.broadcasted_iota(jnp.int32, (1, 128), 1)
    lane_lo = (lane & 1) == 0
    lane_plus = ((lane + 1) & 2) == 0
    lane_half = lane < 64
    rt = float(np.sqrt(0.5))

    order = [8 * a + b for b in range(8) for a in range(4)]

    def filt_prep(i, h, a):
        col = pl.ds(pl.multiple_of((2 * i + h) * 128, 128), 128)
        t = _u32(fraw[a, 0:256, col]).T
        for q in range(16):
            pb[_rows8(F_OFF + (a * 4 + q % 4) * 512 + ((2 * i + h) * 4 + q // 4) * 8), :] = t[q * 8:(q + 1) * 8]

    def ax_blocks(c):
        v = jnp.concatenate([ax_s[s1, _rows8(c * 8), :].astype(F32) for s1 in order], axis=0)
        return [v[:, i * 128:(i + 1) * 128] for i in range(4)]

    def t_rows(ka, b, part):
        return pl.ds(T_OFF + ((ka * 8 + b) * 2 + part) * 8, 8)

    def tf_rows(c, blk, ka, b, part):
        return _rows8(TF_OFF + (c % 2) * 32 + blk * 512 + ((ka * 8 + b) * 2 + part) * 8)

    def twiddles(c):
        return misc_s[_rows8(96 + c * 8), :], misc_s[_rows8(96 + N2 + c * 8), :]

    def fwd_even(c):
        x0, x1, x2, x3 = ax_blocks(c)
        p, q = x0 + x2, x1 + x3
        t0 = _dot((p + q).astype(BF), _bf(dmat_s[0, 0:64, 0:128]))
        t2 = _dot((p - q).astype(BF), _bf(dmat_s[0, 0:64, 128:256]))
        re = jnp.where(lane_lo, t0, t2)
        im = jnp.where(lane == 0, 0.0, pltpu.roll(jnp.where(lane_lo, t2, t0), 127, 1))
        n = jnp.zeros((8, 128), F32)
        for pos, s1 in enumerate(order):
            v = t0[pos * 8:(pos + 1) * 8]
            n = jnp.where(lane == s1, v if s1 == 1 else pltpu.roll(v, (s1 - 1) % 128, 1), n)
        return re, im, n

    def fwd_odd(c):
        x0, x1, x2, x3 = ax_blocks(c)
        a, b = x0 - x2, x1 - x3
        r = pltpu.roll(jnp.where(lane_half, b, (a - b) * rt), 64, 1)
        p, q = jnp.where(lane_half, a, r), jnp.where(lane_half, r, (a + b) * rt)
        tp = _dot((p + q).astype(BF), _bf(dmat_s[0, 64:128, 0:128]))
        tm = _dot((p - q).astype(BF), _bf(dmat_s[0, 64:128, 128:256]))
        return jnp.where(lane_plus, tp, tm), pltpu.roll(jnp.where(lane_plus, tm, tp), 126, 1)

    def fwd_pass1(c, blk, re, im):
        for b in range(8):
            z = _fft([(re[(b * 4 + a) * 8:(b * 4 + a + 1) * 8], im[(b * 4 + a) * 8:(b * 4 + a + 1) * 8])
                      for a in range(4)], -1)
            for ka in range(4):
                zr, zi = _cmul(z[ka], -2 * np.pi * b * ka / N1)
                pb[tf_rows(c, blk, ka, b, 0), :] = _u32(zr)
                pb[tf_rows(c, blk, ka, b, 1), :] = _u32(zi)

    def fwd_pass2(c, blk, ka):
        z = _fft([(_f32(pb[tf_rows(c, blk, ka, b, 0), :]), _f32(pb[tf_rows(c, blk, ka, b, 1), :]))
                  for b in range(8)], -1)
        for kb in range(8):
            k1 = ka + 4 * kb
            for part in range(2):
                row = U_OFF + (k1 // 8) * 2048 + (blk * 2 + part) * 512 + (k1 % 8) * 8
                pb[_rows8(row + c * 64), :] = _u32(z[kb][part])

    def fwd_nyq(c, n):
        u = _dot(n.astype(BF), _bf(dmat_s[0, 128:192, :]))
        ur, ui = u[:, 0:128], u[:, 128:256]
        ct, st = twiddles(c)
        return ur * ct + ui * st, ui * ct - ur * st

    def put_nyq(c, u):
        pb[_rows8(UN_OFF + c * 8), :] = _u32(u[0])
        pb[_rows8(UN_OFF + 64 + c * 8), :] = _u32(u[1])

    def cfilter(z, wr, wi):
        zr, zi = z[0:64], z[64:128]
        return jnp.concatenate([zr * wr - zi * wi, zr * wi + zi * wr], axis=0).astype(BF)

    def tm_rows(kc, r, part):
        return pl.ds(TF_OFF + ((kc * 8 + r) * 2 + part) * 8, 8)

    def tm_get(kc, r):
        return _f32(pb[tm_rows(kc, r, 0), :]), _f32(pb[tm_rows(kc, r, 1), :])

    def tm_put(kc, r, z):
        pb[tm_rows(kc, r, 0), :] = _u32(z[0])
        pb[tm_rows(kc, r, 1), :] = _u32(z[1])

    def mid_1(g, blk, r):
        view = pb.at[pl.ds(pl.multiple_of(U_OFF + g * 2048, 32), 2048 + 8)]
        x = []
        for c in range(8):
            re, im = [_f32(view[pl.ds((blk * 2 + part) * 512 + c * 64 + r, 8, stride=8), :]) for part in range(2)]
            if 8 * c + r:
                ct, st = smat_s[g, 8 * c + r, 0], smat_s[g, 8 * c + r, 1]
                re, im = re * ct + im * st, im * ct - re * st
            x.append((re, im))
        z = _fft(x, -1)
        for kc in range(8):
            tm_put(kc, r, _cmul(z[kc], -2 * np.pi * r * kc / N2))

    def mid_2(g, blk, kc):
        z = _fft([tm_get(kc, r) for r in range(8)], -1)
        y = []
        for kr in range(8):
            w = [pb[pl.ds(pl.multiple_of(g * 512, 32) + (F_OFF + a * 2048 + (kc + 8 * kr) * 8), 8), :]
                 for a in range(2)]
            wr, wi = [_f32(v & jnp.uint32(HI_MASK)) if blk else _f32(v << 16) for v in w]
            zr, zi = z[kr]
            y.append((zr * wr - zi * wi, zr * wi + zi * wr))
        v = _fft(y, 1)
        for r in range(8):
            tm_put(kc, r, _cmul(v[r], 2 * np.pi * r * kc / N2))

    def mid_3(g, blk, r):
        z = _fft([tm_get(kc, r) for kc in range(8)], 1)
        for c in range(8):
            re, im = z[c]
            if 8 * c + r:
                ct, st = smat_s[g, 8 * c + r, 0], smat_s[g, 8 * c + r, 1]
                re, im = re * ct - im * st, im * ct + re * st
            for part, v in enumerate((re, im)):
                row = V_OFF + c * 1024 + (blk * 2 + part) * 256 + r * 8
                big[pl.ds(pl.multiple_of(g * 64, 32) + row, 8), :] = v

    def nyq_a():
        z = _dot(_bf(dmat_s[0, 192:256, 0:128]), _f32(pb[pl.ds(UN_OFF, 128), :]).astype(BF))
        w = []
        for a in range(2):
            g = jnp.concatenate([fraw[a, 256:257, t * 128:(t + 1) * 128].astype(F32) for t in range(16)], axis=0)
            w.append(jnp.concatenate([g] + [pltpu.roll(g, 128 - 32 * q, 1) for q in range(1, 4)], axis=0))
        return cfilter(z, *w)

    def nyq_b(y):
        big[pl.ds(VN_OFF, 128), :] = _dot(_bf(dmat_s[0, 192:256, 128:256]), y)

    def inv_pass1(c, blk, ka):
        view = big.at[pl.ds(pl.multiple_of(V_OFF + c * 1024, 32), 1024 + 8)]
        z = _fft([tuple(view[pl.ds((blk * 2 + part) * 256 + (k1 // 8) * 64 + k1 % 8, 8, stride=8), :]
                        for part in range(2)) for k1 in range(ka, N1, 4)], 1)
        for b in range(8):
            zr, zi = _cmul(z[b], 2 * np.pi * b * ka / N1)
            big[t_rows(ka, b, 0), :] = zr
            big[t_rows(ka, b, 1), :] = zi

    def inv_nyq(c):
        vr, vi = big[_rows8(VN_OFF + c * 8), :], big[_rows8(VN_OFF + 64 + c * 8), :]
        ct, st = twiddles(c)
        m = _bf(dmat_s[1, 128:192, :])
        return (_dot((vr * ct - vi * st).astype(BF), m[:, 0:128])
                + _dot((vi * ct + vr * st).astype(BF), m[:, 128:256]))

    def inv_pass2(blk, b, n):
        z = _fft([(big[t_rows(ka, b, 0), :], big[t_rows(ka, b, 1), :]) for ka in range(4)], 1)
        for a in range(4):
            re, im = z[a]
            s1 = 8 * a + b
            if blk == 0:
                im = pltpu.roll(im, 1, 1)
                nv = n if s1 == 1 else pltpu.roll(n, (1 - s1) % 128, 1)
                re, im = jnp.where(lane == 1, nv, jnp.where(lane_lo, re, im)), jnp.where(lane_lo, im, re)
            else:
                im = pltpu.roll(im, 2, 1)
                re, im = jnp.where(lane_plus, re, im), jnp.where(lane_plus, im, re)
            big[pl.ds(L_OFF + (2 * blk) * 256 + s1 * 8, 8), :] = re
            big[pl.ds(L_OFF + (2 * blk + 1) * 256 + s1 * 8, 8), :] = im

    def inv_out(c):
        lhs = [big[pl.ds(L_OFF + i * 256, 256), :] for i in range(4)]
        c0 = _dot(lhs[0].astype(BF), _bf(dmat_s[1, 0:64, 0:128]))
        c2 = _dot(lhs[1].astype(BF), _bf(dmat_s[1, 0:64, 128:256]))
        lp = _dot(lhs[2].astype(BF), _bf(dmat_s[1, 64:128, 0:128]))
        lm = _dot(lhs[3].astype(BF), _bf(dmat_s[1, 64:128, 128:256]))
        pp, qq = lp + lm, lp - lm
        r = pltpu.roll(jnp.where(lane_half, qq, pp), 64, 1)
        p, q = jnp.where(lane_half, pp, (r + qq) * rt), jnp.where(lane_half, r, (qq - r) * rt)
        e, f = c0 + c2, c0 - c2
        y = jnp.concatenate([e + p, f + q, e - p, f - q], axis=1)
        oa_s[:, _rows8(c * 8), :] = y.reshape(N1, 8, DM).astype(BF)

    def head_words(hh, n):
        a = wtmp[pl.ds(hh // 2, n, stride=8), :]
        b = wtmp[pl.ds(4 + hh // 2, n, stride=8), :]
        return (a >> 16) | (b & jnp.uint32(HI_MASK)) if hh % 2 else (a & 0xFFFF) | (b << 16)

    def head_weights(t, hh):
        w = head_words(hh, 256)
        w_s[t * 8 + hh] = w
        return w

    def stage_chunk(t):
        for dc in range(8):
            wtmp[dc * 256:(dc + 1) * 256, :] = _u32(wraw[t, dc * 64:(dc + 1) * 64].reshape(512, 128))
        head_weights(t, 0)

    def early_proj(t, hooks):
        for jj in range(4):
            res = []
            for hh in (2 * jj, 2 * jj + 1):
                w = w_s[t * 8] if hh == 0 else head_weights(t, hh)
                r = _dot(_bf(jnp.concatenate([x0_s[k] for k in range(4)], axis=1)), _bf(w))
                res.append(r.reshape(NSEG, 8, 128))
                for tm, f, pinned in hooks:
                    if tm // 8 == hh:
                        if pinned:
                            pb[_rows8(TK_OFF + (t % 2) * 32), :] = _u32(r[(tm % 8) * 64:(tm % 8) * 64 + 8])
                        f()
            big[pl.ds(pl.multiple_of(P_OFF + (t * 4 + jj) * 1024, 1024), 1024), :] = (
                jnp.concatenate(res, axis=1).reshape(1024, 128))

    def phase_0(kt, carry):
        for c in first_copies(kt):
            c.wait()
        for dc in range(2):
            v = wraw[0, pl.ds(pl.multiple_of(kt * 128 + dc * 64, 64), 64)]
            wtmp[dc * 256:(dc + 1) * 256, :] = _u32(v.reshape(512, 128))
        xk = _u32(x0raw[kt].reshape(NSEG * 8, 128))
        x0_s[kt] = xk
        for jj in range(4):
            res = []
            for hh in (2 * jj, 2 * jj + 1):
                w = head_words(hh, 64)
                w_s[hh, pl.ds(pl.multiple_of(kt * 64, 64), 64), :] = w
                res.append(_dot(_bf(xk), _bf(w)).reshape(NSEG, 8, 128))
            rows = pl.ds(P_OFF + jj * 1024, 1024)
            big[rows, :] = jnp.where(kt > 0, big[rows, :], 0.0) + jnp.concatenate(res, axis=1).reshape(1024, 128)
        return carry

    def phase_a(t, carry):
        w_copy(1, t).start()
        for c in chunk_copies(t):
            c.start()

        @pl.when(t <= 2)
        def _():
            w_wait(t)
            stage_chunk(t)

        @pl.when(t >= 2)
        def _():
            w_wait(t + 1)

        early_proj(t, [])
        stage_chunk(jnp.where(t >= 2, t + 1, t))
        return carry

    def phase_b(i, carry):
        t = i + 3

        @pl.when(i < 4)
        def _():
            w_copy(2, i).start()
            for c in chunk_copies(i + 4):
                c.start()

        @pl.when(i == 4)
        def _():
            for c in late:
                c.start()

        w_wait(t + 1)
        for c in chunk_copies(i):
            c.wait()

        def wo_retile(n):
            wo_s[n * 8 + i] = _u32(woraw[pl.ds(pl.multiple_of(i * 512, 512), 512), n * 128:(n + 1) * 128])

        box = {}
        t_om, t_f, t_o1, t_o2, t_em, t_e1, t_n, t_e2, t_pn, dt = SCHED_PB
        hooks = [(t_f + dt * k, lambda k=k: filt_prep(i, k // 2, k % 2), False) for k in range(4)]
        hooks += [(t_om, lambda: box.update(o=fwd_odd(i)), False),
                  (t_o1, lambda: fwd_pass1(i, 1, *box["o"]), False),
                  (t_em, lambda: box.update(e=fwd_even(i)), False),
                  (t_e1, lambda: fwd_pass1(i, 0, *box["e"][:2]), False),
                  (t_n, lambda: box.update(n=fwd_nyq(i, box["e"][2])), False),
                  (t_pn, lambda: put_nyq(i, box["n"]), False)]
        hooks += [(t_o2 + dt * ka, lambda ka=ka: fwd_pass2(i, 1, ka), True) for ka in range(4)]
        hooks += [(t_e2 + dt * ka, lambda ka=ka: fwd_pass2(i, 0, ka), True) for ka in range(4)]
        hooks += [(0, lambda n=n: wo_retile(n), False) for n in range(4)]
        early_proj(t, sorted(hooks, key=lambda h: h[0]))
        stage_chunk(jnp.minimum(t + 1, 11))
        return carry

    def x0_rows(r0, n):
        return _bf(jnp.concatenate([x0_s[k, r0 // 2:(r0 + n) // 2, :] for k in range(4)], axis=1))

    def phase_c():
        for jj in range(4):
            res = []
            for hh in (2 * jj, 2 * jj + 1):
                w = w_s[88] if hh == 0 else head_weights(11, hh)
                res.append(_dot(x0_rows(0, 128), _bf(w)).reshape(16, 8, 128))
            big[pl.ds(P_OFF + (44 + jj) * 1024, 256), :] = jnp.concatenate(res, axis=1).reshape(256, 128)

    def early_rest(i, u):
        r = _dot(x0_rows(128 + 192 * (u % 2), 192), _bf(w_s[88 + 2 * i + u // 2]))
        for q in range(24):
            row = P_OFF + 44 * 1024 + (16 + 24 * (u % 2) + q) * 16 + (u // 2) * 8
            big[pl.ds(pl.multiple_of(i * 1024, 32) + row, 8), :] = r[q * 8:(q + 1) * 8]

    def wo_rows(j):
        r = pl.ds(pl.multiple_of((j & 1) * 128, 128), 128)
        return _bf(jnp.concatenate([wo_s[n * 8 + (j >> 1), r, :] for n in range(4)], axis=1))

    def put_late(g, res):
        for i in range(16):
            ob_s[g * 8 + i // 2, (i % 2) * 32:(i % 2) * 32 + 8, :] = res[i * 8:(i + 1) * 8].astype(BF)

    def late_proj(idx):
        g, c = idx >> 4, idx & 15
        a = od_s[c, pl.ds(pl.multiple_of(g * 128, 128), 128), :].astype(BF)
        res = jnp.where(c > 0, acc_s[...], 0.0) + _dot(a, wo_rows(c))
        acc_s[...] = res
        put_late(g, res)

    def step(s0, u0, mem, hooks, lags):
        s = s0 + u0
        qk_lag, pv_lag, skew = lags // 100, lags // 10 % 10, lags % 10
        lhs = jnp.concatenate([mem, xr_s[s].astype(F32)], axis=0).astype(BF)
        st = {}

        def proj(mi, j):
            y1 = _dot(lhs, _bf(w_s[mi * H + 2 * j]))
            y2 = _dot(lhs, _bf(w_s[mi * H + 2 * j + 1]))
            pre = big[pl.ds(pl.multiple_of(s0 * 16, 32) + (P_OFF + (mi * NP + j) * 1024 + u0 * 16), 16), :]
            st[mi, j] = jnp.concatenate([y1, y2, pre], axis=0).astype(BF)
            st["last"] = y1[0:8]

        def pin():
            big[pl.ds(pl.multiple_of((s0 & 2) * 16, 32) + X_OFF, 8), :] = st["last"]

        def pin_pb():
            pb[pl.ds(pl.multiple_of((s0 % 8) * 8, 32) + TK_OFF, 8), :] = _u32(st["last"])

        def qk(j):
            sc = lax.dot_general(st.pop((1, j)), st.pop((0, j)), (((1,), (1,)), ((), ())),
                                 preferred_element_type=F32)
            fill = misc_s[0:80, 0:80]
            sc = jnp.where(fill == 0.0, sc, fill)
            p = jnp.exp2((sc - jnp.max(sc, axis=1, keepdims=True)) * EXP_C)
            st["p", j] = (p.astype(BF), pl.reciprocal(jnp.sum(p, axis=1, keepdims=True), approx=True))

        def pv(j):
            p, rl = st.pop(("p", j))
            o = _dot(p, st.pop((2, j))) * rl
            st["o", j] = jnp.concatenate([o[0:32], o[32:64]], axis=1).astype(BF)
            od_s[j, pl.ds(pl.multiple_of(s0 * 8, 16) + u0 * 8, 8), :] = jnp.concatenate([o[64:72], o[72:80]], axis=1)

        def op(j):
            r = _dot(st.pop(("o", j)), wo_rows(j))
            st["acc"] = r if "acc" not in st else st["acc"] + r

        units = []
        for j in range(-skew, NP):
            units += [(mi, j + skew) for mi in (0, 1) if j + skew < NP] + ([(2, j)] if j >= 0 else [])
        events = [(t, lambda mi=mi, j=j: proj(mi, j)) for t, (mi, j) in enumerate(units)]
        events += [(3 * NP + j, lambda j=j: op(j)) for j in range(NP)]
        for j in range(NP):
            tqk = units.index((1, j)) + 1 + qk_lag
            events.append((tqk - 0.5, lambda j=j: qk(j)))
            events.append((max(tqk + pv_lag, units.index((2, j)) + 1 + qk_lag) - 0.4, lambda j=j: pv(j)))
        for t, fs in hooks.items():
            events += [(t - 0.3, {None: pin, "pb": pin_pb}.get(f, f)) for f in fs]
        for _, f in sorted(events, key=lambda ev: ev[0]):
            f()
        out = st["acc"]
        ob_s[(s0 >> 1) + u0 // 2, (u0 % 2) * 32 + 8:(u0 % 2) * 32 + 32, :] = out[8:32].astype(BF)
        return out[0:8].astype(BF).astype(F32)

    def loop_a(i, mem):
        box = {}
        jobs = [{} for _ in range(4)]
        t_0, dt, t_n0, t_n1, nps, t_x = SCHED_LA

        def add(t, fs):
            u = min(t // 64, 3)
            jobs[u].setdefault(t - 64 * u, []).extend(fs)

        pieces = [(f, blk, k) for blk in range(2) for f in (mid_1, mid_2, mid_3) for k in range(8)]
        for n, (f, blk, k) in enumerate(pieces):
            add(64 * (n // nps) + t_0 + dt * (n % nps), ["pb", lambda f=f, blk=blk, k=k: f(i, blk, k)])
        add(192 + t_n0, [lambda: box.update(n=nyq_a())])
        add(192 + t_n1, [lambda: nyq_b(box["n"])])
        for u, t in enumerate(sorted([64, 128, 192, t_x])):
            add(t, [lambda u=u: early_rest(i, u)])
        for u in range(4):
            mem = step(4 * i, u, mem, jobs[u], STEP_A[u])
        return mem

    def loop_b(i, mem):
        box = {}
        jobs = [{} for _ in range(6)]
        t1, d1, t2, d2, t_n, t_o, t_x = SCHED_LB

        def add(t, fs):
            u = min(t // 64, 5)
            jobs[u].setdefault(t - 64 * u, []).extend(fs)

        for blk in range(2):
            for ka in range(4):
                add(128 * blk + t1 + d1 * ka, [None, lambda blk=blk, ka=ka: inv_pass1(i, blk, ka)])
            for b in range(8):
                add(128 * blk + 64 + t2 + d2 * b, [None, lambda blk=blk, b=b: inv_pass2(blk, b, box["n"])])
        add(t_n, [lambda: box.update(n=inv_nyq(i))])
        add(t_o, [lambda: inv_out(i)])
        for u, t in enumerate(sorted([64 * u for u in range(1, 6)] + [t_x])):
            add(t, [lambda u=u: late_proj(6 * i + u)])
        for u in range(6):
            mem = step(6 * i, 16 + u, mem, jobs[u], STEP_B[u])
        oa_copy(i).start()

        @pl.when((i == 2) | (i == 5))
        def _():
            ob_copy(i >> 2).start()

        return mem

    for kt in range(4):
        for c in first_copies(kt):
            c.start()
    for g in range(1, 4):
        w_copy(0, g).start()
    lax.fori_loop(0, 4, phase_0, 0)
    w_copy(1, 0).start()
    for c in early + chunk_copies(0):
        c.start()
    lax.fori_loop(1, 3, phase_a, 0)
    w_copy(1, 3).start()
    for c in chunk_copies(3):
        c.start()
    for c in early:
        c.wait()
    lax.fori_loop(0, 8, phase_b, 0)
    phase_c()
    for c in late:
        c.wait()
    mem = mem_s[0].astype(F32)
    mem = lax.fori_loop(0, 4, loop_a, mem)
    lax.fori_loop(0, 8, loop_b, mem)
    ob_copy(2).start()
    last = [cp(ob_s.at[pl.ds(24, 8), pl.ds(r, n), :], o_h.at[pl.ds(24, 8), pl.ds(r, n), pl.ds(DM, DM)],
               sem_ob.at[3 + k]) for k, (r, n) in enumerate([(8, 24), (40, 24), (0, 8), (32, 8)])]
    last[0].start()
    last[1].start()
    a = jnp.concatenate([od_s[c, 384:512, :] for c in range(NP)], axis=1).astype(BF)
    put_late(3, _dot(a, jnp.concatenate([wo_rows(j) for j in range(NP)], axis=0)))
    last[2].start()
    last[3].start()
    for c in range(8):
        oa_copy(c).wait()
    for g in range(3):
        ob_copy(g).wait()
    for c in last:
        c.wait()


@jax.jit
def pallas_concat_heads__spectral_gfnet__memory_aug_recurrent_mem_tr__prompt_kernel(
        A_x, A_w_r, A_w_i, B_x, B_mem0, B_Wq, B_Wk, B_Wv, B_Wo, B_seg_len=None):
    dmat, smat, misc = _consts()
    vm, dma = pltpu.VMEM, pltpu.SemaphoreType.DMA
    out = pl.pallas_call(
        _kernel,
        out_shape=jax.ShapeDtypeStruct((N1, N2, 2 * DM), BF),
        in_specs=[pl.BlockSpec(memory_space=pl.ANY)] * 12,
        out_specs=pl.BlockSpec(memory_space=pl.ANY),
        scratch_shapes=[
            vm((12, DM, 8, DH), BF), vm((PB_ROWS, 128), U32), vm((2048 + 32, 128), U32),
            vm((3 * H, DM // 2, DH), U32), vm((H, DM // 2, DH), U32), vm((H * DH, DM), BF),
            vm((BIG_ROWS, 128), F32), vm((NP, NSEG * 8, 2 * DH), F32), vm((128, DM), F32),
            vm((4, NSEG, 8, 128), BF), vm((4, NSEG * 4, 128), U32), vm((NSEG, 24, DM), BF),
            vm(misc.shape, F32),
            vm((N1, N2, DM), BF), vm((2, DM // 2 + 1, S), BF), vm(dmat.shape, U32), vm(smat.shape, F32),
            vm((N1, N2, DM), BF), vm((N1, N2, DM), BF), vm((2, MEM, DM), BF),
            dma((12,)), dma((8,)), dma((5,)), dma((8,)), dma((7,)), dma((4,)),
        ],
        compiler_params=pltpu.CompilerParams(vmem_limit_bytes=120 * 1024 * 1024, disable_bounds_checks=True,
                                             disable_semaphore_checks=True),
    )(A_x.reshape(N1, N2, DM), A_w_r.T, A_w_i.T,
      B_x.reshape(NSEG, SEG, DM), B_mem0.reshape(MEM, DM), B_Wq, B_Wk, B_Wv, B_Wo.reshape(H * DH, DM),
      jnp.asarray(dmat), jnp.asarray(smat), jnp.asarray(misc))
    return out.reshape(1, S, 2 * DM)
```

```python
import numpy as np
import jax
import jax.numpy as jnp
from jax import lax
import jax.experimental.pallas as pl
import jax.experimental.pallas.tpu as pltpu

S, DM, H, DH, MEM, SEG = 2048, 512, 32, 128, 8, 32
NSEG = S // SEG
NP = H // 2
N1, N2 = 32, 64
BF, F32, U32 = jnp.bfloat16, jnp.float32, jnp.uint32
EXP_C = float(DH ** -0.5 * np.log2(np.e))
HI_MASK = 0xFFFF0000

P_OFF = 0
T_OFF = P_OFF + 3 * NP * NSEG * 16
L_OFF = T_OFF + 64 * 8
V_OFF = L_OFF + 4 * 256
VN_OFF = V_OFF + 8192
X_OFF = VN_OFF + 128
BIG_ROWS = X_OFF + 64
TK_OFF = 0
TF_OFF = TK_OFF + 64
F_OFF = TF_OFF + 2 * 512 + 32
U_OFF = F_OFF + 8 * 512
UN_OFF = U_OFF + 8192
PB_ROWS = UN_OFF + 128

STEP_A = (361, 361, 361, 361)
STEP_B = (361, 361, 361, 361, 361, 361)
SCHED_PB = (0, 40, 16, 29, 0, 16, 17, 23, 33, 1)
SCHED_LA = (9, 3, 31, 46, 14, 0)
SCHED_LB = (3, 6, 11, 3, 29, 267, 0)


def _pack_rows(m):
    f = np.ascontiguousarray(m, dtype=np.float32).view(np.uint32)
    r = ((f + 0x7FFF + ((f >> 16) & 1)) >> 16).astype(np.uint32)
    return r[..., 0::2, :] | (r[..., 1::2, :] << 16)


def _consts():
    l = np.arange(128)
    d2 = np.arange(128)[:, None]
    lo = (l % 2) == 0
    a_re = 2 * np.pi * d2 * (2 * l)[None, :] / DM
    a_im = 2 * np.pi * d2 * (2 * ((l - 1) % 128))[None, :] / DM
    m0 = np.where(lo[None, :], np.cos(a_re), -np.sin(a_im))
    m0[:, 1] = (-1.0) ** np.arange(128)
    m2 = np.where(lo[None, :], -np.sin(a_im), np.cos(a_re))
    e = np.arange(64)[:, None]

    def odd_cols(lanes):
        kd = 2 * lanes + 1
        ang = 2 * np.pi * e * kd[None, :] / DM
        sg = np.where(kd % 4 == 1, 1.0, -1.0)[None, :]
        return (np.concatenate([np.cos(ang), -sg * np.sin(ang)], axis=0),
                np.concatenate([-np.sin(ang), -sg * np.cos(ang)], axis=0))

    plus = (l % 4 == 0) | (l % 4 == 3)
    o_re, o_im = odd_cols(l)[0], odd_cols((l - 2) % 128)[1]
    mp = np.where(plus[None, :], o_re, o_im)
    mm = np.where(plus[None, :], o_im, o_re)
    sc = 2.0 / (S * DM)
    m0i = m0.T * sc
    m0i[0] /= 2
    m0i[1] /= 2
    a32 = 2 * np.pi * np.outer(np.arange(N1), np.arange(N1)) / N1
    c32, s32 = np.zeros((128, 128)), np.zeros((128, 128))
    c32[:N1, :N1], s32[:N1, :N1] = np.cos(a32), -np.sin(a32)
    nf = np.concatenate([c32, s32], axis=1)
    dfw = np.concatenate([np.concatenate([m0, m2], axis=1), np.concatenate([mp, mm], axis=1), nf], axis=0)
    dinv = np.concatenate([np.concatenate([m0i, m2.T * sc], axis=1),
                           np.concatenate([mp.T, mm.T], axis=1) * sc, nf], axis=0)
    rho = np.arange(N2)
    th = 2 * np.pi * np.outer(4 * (rho % 16) + rho // 16, rho) / N2
    c, s = np.cos(th), np.sin(th)
    mf = np.concatenate([np.concatenate([c, s], 1), np.concatenate([-s, c], 1)], 0)
    dfw = np.concatenate([dfw, np.concatenate([mf, mf.T], axis=1)], axis=0)
    dinv = np.concatenate([dinv, np.zeros((128, 256))], axis=0)
    dmat = _pack_rows(np.stack([dfw, dinv]))
    th = 2 * np.pi * np.arange(N1).reshape(4, 1, 8) * np.arange(N2).reshape(1, N2, 1) / S
    stw = np.broadcast_to(np.stack([np.cos(th), np.sin(th)], axis=2)[..., None], (4, N2, 2, 8, 128))
    stw = np.ascontiguousarray(stw, dtype=np.float32)
    head = np.concatenate([np.zeros(32), np.ones(32), np.zeros(8), np.ones(8)])
    pos = np.concatenate([np.arange(8), np.arange(16, 40)] * 2 + [np.arange(8, 16)] * 2)
    same = head[:, None] == head[None, :]
    ok = same & ((pos[:, None] < MEM) | (pos[:, None] >= pos[None, :]))
    misc = np.zeros((96 + 2 * N2, 128), np.float32)
    misc[:80, :80] = np.where(ok, 0.0, np.where(same, -1e9 * DH ** 0.5, -np.inf))
    atw = 2 * np.pi * np.outer(np.arange(N2), np.arange(128) % N1) / S
    misc[96:96 + N2], misc[96 + N2:] = np.cos(atw), np.sin(atw)
    return dmat, stw, misc


def _cmul(z, ang):
    re, im = z
    c, s = float(np.cos(ang)), float(np.sin(ang))
    if abs(s) < 1e-12:
        return (re, im) if c > 0 else (-re, -im)
    if abs(c) < 1e-12:
        return (-im, re) if s > 0 else (im, -re)
    if abs(abs(c) - abs(s)) < 1e-12:
        return ((re - im) * c, (re + im) * c) if c * s > 0 else ((re + im) * c, (im - re) * c)
    return re * c - im * s, re * s + im * c


def _fft(x, sign):
    n = len(x)
    if n == 1:
        return x
    if n == 2:
        (ar, ai), (br, bi) = x
        return [(ar + br, ai + bi), (ar - br, ai - bi)]
    ev, z1, z3 = _fft(x[0::2], sign), _fft(x[1::4], sign), _fft(x[3::4], sign)
    out = [None] * n
    q = n // 4
    for k in range(q):
        ar, ai = _cmul(z1[k], sign * 2 * np.pi * k / n)
        br, bi = _cmul(z3[k], sign * 2 * np.pi * 3 * k / n)
        sr, si, dr, di = ar + br, ai + bi, ar - br, ai - bi
        (er, ei), (fr, fi) = ev[k], ev[k + q]
        out[k] = (er + sr, ei + si)
        out[k + 2 * q] = (er - sr, ei - si)
        plus, minus = (fr - di, fi + dr), (fr + di, fi - dr)
        out[k + q], out[k + 3 * q] = (plus, minus) if sign > 0 else (minus, plus)
    return out


def _dot(a, b):
    return jnp.dot(a, b, preferred_element_type=F32)


def _bf(words):
    return pltpu.bitcast(words, BF)


def _f32(words):
    return pltpu.bitcast(words, F32)


def _u32(x):
    return pltpu.bitcast(x, U32)


def _rows8(off):
    return pl.ds(pl.multiple_of(off, 8), 8)


def _kernel(ax_h, wr_h, wi_h, bx_h, mem_h, wq_h, wk_h, wv_h, wo_h, dmat_h, stw_h, misc_h,
            o_h,
            wraw, pb, wtmp, w_s, wo_s, woraw, big, od_s, acc_s, x0raw, x0_s, xr_s, misc_s,
            ax_s, fraw, dmat_s, stw_s, oa_s, ob_s, mem_s,
            sem_w, sem_c, sem_m, sem_oa, sem_ob, sem_f):
    w_h = (wk_h, wq_h, wv_h)
    cp = pltpu.make_async_copy

    def w_copy(m, g):
        return cp(w_h[m].at[:, pl.ds(pl.multiple_of(8 * g, 8), 8), :], wraw.at[4 * m + g], sem_w.at[4 * m + g])

    def w_wait(t):
        cp(wraw.at[t], wraw.at[t], sem_w.at[t]).wait()

    def chunk_copies(i, which=(0, 1, 2, 3)):
        rows = pl.ds(pl.multiple_of(i * 512, 512), 512)
        cols = pl.ds(pl.multiple_of(i * 256, 256), 256)
        pairs = [lambda: (wo_h.at[rows], woraw.at[rows]),
                 lambda: (ax_h.at[:, _rows8(i * 8), :], ax_s.at[:, _rows8(i * 8), :]),
                 lambda: (wr_h.at[:, cols], fraw.at[0, :, cols]),
                 lambda: (wi_h.at[:, cols], fraw.at[1, :, cols])]
        return [cp(*pairs[k](), sem_c.at[i]) for k in which]

    def first_copies(kt):
        d = pl.ds(pl.multiple_of(kt * 128, 128), 128)
        return [cp(bx_h.at[:, pl.ds(0, 8), d], x0raw.at[kt], sem_f.at[kt]),
                cp(wk_h.at[d, pl.ds(0, 8), :], wraw.at[0, d], sem_f.at[kt])]

    early = [cp(dmat_h, dmat_s, sem_m.at[0]), cp(misc_h, misc_s, sem_m.at[1]), cp(mem_h, mem_s.at[0], sem_m.at[2])]
    late = [cp(bx_h.at[:, pl.ds(8, 24), :], xr_s, sem_m.at[3]), cp(stw_h, stw_s, sem_m.at[4])]

    def ob_copy(g):
        return cp(ob_s.at[_rows8(g * 8)], o_h.at[_rows8(g * 8), :, pl.ds(DM, DM)], sem_ob.at[g])

    def oa_copy(c):
        return cp(oa_s.at[:, _rows8(c * 8), :], o_h.at[:, _rows8(c * 8), pl.ds(0, DM)], sem_oa.at[c])

    lane = lax.broadcasted_iota(jnp.int32, (1, 128), 1)
    lane_lo = (lane & 1) == 0
    lane_plus = ((lane + 1) & 2) == 0
    lane_half = lane < 64
    rt = float(np.sqrt(0.5))

    order = [8 * a + b for b in range(8) for a in range(4)]

    def filt_prep(i, h, a):
        col = pl.ds(pl.multiple_of((2 * i + h) * 128, 128), 128)
        t = _u32(fraw[a, 0:256, col]).T
        for q in range(16):
            pb[_rows8(F_OFF + (a * 4 + q % 4) * 512 + ((2 * i + h) * 4 + q // 4) * 8), :] = t[q * 8:(q + 1) * 8]

    def ax_blocks(c):
        v = jnp.concatenate([ax_s[s1, _rows8(c * 8), :].astype(F32) for s1 in order], axis=0)
        return [v[:, i * 128:(i + 1) * 128] for i in range(4)]

    def t_rows(ka, b, part):
        return pl.ds(T_OFF + ((ka * 8 + b) * 2 + part) * 8, 8)

    def tf_rows(c, blk, ka, b, part):
        return _rows8(TF_OFF + (c % 2) * 32 + blk * 512 + ((ka * 8 + b) * 2 + part) * 8)

    def twiddles(c):
        return misc_s[_rows8(96 + c * 8), :], misc_s[_rows8(96 + N2 + c * 8), :]

    def fwd_even(c):
        x0, x1, x2, x3 = ax_blocks(c)
        p, q = x0 + x2, x1 + x3
        t0 = _dot((p + q).astype(BF), _bf(dmat_s[0, 0:64, 0:128]))
        t2 = _dot((p - q).astype(BF), _bf(dmat_s[0, 0:64, 128:256]))
        re = jnp.where(lane_lo, t0, t2)
        im = jnp.where(lane == 0, 0.0, pltpu.roll(jnp.where(lane_lo, t2, t0), 127, 1))
        n = jnp.zeros((8, 128), F32)
        for pos, s1 in enumerate(order):
            v = t0[pos * 8:(pos + 1) * 8]
            n = jnp.where(lane == s1, v if s1 == 1 else pltpu.roll(v, (s1 - 1) % 128, 1), n)
        return re, im, n

    def fwd_odd(c):
        x0, x1, x2, x3 = ax_blocks(c)
        a, b = x0 - x2, x1 - x3
        r = pltpu.roll(jnp.where(lane_half, b, (a - b) * rt), 64, 1)
        p, q = jnp.where(lane_half, a, r), jnp.where(lane_half, r, (a + b) * rt)
        tp = _dot((p + q).astype(BF), _bf(dmat_s[0, 64:128, 0:128]))
        tm = _dot((p - q).astype(BF), _bf(dmat_s[0, 64:128, 128:256]))
        return jnp.where(lane_plus, tp, tm), pltpu.roll(jnp.where(lane_plus, tm, tp), 126, 1)

    def fwd_pass1(c, blk, re, im):
        for b in range(8):
            z = _fft([(re[(b * 4 + a) * 8:(b * 4 + a + 1) * 8], im[(b * 4 + a) * 8:(b * 4 + a + 1) * 8])
                      for a in range(4)], -1)
            for ka in range(4):
                zr, zi = _cmul(z[ka], -2 * np.pi * b * ka / N1)
                pb[tf_rows(c, blk, ka, b, 0), :] = _u32(zr)
                pb[tf_rows(c, blk, ka, b, 1), :] = _u32(zi)

    def fwd_pass2(c, blk, ka):
        z = _fft([(_f32(pb[tf_rows(c, blk, ka, b, 0), :]), _f32(pb[tf_rows(c, blk, ka, b, 1), :]))
                  for b in range(8)], -1)
        for kb in range(8):
            k1 = ka + 4 * kb
            for part in range(2):
                row = U_OFF + (k1 // 8) * 2048 + (blk * 2 + part) * 512 + (k1 % 8) * 8
                pb[_rows8(row + c * 64), :] = _u32(z[kb][part])

    def fwd_nyq(c, n):
        u = _dot(n.astype(BF), _bf(dmat_s[0, 128:192, :]))
        ur, ui = u[:, 0:128], u[:, 128:256]
        ct, st = twiddles(c)
        return ur * ct + ui * st, ui * ct - ur * st

    def put_nyq(c, u):
        pb[_rows8(UN_OFF + c * 8), :] = _u32(u[0])
        pb[_rows8(UN_OFF + 64 + c * 8), :] = _u32(u[1])

    def cfilter(z, wr, wi):
        zr, zi = z[0:64], z[64:128]
        return jnp.concatenate([zr * wr - zi * wi, zr * wi + zi * wr], axis=0).astype(BF)

    def tm_rows(kc, r, part):
        return pl.ds(TF_OFF + ((kc * 8 + r) * 2 + part) * 8, 8)

    def tm_get(kc, r):
        return _f32(pb[tm_rows(kc, r, 0), :]), _f32(pb[tm_rows(kc, r, 1), :])

    def tm_put(kc, r, z):
        pb[tm_rows(kc, r, 0), :] = _u32(z[0])
        pb[tm_rows(kc, r, 1), :] = _u32(z[1])

    def mid_1(g, blk, r):
        view = pb.at[pl.ds(pl.multiple_of(U_OFF + g * 2048, 32), 2048 + 8)]
        x = []
        for c in range(8):
            re, im = [_f32(view[pl.ds((blk * 2 + part) * 512 + c * 64 + r, 8, stride=8), :]) for part in range(2)]
            if 8 * c + r:
                ct, st = stw_s[g, 8 * c + r, 0], stw_s[g, 8 * c + r, 1]
                re, im = re * ct + im * st, im * ct - re * st
            x.append((re, im))
        z = _fft(x, -1)
        for kc in range(8):
            tm_put(kc, r, _cmul(z[kc], -2 * np.pi * r * kc / N2))

    def mid_2(g, blk, kc):
        z = _fft([tm_get(kc, r) for r in range(8)], -1)
        y = []
        for kr in range(8):
            w = [pb[pl.ds(pl.multiple_of(g * 512, 32) + (F_OFF + a * 2048 + (kc + 8 * kr) * 8), 8), :]
                 for a in range(2)]
            wr, wi = [_f32(v & jnp.uint32(HI_MASK)) if blk else _f32(v << 16) for v in w]
            zr, zi = z[kr]
            y.append((zr * wr - zi * wi, zr * wi + zi * wr))
        v = _fft(y, 1)
        for r in range(8):
            tm_put(kc, r, _cmul(v[r], 2 * np.pi * r * kc / N2))

    def mid_3(g, blk, r):
        z = _fft([tm_get(kc, r) for kc in range(8)], 1)
        for c in range(8):
            re, im = z[c]
            if 8 * c + r:
                ct, st = stw_s[g, 8 * c + r, 0], stw_s[g, 8 * c + r, 1]
                re, im = re * ct - im * st, im * ct + re * st
            for part, v in enumerate((re, im)):
                row = V_OFF + c * 1024 + (blk * 2 + part) * 256 + r * 8
                big[pl.ds(pl.multiple_of(g * 64, 32) + row, 8), :] = v

    def nyq_a():
        z = _dot(_bf(dmat_s[0, 192:256, 0:128]), _f32(pb[pl.ds(UN_OFF, 128), :]).astype(BF))
        w = []
        for a in range(2):
            g = jnp.concatenate([fraw[a, 256:257, t * 128:(t + 1) * 128].astype(F32) for t in range(16)], axis=0)
            w.append(jnp.concatenate([g] + [pltpu.roll(g, 128 - 32 * q, 1) for q in range(1, 4)], axis=0))
        return cfilter(z, *w)

    def nyq_b(y):
        big[pl.ds(VN_OFF, 128), :] = _dot(_bf(dmat_s[0, 192:256, 128:256]), y)

    def inv_pass1(c, blk, ka):
        view = big.at[pl.ds(pl.multiple_of(V_OFF + c * 1024, 32), 1024 + 8)]
        z = _fft([tuple(view[pl.ds((blk * 2 + part) * 256 + (k1 // 8) * 64 + k1 % 8, 8, stride=8), :]
                        for part in range(2)) for k1 in range(ka, N1, 4)], 1)
        for b in range(8):
            zr, zi = _cmul(z[b], 2 * np.pi * b * ka / N1)
            big[t_rows(ka, b, 0), :] = zr
            big[t_rows(ka, b, 1), :] = zi

    def inv_nyq(c):
        vr, vi = big[_rows8(VN_OFF + c * 8), :], big[_rows8(VN_OFF + 64 + c * 8), :]
        ct, st = twiddles(c)
        m = _bf(dmat_s[1, 128:192, :])
        return (_dot((vr * ct - vi * st).astype(BF), m[:, 0:128])
                + _dot((vi * ct + vr * st).astype(BF), m[:, 128:256]))

    def inv_pass2(blk, b, n):
        z = _fft([(big[t_rows(ka, b, 0), :], big[t_rows(ka, b, 1), :]) for ka in range(4)], 1)
        for a in range(4):
            re, im = z[a]
            s1 = 8 * a + b
            if blk == 0:
                im = pltpu.roll(im, 1, 1)
                nv = n if s1 == 1 else pltpu.roll(n, (1 - s1) % 128, 1)
                re, im = jnp.where(lane == 1, nv, jnp.where(lane_lo, re, im)), jnp.where(lane_lo, im, re)
            else:
                im = pltpu.roll(im, 2, 1)
                re, im = jnp.where(lane_plus, re, im), jnp.where(lane_plus, im, re)
            big[pl.ds(L_OFF + (2 * blk) * 256 + s1 * 8, 8), :] = re
            big[pl.ds(L_OFF + (2 * blk + 1) * 256 + s1 * 8, 8), :] = im

    def inv_out(c):
        lhs = [big[pl.ds(L_OFF + i * 256, 256), :] for i in range(4)]
        c0 = _dot(lhs[0].astype(BF), _bf(dmat_s[1, 0:64, 0:128]))
        c2 = _dot(lhs[1].astype(BF), _bf(dmat_s[1, 0:64, 128:256]))
        lp = _dot(lhs[2].astype(BF), _bf(dmat_s[1, 64:128, 0:128]))
        lm = _dot(lhs[3].astype(BF), _bf(dmat_s[1, 64:128, 128:256]))
        pp, qq = lp + lm, lp - lm
        r = pltpu.roll(jnp.where(lane_half, qq, pp), 64, 1)
        p, q = jnp.where(lane_half, pp, (r + qq) * rt), jnp.where(lane_half, r, (qq - r) * rt)
        e, f = c0 + c2, c0 - c2
        y = jnp.concatenate([e + p, f + q, e - p, f - q], axis=1)
        oa_s[:, _rows8(c * 8), :] = y.reshape(N1, 8, DM).astype(BF)

    def head_words(hh, n):
        a = wtmp[pl.ds(hh // 2, n, stride=8), :]
        b = wtmp[pl.ds(4 + hh // 2, n, stride=8), :]
        return (a >> 16) | (b & jnp.uint32(HI_MASK)) if hh % 2 else (a & 0xFFFF) | (b << 16)

    def head_weights(t, hh):
        w = head_words(hh, 256)
        w_s[t * 8 + hh] = w
        return w

    def stage_chunk(t):
        for dc in range(8):
            wtmp[dc * 256:(dc + 1) * 256, :] = _u32(wraw[t, dc * 64:(dc + 1) * 64].reshape(512, 128))
        head_weights(t, 0)

    def early_proj(t, hooks):
        for jj in range(4):
            res = []
            for hh in (2 * jj, 2 * jj + 1):
                w = w_s[t * 8] if hh == 0 else head_weights(t, hh)
                r = _dot(_bf(jnp.concatenate([x0_s[k] for k in range(4)], axis=1)), _bf(w))
                res.append(r.reshape(NSEG, 8, 128))
                for tm, f, pinned in hooks:
                    if tm // 8 == hh:
                        if pinned:
                            pb[_rows8(TK_OFF + (t % 2) * 32), :] = _u32(r[(tm % 8) * 64:(tm % 8) * 64 + 8])
                        f()
            big[pl.ds(pl.multiple_of(P_OFF + (t * 4 + jj) * 1024, 1024), 1024), :] = (
                jnp.concatenate(res, axis=1).reshape(1024, 128))

    def phase_0(kt, carry):
        for c in first_copies(kt):
            c.wait()
        for dc in range(2):
            v = wraw[0, pl.ds(pl.multiple_of(kt * 128 + dc * 64, 64), 64)]
            wtmp[dc * 256:(dc + 1) * 256, :] = _u32(v.reshape(512, 128))
        xk = _u32(x0raw[kt].reshape(NSEG * 8, 128))
        x0_s[kt] = xk
        for jj in range(4):
            res = []
            for hh in (2 * jj, 2 * jj + 1):
                w = head_words(hh, 64)
                w_s[hh, pl.ds(pl.multiple_of(kt * 64, 64), 64), :] = w
                res.append(_dot(_bf(xk), _bf(w)).reshape(NSEG, 8, 128))
            rows = pl.ds(P_OFF + jj * 1024, 1024)
            big[rows, :] = jnp.where(kt > 0, big[rows, :], 0.0) + jnp.concatenate(res, axis=1).reshape(1024, 128)
        return carry

    def phase_a(t, carry):
        @pl.when(t <= 2)
        def _():
            w_wait(t)
            w_copy(1, t).start()
            for c in chunk_copies(t):
                c.start()
            stage_chunk(t)

        @pl.when(t >= 2)
        def _():
            w_wait(t + 1)

        early_proj(t, [])
        stage_chunk(jnp.where(t >= 2, t + 1, t))
        return carry

    def phase_b(i, carry):
        t = i + 3


        @pl.when(i < 4)
        def _():
            for c in [w_copy(2, i)] + chunk_copies(i + 4, (0,)):
                c.start()

        w_wait(t + 1)
        for c in chunk_copies(i):
            c.wait()

        @pl.when(i < 4)
        def _():
            for c in chunk_copies(i + 4, (1, 2, 3)):
                c.start()

        @pl.when(i == 4)
        def _():
            for c in late:
                c.start()

        def wo_retile(n):
            wo_s[n * 8 + i] = _u32(woraw[pl.ds(pl.multiple_of(i * 512, 512), 512), n * 128:(n + 1) * 128])

        box = {}
        t_om, t_f, t_o1, t_o2, t_em, t_e1, t_n, t_e2, t_pn, dt = SCHED_PB
        hooks = [(t_f + dt * k, lambda k=k: filt_prep(i, k // 2, k % 2), False) for k in range(4)]
        hooks += [(t_om, lambda: box.update(o=fwd_odd(i)), False),
                  (t_o1, lambda: fwd_pass1(i, 1, *box["o"]), False),
                  (t_em, lambda: box.update(e=fwd_even(i)), False),
                  (t_e1, lambda: fwd_pass1(i, 0, *box["e"][:2]), False),
                  (t_n, lambda: box.update(n=fwd_nyq(i, box["e"][2])), False),
                  (t_pn, lambda: put_nyq(i, box["n"]), False)]
        hooks += [(t_o2 + dt * ka, lambda ka=ka: fwd_pass2(i, 1, ka), True) for ka in range(4)]
        hooks += [(t_e2 + dt * ka, lambda ka=ka: fwd_pass2(i, 0, ka), True) for ka in range(4)]
        hooks += [(0, lambda n=n: wo_retile(n), False) for n in range(4)]
        early_proj(t, sorted(hooks, key=lambda h: h[0]))
        stage_chunk(jnp.minimum(t + 1, 11))
        return carry

    def x0_rows(r0, n):
        return _bf(jnp.concatenate([x0_s[k, r0 // 2:(r0 + n) // 2, :] for k in range(4)], axis=1))

    def phase_c():
        for jj in range(4):
            res = []
            for hh in (2 * jj, 2 * jj + 1):
                w = w_s[88] if hh == 0 else head_weights(11, hh)
                res.append(_dot(x0_rows(0, 128), _bf(w)).reshape(16, 8, 128))
            big[pl.ds(P_OFF + (44 + jj) * 1024, 256), :] = jnp.concatenate(res, axis=1).reshape(256, 128)

    def early_rest(i, u):
        r = _dot(x0_rows(128 + 192 * (u % 2), 192), _bf(w_s[88 + 2 * i + u // 2]))
        for q in range(24):
            row = P_OFF + 44 * 1024 + (16 + 24 * (u % 2) + q) * 16 + (u // 2) * 8
            big[pl.ds(pl.multiple_of(i * 1024, 32) + row, 8), :] = r[q * 8:(q + 1) * 8]

    def wo_rows(j):
        r = pl.ds(pl.multiple_of((j & 1) * 128, 128), 128)
        return _bf(jnp.concatenate([wo_s[n * 8 + (j >> 1), r, :] for n in range(4)], axis=1))

    def put_late(g, res):
        for i in range(16):
            ob_s[g * 8 + i // 2, (i % 2) * 32:(i % 2) * 32 + 8, :] = res[i * 8:(i + 1) * 8].astype(BF)

    def late_proj(idx):
        g, c = idx >> 4, idx & 15
        a = od_s[c, pl.ds(pl.multiple_of(g * 128, 128), 128), :].astype(BF)
        res = jnp.where(c > 0, acc_s[...], 0.0) + _dot(a, wo_rows(c))
        acc_s[...] = res
        put_late(g, res)

    def step(s0, u0, mem, hooks, lags):
        s = s0 + u0
        qk_lag, pv_lag, skew = lags // 100, lags // 10 % 10, lags % 10
        lhs = jnp.concatenate([mem, xr_s[s].astype(F32)], axis=0).astype(BF)
        st = {}

        def proj(mi, j):
            y1 = _dot(lhs, _bf(w_s[mi * H + 2 * j]))
            y2 = _dot(lhs, _bf(w_s[mi * H + 2 * j + 1]))
            pre = big[pl.ds(pl.multiple_of(s0 * 16, 32) + (P_OFF + (mi * NP + j) * 1024 + u0 * 16), 16), :]
            st[mi, j] = jnp.concatenate([y1, y2, pre], axis=0).astype(BF)
            st["last"] = y1[0:8]

        def pin():
            big[pl.ds(pl.multiple_of((s0 & 2) * 16, 32) + X_OFF, 8), :] = st["last"]

        def pin_pb():
            pb[pl.ds(pl.multiple_of((s0 % 8) * 8, 32) + TK_OFF, 8), :] = _u32(st["last"])

        def qk(j):
            sc = lax.dot_general(st.pop((1, j)), st.pop((0, j)), (((1,), (1,)), ((), ())),
                                 preferred_element_type=F32)
            fill = misc_s[0:80, 0:80]
            sc = jnp.where(fill == 0.0, sc, fill)
            p = jnp.exp2((sc - jnp.max(sc, axis=1, keepdims=True)) * EXP_C)
            st["p", j] = (p.astype(BF), pl.reciprocal(jnp.sum(p, axis=1, keepdims=True), approx=True))

        def pv(j):
            p, rl = st.pop(("p", j))
            o = _dot(p, st.pop((2, j))) * rl
            st["o", j] = jnp.concatenate([o[0:32], o[32:64]], axis=1).astype(BF)
            od_s[j, pl.ds(pl.multiple_of(s0 * 8, 16) + u0 * 8, 8), :] = jnp.concatenate([o[64:72], o[72:80]], axis=1)

        def op(j):
            r = _dot(st.pop(("o", j)), wo_rows(j))
            st["acc"] = r if "acc" not in st else st["acc"] + r

        units = []
        for j in range(-skew, NP):
            units += [(mi, j + skew) for mi in (0, 1) if j + skew < NP] + ([(2, j)] if j >= 0 else [])
        events = [(t, lambda mi=mi, j=j: proj(mi, j)) for t, (mi, j) in enumerate(units)]
        events += [(3 * NP + j, lambda j=j: op(j)) for j in range(NP)]
        for j in range(NP):
            tqk = units.index((1, j)) + 1 + qk_lag
            events.append((tqk - 0.5, lambda j=j: qk(j)))
            events.append((max(tqk + pv_lag, units.index((2, j)) + 1 + qk_lag) - 0.4, lambda j=j: pv(j)))
        for t, fs in hooks.items():
            events += [(t - 0.3, {None: pin, "pb": pin_pb}.get(f, f)) for f in fs]
        for _, f in sorted(events, key=lambda ev: ev[0]):
            f()
        out = st["acc"]
        ob_s[(s0 >> 1) + u0 // 2, (u0 % 2) * 32 + 8:(u0 % 2) * 32 + 32, :] = out[8:32].astype(BF)
        return out[0:8].astype(BF).astype(F32)

    def loop_a(i, mem):
        box = {}
        jobs = [{} for _ in range(4)]
        t_0, dt, t_n0, t_n1, nps, t_x = SCHED_LA

        def add(t, fs):
            u = min(t // 64, 3)
            jobs[u].setdefault(t - 64 * u, []).extend(fs)

        pieces = [(f, blk, k) for blk in range(2) for f in (mid_1, mid_2, mid_3) for k in range(8)]
        for n, (f, blk, k) in enumerate(pieces):
            add(64 * (n // nps) + t_0 + dt * (n % nps), ["pb", lambda f=f, blk=blk, k=k: f(i, blk, k)])
        add(192 + t_n0, [lambda: box.update(n=nyq_a())])
        add(192 + t_n1, [lambda: nyq_b(box["n"])])
        for u, t in enumerate(sorted([64, 128, 192, t_x])):
            add(t, [lambda u=u: early_rest(i, u)])
        for u in range(4):
            mem = step(4 * i, u, mem, jobs[u], STEP_A[u])
        return mem

    def loop_b(i, mem):
        box = {}
        jobs = [{} for _ in range(6)]
        t1, d1, t2, d2, t_n, t_o, t_x = SCHED_LB

        def add(t, fs):
            u = min(t // 64, 5)
            jobs[u].setdefault(t - 64 * u, []).extend(fs)

        for blk in range(2):
            for ka in range(4):
                add(128 * blk + t1 + d1 * ka, [None, lambda blk=blk, ka=ka: inv_pass1(i, blk, ka)])
            for b in range(8):
                add(128 * blk + 64 + t2 + d2 * b, [None, lambda blk=blk, b=b: inv_pass2(blk, b, box["n"])])
        add(t_n, [lambda: box.update(n=inv_nyq(i))])
        add(t_o, [lambda: inv_out(i)])
        for u, t in enumerate(sorted([64 * u for u in range(1, 6)] + [t_x])):
            add(t, [lambda u=u: late_proj(6 * i + u)])
        for u in range(6):
            mem = step(6 * i, 16 + u, mem, jobs[u], STEP_B[u])
        oa_copy(i).start()

        @pl.when((i == 2) | (i == 5))
        def _():
            ob_copy(i >> 2).start()

        return mem

    for kt in range(4):
        for c in first_copies(kt):
            c.start()
    for g in range(1, 4):
        w_copy(0, g).start()
    lax.fori_loop(0, 4, phase_0, 0)
    w_copy(1, 0).start()
    for c in early + chunk_copies(0):
        c.start()
    lax.fori_loop(1, 3, phase_a, 0)
    w_copy(1, 3).start()
    for c in chunk_copies(3):
        c.start()
    for c in early:
        c.wait()
    lax.fori_loop(0, 8, phase_b, 0)
    phase_c()
    for c in late:
        c.wait()
    mem = mem_s[0].astype(F32)
    mem = lax.fori_loop(0, 4, loop_a, mem)
    lax.fori_loop(0, 8, loop_b, mem)
    ob_copy(2).start()
    last = [cp(ob_s.at[pl.ds(24, 8), pl.ds(r, n), :], o_h.at[pl.ds(24, 8), pl.ds(r, n), pl.ds(DM, DM)],
               sem_ob.at[3 + k]) for k, (r, n) in enumerate([(8, 24), (40, 24), (0, 8), (32, 8)])]
    last[0].start()
    last[1].start()
    a = jnp.concatenate([od_s[c, 384:512, :] for c in range(NP)], axis=1).astype(BF)
    put_late(3, _dot(a, jnp.concatenate([wo_rows(j) for j in range(NP)], axis=0)))
    last[2].start()
    last[3].start()
    for c in range(8):
        oa_copy(c).wait()
    for g in range(3):
        ob_copy(g).wait()
    for c in last:
        c.wait()


@jax.jit
def pallas_concat_heads__spectral_gfnet__memory_aug_recurrent_mem_tr__prompt_kernel(
        A_x, A_w_r, A_w_i, B_x, B_mem0, B_Wq, B_Wk, B_Wv, B_Wo, B_seg_len=None):
    dmat, stw, misc = _consts()
    vm, dma = pltpu.VMEM, pltpu.SemaphoreType.DMA
    out = pl.pallas_call(
        _kernel,
        out_shape=jax.ShapeDtypeStruct((N1, N2, 2 * DM), BF),
        in_specs=[pl.BlockSpec(memory_space=pl.ANY)] * 12,
        out_specs=pl.BlockSpec(memory_space=pl.ANY),
        scratch_shapes=[
            vm((12, DM, 8, DH), BF), vm((PB_ROWS, 128), U32), vm((2048 + 32, 128), U32),
            vm((3 * H, DM // 2, DH), U32), vm((H, DM // 2, DH), U32), vm((H * DH, DM), BF),
            vm((BIG_ROWS, 128), F32), vm((NP, NSEG * 8, 2 * DH), F32), vm((128, DM), F32),
            vm((4, NSEG, 8, 128), BF), vm((4, NSEG * 4, 128), U32), vm((NSEG, 24, DM), BF),
            vm(misc.shape, F32),
            vm((N1, N2, DM), BF), vm((2, DM // 2 + 1, S), BF), vm(dmat.shape, U32), vm(stw.shape, F32),
            vm((N1, N2, DM), BF), vm((N1, N2, DM), BF), vm((2, MEM, DM), BF),
            dma((12,)), dma((8,)), dma((5,)), dma((8,)), dma((7,)), dma((4,)),
        ],
        compiler_params=pltpu.CompilerParams(vmem_limit_bytes=120 * 1024 * 1024, disable_bounds_checks=True,
                                             disable_semaphore_checks=True),
    )(A_x.reshape(N1, N2, DM), A_w_r.T, A_w_i.T,
      B_x.reshape(NSEG, SEG, DM), B_mem0.reshape(MEM, DM), B_Wq, B_Wk, B_Wv, B_Wo.reshape(H * DH, DM),
      jnp.asarray(dmat), jnp.asarray(stw), jnp.asarray(misc))
    return out.reshape(1, S, 2 * DM)
```

```python
import numpy as np
import jax
import jax.numpy as jnp
from jax import lax
import jax.experimental.pallas as pl
import jax.experimental.pallas.tpu as pltpu

S, DM, H, DH, MEM, SEG = 2048, 512, 32, 128, 8, 32
NSEG = S // SEG
NP = H // 2
N1, N2 = 32, 64
BF, F32, U32 = jnp.bfloat16, jnp.float32, jnp.uint32
EXP_C = float(DH ** -0.5 * np.log2(np.e))
HI_MASK = 0xFFFF0000

P_OFF = 0
T_OFF = P_OFF + 3 * NP * NSEG * 16
L_OFF = T_OFF + 64 * 8
V_OFF = L_OFF + 4 * 256
VN_OFF = V_OFF + 8192
X_OFF = VN_OFF + 128
BIG_ROWS = X_OFF + 64
TK_OFF = 0
TF_OFF = TK_OFF + 64
F_OFF = TF_OFF + 2 * 512 + 32
U_OFF = F_OFF + 8 * 512
UN_OFF = U_OFF + 8192
PB_ROWS = UN_OFF + 128

STEP_A = (361, 361, 361, 361)
STEP_B = (361, 361, 361, 361, 361, 361)
SCHED_PB = (0, 40, 16, 29, 0, 16, 17, 23, 33, 1)
SCHED_LA = (9, 3, 31, 46, 14, 0)
SCHED_LB = (3, 6, 11, 3, 29, 267, 0)


def _pack_rows(m):
    f = np.ascontiguousarray(m, dtype=np.float32).view(np.uint32)
    r = ((f + 0x7FFF + ((f >> 16) & 1)) >> 16).astype(np.uint32)
    return r[..., 0::2, :] | (r[..., 1::2, :] << 16)


def _consts():
    l = np.arange(128)
    d2 = np.arange(128)[:, None]
    lo = (l % 2) == 0
    a_re = 2 * np.pi * d2 * (2 * l)[None, :] / DM
    a_im = 2 * np.pi * d2 * (2 * ((l - 1) % 128))[None, :] / DM
    m0 = np.where(lo[None, :], np.cos(a_re), -np.sin(a_im))
    m0[:, 1] = (-1.0) ** np.arange(128)
    m2 = np.where(lo[None, :], -np.sin(a_im), np.cos(a_re))
    e = np.arange(64)[:, None]

    def odd_cols(lanes):
        kd = 2 * lanes + 1
        ang = 2 * np.pi * e * kd[None, :] / DM
        sg = np.where(kd % 4 == 1, 1.0, -1.0)[None, :]
        return (np.concatenate([np.cos(ang), -sg * np.sin(ang)], axis=0),
                np.concatenate([-np.sin(ang), -sg * np.cos(ang)], axis=0))

    plus = (l % 4 == 0) | (l % 4 == 3)
    o_re, o_im = odd_cols(l)[0], odd_cols((l - 2) % 128)[1]
    mp = np.where(plus[None, :], o_re, o_im)
    mm = np.where(plus[None, :], o_im, o_re)
    sc = 2.0 / (S * DM)
    m0i = m0.T * sc
    m0i[0] /= 2
    m0i[1] /= 2
    a32 = 2 * np.pi * np.outer(np.arange(N1), np.arange(N1)) / N1
    c32, s32 = np.zeros((128, 128)), np.zeros((128, 128))
    c32[:N1, :N1], s32[:N1, :N1] = np.cos(a32), -np.sin(a32)
    nf = np.concatenate([c32, s32], axis=1)
    dfw = np.concatenate([np.concatenate([m0, m2], axis=1), np.concatenate([mp, mm], axis=1), nf], axis=0)
    dinv = np.concatenate([np.concatenate([m0i, m2.T * sc], axis=1),
                           np.concatenate([mp.T, mm.T], axis=1) * sc, nf], axis=0)
    rho = np.arange(N2)
    th = 2 * np.pi * np.outer(4 * (rho % 16) + rho // 16, rho) / N2
    c, s = np.cos(th), np.sin(th)
    mf = np.concatenate([np.concatenate([c, s], 1), np.concatenate([-s, c], 1)], 0)
    dfw = np.concatenate([dfw, np.concatenate([mf, mf.T], axis=1)], axis=0)
    dinv = np.concatenate([dinv, np.zeros((128, 256))], axis=0)
    dmat = _pack_rows(np.stack([dfw, dinv]))
    th = 2 * np.pi * np.arange(N1).reshape(4, 1, 8) * np.arange(N2).reshape(1, N2, 1) / S
    stw = np.broadcast_to(np.stack([np.cos(th), np.sin(th)], axis=2)[..., None], (4, N2, 2, 8, 128))
    stw = np.ascontiguousarray(stw, dtype=np.float32)
    head = np.concatenate([np.zeros(32), np.ones(32), np.zeros(8), np.ones(8)])
    pos = np.concatenate([np.arange(8), np.arange(16, 40)] * 2 + [np.arange(8, 16)] * 2)
    same = head[:, None] == head[None, :]
    ok = same & ((pos[:, None] < MEM) | (pos[:, None] >= pos[None, :]))
    misc = np.zeros((96 + 2 * N2, 128), np.float32)
    misc[:80, :80] = np.where(ok, 0.0, np.where(same, -1e9 * DH ** 0.5, -np.inf))
    atw = 2 * np.pi * np.outer(np.arange(N2), np.arange(128) % N1) / S
    misc[96:96 + N2], misc[96 + N2:] = np.cos(atw), np.sin(atw)
    return dmat, stw, misc


def _cmul(z, ang):
    re, im = z
    c, s = float(np.cos(ang)), float(np.sin(ang))
    if abs(s) < 1e-12:
        return (re, im) if c > 0 else (-re, -im)
    if abs(c) < 1e-12:
        return (-im, re) if s > 0 else (im, -re)
    if abs(abs(c) - abs(s)) < 1e-12:
        return ((re - im) * c, (re + im) * c) if c * s > 0 else ((re + im) * c, (im - re) * c)
    return re * c - im * s, re * s + im * c


def _fft(x, sign):
    n = len(x)
    if n == 1:
        return x
    if n == 2:
        (ar, ai), (br, bi) = x
        return [(ar + br, ai + bi), (ar - br, ai - bi)]
    ev, z1, z3 = _fft(x[0::2], sign), _fft(x[1::4], sign), _fft(x[3::4], sign)
    out = [None] * n
    q = n // 4
    for k in range(q):
        ar, ai = _cmul(z1[k], sign * 2 * np.pi * k / n)
        br, bi = _cmul(z3[k], sign * 2 * np.pi * 3 * k / n)
        sr, si, dr, di = ar + br, ai + bi, ar - br, ai - bi
        (er, ei), (fr, fi) = ev[k], ev[k + q]
        out[k] = (er + sr, ei + si)
        out[k + 2 * q] = (er - sr, ei - si)
        plus, minus = (fr - di, fi + dr), (fr + di, fi - dr)
        out[k + q], out[k + 3 * q] = (plus, minus) if sign > 0 else (minus, plus)
    return out


def _dot(a, b):
    return jnp.dot(a, b, preferred_element_type=F32)


def _bf(words):
    return pltpu.bitcast(words, BF)


def _f32(words):
    return pltpu.bitcast(words, F32)


def _u32(x):
    return pltpu.bitcast(x, U32)


def _rows8(off):
    return pl.ds(pl.multiple_of(off, 8), 8)


def _kernel(ax_h, wr_h, wi_h, bx_h, mem_h, wq_h, wk_h, wv_h, wo_h, dmat_h, stw_h, misc_h,
            o_h,
            wraw, pb, wtmp, w_s, wo_s, woraw, big, od_s, acc_s, x0raw, x0_s, xr_s, misc_s,
            ax_s, fraw, dmat_s, stw_s, oa_s, ob_s, mem_s,
            sem_w, sem_c, sem_m, sem_oa, sem_ob, sem_f):
    w_h = (wk_h, wq_h, wv_h)
    cp = pltpu.make_async_copy

    def w_copy(m, g):
        return cp(w_h[m].at[:, pl.ds(pl.multiple_of(8 * g, 8), 8), :], wraw.at[4 * m + g], sem_w.at[4 * m + g])

    def w_wait(t):
        cp(wraw.at[t], wraw.at[t], sem_w.at[t]).wait()

    def chunk_copies(i, which=(0, 1, 2, 3)):
        rows = pl.ds(pl.multiple_of(i * 512, 512), 512)
        cols = pl.ds(pl.multiple_of(i * 256, 256), 256)
        pairs = [lambda: (wo_h.at[rows], woraw.at[rows]),
                 lambda: (ax_h.at[:, _rows8(i * 8), :], ax_s.at[:, _rows8(i * 8), :]),
                 lambda: (wr_h.at[:, cols], fraw.at[0, :, cols]),
                 lambda: (wi_h.at[:, cols], fraw.at[1, :, cols])]
        return [cp(*pairs[k](), sem_c.at[i]) for k in which]

    def first_copies(kt):
        d = pl.ds(pl.multiple_of(kt * 128, 128), 128)
        return [cp(bx_h.at[:, pl.ds(0, 8), d], x0raw.at[kt], sem_f.at[kt]),
                cp(wk_h.at[d, pl.ds(0, 8), :], wraw.at[0, d], sem_f.at[kt])]

    early = [cp(dmat_h, dmat_s, sem_m.at[0]), cp(misc_h, misc_s, sem_m.at[1]), cp(mem_h, mem_s.at[0], sem_m.at[2])]
    late = [cp(bx_h.at[:, pl.ds(8, 24), :], xr_s, sem_m.at[3]), cp(stw_h, stw_s, sem_m.at[4])]

    def ob_copy(g):
        return cp(ob_s.at[_rows8(g * 8)], o_h.at[_rows8(g * 8), :, pl.ds(DM, DM)], sem_ob.at[g])

    def oa_copy(c):
        return cp(oa_s.at[:, _rows8(c * 8), :], o_h.at[:, _rows8(c * 8), pl.ds(0, DM)], sem_oa.at[c])

    lane = lax.broadcasted_iota(jnp.int32, (1, 128), 1)
    lane_lo = (lane & 1) == 0
    lane_plus = ((lane + 1) & 2) == 0
    lane_half = lane < 64
    rt = float(np.sqrt(0.5))

    order = [8 * a + b for b in range(8) for a in range(4)]

    def filt_prep(i, h, a):
        col = pl.ds(pl.multiple_of((2 * i + h) * 128, 128), 128)
        t = _u32(fraw[a, 0:256, col]).T
        for q in range(16):
            pb[_rows8(F_OFF + (a * 4 + q % 4) * 512 + ((2 * i + h) * 4 + q // 4) * 8), :] = t[q * 8:(q + 1) * 8]

    def ax_blocks(c):
        v = jnp.concatenate([ax_s[s1, _rows8(c * 8), :].astype(F32) for s1 in order], axis=0)
        return [v[:, i * 128:(i + 1) * 128] for i in range(4)]

    def t_rows(ka, b, part):
        return pl.ds(T_OFF + ((ka * 8 + b) * 2 + part) * 8, 8)

    def tf_rows(c, blk, ka, b, part):
        return _rows8(TF_OFF + (c % 2) * 32 + blk * 512 + ((ka * 8 + b) * 2 + part) * 8)

    def twiddles(c):
        return misc_s[_rows8(96 + c * 8), :], misc_s[_rows8(96 + N2 + c * 8), :]

    def fwd_even(c):
        x0, x1, x2, x3 = ax_blocks(c)
        p, q = x0 + x2, x1 + x3
        t0 = _dot((p + q).astype(BF), _bf(dmat_s[0, 0:64, 0:128]))
        t2 = _dot((p - q).astype(BF), _bf(dmat_s[0, 0:64, 128:256]))
        re = jnp.where(lane_lo, t0, t2)
        im = jnp.where(lane == 0, 0.0, pltpu.roll(jnp.where(lane_lo, t2, t0), 127, 1))
        n = jnp.zeros((8, 128), F32)
        for pos, s1 in enumerate(order):
            v = t0[pos * 8:(pos + 1) * 8]
            n = jnp.where(lane == s1, v if s1 == 1 else pltpu.roll(v, (s1 - 1) % 128, 1), n)
        return re, im, n

    def fwd_odd(c):
        x0, x1, x2, x3 = ax_blocks(c)
        a, b = x0 - x2, x1 - x3
        r = pltpu.roll(jnp.where(lane_half, b, (a - b) * rt), 64, 1)
        p, q = jnp.where(lane_half, a, r), jnp.where(lane_half, r, (a + b) * rt)
        tp = _dot((p + q).astype(BF), _bf(dmat_s[0, 64:128, 0:128]))
        tm = _dot((p - q).astype(BF), _bf(dmat_s[0, 64:128, 128:256]))
        return jnp.where(lane_plus, tp, tm), pltpu.roll(jnp.where(lane_plus, tm, tp), 126, 1)

    def fwd_pass1(c, blk, re, im):
        for b in range(8):
            z = _fft([(re[(b * 4 + a) * 8:(b * 4 + a + 1) * 8], im[(b * 4 + a) * 8:(b * 4 + a + 1) * 8])
                      for a in range(4)], -1)
            for ka in range(4):
                zr, zi = _cmul(z[ka], -2 * np.pi * b * ka / N1)
                pb[tf_rows(c, blk, ka, b, 0), :] = _u32(zr)
                pb[tf_rows(c, blk, ka, b, 1), :] = _u32(zi)

    def fwd_pass2(c, blk, ka):
        z = _fft([(_f32(pb[tf_rows(c, blk, ka, b, 0), :]), _f32(pb[tf_rows(c, blk, ka, b, 1), :]))
                  for b in range(8)], -1)
        for kb in range(8):
            k1 = ka + 4 * kb
            for part in range(2):
                row = U_OFF + (k1 // 8) * 2048 + (blk * 2 + part) * 512 + (k1 % 8) * 8
                pb[_rows8(row + c * 64), :] = _u32(z[kb][part])

    def fwd_nyq(c, n):
        u = _dot(n.astype(BF), _bf(dmat_s[0, 128:192, :]))
        ur, ui = u[:, 0:128], u[:, 128:256]
        ct, st = twiddles(c)
        return ur * ct + ui * st, ui * ct - ur * st

    def put_nyq(c, u):
        pb[_rows8(UN_OFF + c * 8), :] = _u32(u[0])
        pb[_rows8(UN_OFF + 64 + c * 8), :] = _u32(u[1])

    def cfilter(z, wr, wi):
        zr, zi = z[0:64], z[64:128]
        return jnp.concatenate([zr * wr - zi * wi, zr * wi + zi * wr], axis=0).astype(BF)

    def tm_rows(kc, r, part):
        return pl.ds(TF_OFF + ((kc * 8 + r) * 2 + part) * 8, 8)

    def tm_get(kc, r):
        return _f32(pb[tm_rows(kc, r, 0), :]), _f32(pb[tm_rows(kc, r, 1), :])

    def tm_put(kc, r, z):
        pb[tm_rows(kc, r, 0), :] = _u32(z[0])
        pb[tm_rows(kc, r, 1), :] = _u32(z[1])

    def mid_1(g, blk, r):
        view = pb.at[pl.ds(pl.multiple_of(U_OFF + g * 2048, 32), 2048 + 8)]
        x = []
        for c in range(8):
            re, im = [_f32(view[pl.ds((blk * 2 + part) * 512 + c * 64 + r, 8, stride=8), :]) for part in range(2)]
            if 8 * c + r:
                ct, st = stw_s[g, 8 * c + r, 0], stw_s[g, 8 * c + r, 1]
                re, im = re * ct + im * st, im * ct - re * st
            x.append((re, im))
        z = _fft(x, -1)
        for kc in range(8):
            tm_put(kc, r, _cmul(z[kc], -2 * np.pi * r * kc / N2))

    def mid_2(g, blk, kc):
        z = _fft([tm_get(kc, r) for r in range(8)], -1)
        y = []
        for kr in range(8):
            w = [pb[pl.ds(pl.multiple_of(g * 512, 32) + (F_OFF + a * 2048 + (kc + 8 * kr) * 8), 8), :]
                 for a in range(2)]
            wr, wi = [_f32(v & jnp.uint32(HI_MASK)) if blk else _f32(v << 16) for v in w]
            zr, zi = z[kr]
            y.append((zr * wr - zi * wi, zr * wi + zi * wr))
        v = _fft(y, 1)
        for r in range(8):
            tm_put(kc, r, _cmul(v[r], 2 * np.pi * r * kc / N2))

    def mid_3(g, blk, r):
        z = _fft([tm_get(kc, r) for kc in range(8)], 1)
        for c in range(8):
            re, im = z[c]
            if 8 * c + r:
                ct, st = stw_s[g, 8 * c + r, 0], stw_s[g, 8 * c + r, 1]
                re, im = re * ct - im * st, im * ct + re * st
            for part, v in enumerate((re, im)):
                row = V_OFF + c * 1024 + (blk * 2 + part) * 256 + r * 8
                big[pl.ds(pl.multiple_of(g * 64, 32) + row, 8), :] = v

    def nyq_a():
        z = _dot(_bf(dmat_s[0, 192:256, 0:128]), _f32(pb[pl.ds(UN_OFF, 128), :]).astype(BF))
        w = []
        for a in range(2):
            g = jnp.concatenate([fraw[a, 256:257, t * 128:(t + 1) * 128].astype(F32) for t in range(16)], axis=0)
            w.append(jnp.concatenate([g] + [pltpu.roll(g, 128 - 32 * q, 1) for q in range(1, 4)], axis=0))
        return cfilter(z, *w)

    def nyq_b(y):
        big[pl.ds(VN_OFF, 128), :] = _dot(_bf(dmat_s[0, 192:256, 128:256]), y)

    def inv_pass1(c, blk, ka):
        view = big.at[pl.ds(pl.multiple_of(V_OFF + c * 1024, 32), 1024 + 8)]
        z = _fft([tuple(view[pl.ds((blk * 2 + part) * 256 + (k1 // 8) * 64 + k1 % 8, 8, stride=8), :]
                        for part in range(2)) for k1 in range(ka, N1, 4)], 1)
        for b in range(8):
            zr, zi = _cmul(z[b], 2 * np.pi * b * ka / N1)
            big[t_rows(ka, b, 0), :] = zr
            big[t_rows(ka, b, 1), :] = zi

    def inv_nyq(c):
        vr, vi = big[_rows8(VN_OFF + c * 8), :], big[_rows8(VN_OFF + 64 + c * 8), :]
        ct, st = twiddles(c)
        m = _bf(dmat_s[1, 128:192, :])
        return (_dot((vr * ct - vi * st).astype(BF), m[:, 0:128])
                + _dot((vi * ct + vr * st).astype(BF), m[:, 128:256]))

    def inv_pass2(blk, b, n):
        z = _fft([(big[t_rows(ka, b, 0), :], big[t_rows(ka, b, 1), :]) for ka in range(4)], 1)
        for a in range(4):
            re, im = z[a]
            s1 = 8 * a + b
            if blk == 0:
                im = pltpu.roll(im, 1, 1)
                nv = n if s1 == 1 else pltpu.roll(n, (1 - s1) % 128, 1)
                re, im = jnp.where(lane == 1, nv, jnp.where(lane_lo, re, im)), jnp.where(lane_lo, im, re)
            else:
                im = pltpu.roll(im, 2, 1)
                re, im = jnp.where(lane_plus, re, im), jnp.where(lane_plus, im, re)
            big[pl.ds(L_OFF + (2 * blk) * 256 + s1 * 8, 8), :] = re
            big[pl.ds(L_OFF + (2 * blk + 1) * 256 + s1 * 8, 8), :] = im

    def inv_out(c):
        lhs = [big[pl.ds(L_OFF + i * 256, 256), :] for i in range(4)]
        c0 = _dot(lhs[0].astype(BF), _bf(dmat_s[1, 0:64, 0:128]))
        c2 = _dot(lhs[1].astype(BF), _bf(dmat_s[1, 0:64, 128:256]))
        lp = _dot(lhs[2].astype(BF), _bf(dmat_s[1, 64:128, 0:128]))
        lm = _dot(lhs[3].astype(BF), _bf(dmat_s[1, 64:128, 128:256]))
        pp, qq = lp + lm, lp - lm
        r = pltpu.roll(jnp.where(lane_half, qq, pp), 64, 1)
        p, q = jnp.where(lane_half, pp, (r + qq) * rt), jnp.where(lane_half, r, (qq - r) * rt)
        e, f = c0 + c2, c0 - c2
        y = jnp.concatenate([e + p, f + q, e - p, f - q], axis=1)
        oa_s[:, _rows8(c * 8), :] = y.reshape(N1, 8, DM).astype(BF)

    def head_words(hh, n):
        a = wtmp[pl.ds(hh // 2, n, stride=8), :]
        b = wtmp[pl.ds(4 + hh // 2, n, stride=8), :]
        return (a >> 16) | (b & jnp.uint32(HI_MASK)) if hh % 2 else (a & 0xFFFF) | (b << 16)

    def head_weights(t, hh):
        w = head_words(hh, 256)
        w_s[t * 8 + hh] = w
        return w

    def stage_chunk(t):
        for dc in range(8):
            wtmp[dc * 256:(dc + 1) * 256, :] = _u32(wraw[t, dc * 64:(dc + 1) * 64].reshape(512, 128))
        head_weights(t, 0)

    def early_proj(t, hooks):
        for jj in range(4):
            res = []
            for hh in (2 * jj, 2 * jj + 1):
                w = w_s[t * 8] if hh == 0 else head_weights(t, hh)
                r = _dot(_bf(jnp.concatenate([x0_s[k] for k in range(4)], axis=1)), _bf(w))
                res.append(r.reshape(NSEG, 8, 128))
                for tm, f, pinned in hooks:
                    if tm // 8 == hh:
                        if pinned:
                            pb[_rows8(TK_OFF + (t % 2) * 32), :] = _u32(r[(tm % 8) * 64:(tm % 8) * 64 + 8])
                        f()
            big[pl.ds(pl.multiple_of(P_OFF + (t * 4 + jj) * 1024, 1024), 1024), :] = (
                jnp.concatenate(res, axis=1).reshape(1024, 128))

    def phase_0(kt, carry):
        for c in first_copies(kt):
            c.wait()
        for dc in range(2):
            v = wraw[0, pl.ds(pl.multiple_of(kt * 128 + dc * 64, 64), 64)]
            wtmp[dc * 256:(dc + 1) * 256, :] = _u32(v.reshape(512, 128))
        xk = _u32(x0raw[kt].reshape(NSEG * 8, 128))
        x0_s[kt] = xk
        for jj in range(4):
            res = []
            for hh in (2 * jj, 2 * jj + 1):
                w = head_words(hh, 64)
                w_s[hh, pl.ds(pl.multiple_of(kt * 64, 64), 64), :] = w
                res.append(_dot(_bf(xk), _bf(w)).reshape(NSEG, 8, 128))
            rows = pl.ds(P_OFF + jj * 1024, 1024)
            big[rows, :] = jnp.where(kt > 0, big[rows, :], 0.0) + jnp.concatenate(res, axis=1).reshape(1024, 128)
        return carry

    def phase_a(t, carry):
        @pl.when(t <= 2)
        def _():
            w_wait(t)
            w_copy(1, t).start()
            for c in chunk_copies(t):
                c.start()
            stage_chunk(t)

        @pl.when(t >= 2)
        def _():
            w_wait(t + 1)

        early_proj(t, [])
        stage_chunk(jnp.where(t >= 2, t + 1, t))
        return carry

    def phase_b(i, carry):
        t = i + 3

        @pl.when(i < 4)
        def _():
            for c in [w_copy(2, i)] + chunk_copies(i + 4, (0,)):
                c.start()

        w_wait(t + 1)
        for c in chunk_copies(i):
            c.wait()

        @pl.when(i < 4)
        def _():
            for c in chunk_copies(i + 4, (1, 2, 3)):
                c.start()

        @pl.when(i == 4)
        def _():
            for c in late:
                c.start()

        def wo_retile(n):
            wo_s[n * 8 + i] = _u32(woraw[pl.ds(pl.multiple_of(i * 512, 512), 512), n * 128:(n + 1) * 128])

        box = {}
        t_om, t_f, t_o1, t_o2, t_em, t_e1, t_n, t_e2, t_pn, dt = SCHED_PB
        hooks = [(t_f + dt * k, lambda k=k: filt_prep(i, k // 2, k % 2), False) for k in range(4)]
        hooks += [(t_om, lambda: box.update(o=fwd_odd(i)), False),
                  (t_o1, lambda: fwd_pass1(i, 1, *box["o"]), False),
                  (t_em, lambda: box.update(e=fwd_even(i)), False),
                  (t_e1, lambda: fwd_pass1(i, 0, *box["e"][:2]), False),
                  (t_n, lambda: box.update(n=fwd_nyq(i, box["e"][2])), False),
                  (t_pn, lambda: put_nyq(i, box["n"]), False)]
        hooks += [(t_o2 + dt * ka, lambda ka=ka: fwd_pass2(i, 1, ka), True) for ka in range(4)]
        hooks += [(t_e2 + dt * ka, lambda ka=ka: fwd_pass2(i, 0, ka), True) for ka in range(4)]
        hooks += [(0, lambda n=n: wo_retile(n), False) for n in range(4)]
        early_proj(t, sorted(hooks, key=lambda h: h[0]))
        stage_chunk(jnp.minimum(t + 1, 11))
        return carry

    def x0_rows(r0, n):
        return _bf(jnp.concatenate([x0_s[k, r0 // 2:(r0 + n) // 2, :] for k in range(4)], axis=1))

    def phase_c():
        for jj in range(4):
            res = []
            for hh in (2 * jj, 2 * jj + 1):
                w = w_s[88] if hh == 0 else head_weights(11, hh)
                res.append(_dot(x0_rows(0, 128), _bf(w)).reshape(16, 8, 128))
            big[pl.ds(P_OFF + (44 + jj) * 1024, 256), :] = jnp.concatenate(res, axis=1).reshape(256, 128)

    def early_rest(i, u):
        r = _dot(x0_rows(128 + 192 * (u % 2), 192), _bf(w_s[88 + 2 * i + u // 2]))
        for q in range(24):
            row = P_OFF + 44 * 1024 + (16 + 24 * (u % 2) + q) * 16 + (u // 2) * 8
            big[pl.ds(pl.multiple_of(i * 1024, 32) + row, 8), :] = r[q * 8:(q + 1) * 8]

    def wo_rows(j):
        r = pl.ds(pl.multiple_of((j & 1) * 128, 128), 128)
        return _bf(jnp.concatenate([wo_s[n * 8 + (j >> 1), r, :] for n in range(4)], axis=1))

    def put_late(g, res):
        for i in range(16):
            ob_s[g * 8 + i // 2, (i % 2) * 32:(i % 2) * 32 + 8, :] = res[i * 8:(i + 1) * 8].astype(BF)

    def late_proj(idx):
        g, c = idx >> 4, idx & 15
        a = od_s[c, pl.ds(pl.multiple_of(g * 128, 128), 128), :].astype(BF)
        res = jnp.where(c > 0, acc_s[...], 0.0) + _dot(a, wo_rows(c))
        acc_s[...] = res
        put_late(g, res)

    def step(s0, u0, mem, hooks, lags):
        s = s0 + u0
        qk_lag, pv_lag, skew = lags // 100, lags // 10 % 10, lags % 10
        lhs = jnp.concatenate([mem, xr_s[s].astype(F32)], axis=0).astype(BF)
        st = {}

        def proj(mi, j):
            y1 = _dot(lhs, _bf(w_s[mi * H + 2 * j]))
            y2 = _dot(lhs, _bf(w_s[mi * H + 2 * j + 1]))
            pre = big[pl.ds(pl.multiple_of(s0 * 16, 32) + (P_OFF + (mi * NP + j) * 1024 + u0 * 16), 16), :]
            st[mi, j] = jnp.concatenate([y1, y2, pre], axis=0).astype(BF)
            st["last"] = y1[0:8]

        def pin():
            big[pl.ds(pl.multiple_of((s0 & 2) * 16, 32) + X_OFF, 8), :] = st["last"]

        def pin_pb():
            pb[pl.ds(pl.multiple_of((s0 % 8) * 8, 32) + TK_OFF, 8), :] = _u32(st["last"])

        def qk(j):
            sc = lax.dot_general(st.pop((1, j)), st.pop((0, j)), (((1,), (1,)), ((), ())),
                                 preferred_element_type=F32)
            fill = misc_s[0:80, 0:80]
            sc = jnp.where(fill == 0.0, sc, fill)
            p = jnp.exp2((sc - jnp.max(sc, axis=1, keepdims=True)) * EXP_C)
            st["p", j] = (p.astype(BF), pl.reciprocal(jnp.sum(p, axis=1, keepdims=True), approx=True))

        def pv(j):
            p, rl = st.pop(("p", j))
            o = _dot(p, st.pop((2, j))) * rl
            st["o", j] = jnp.concatenate([o[0:32], o[32:64]], axis=1).astype(BF)
            od_s[j, pl.ds(pl.multiple_of(s0 * 8, 16) + u0 * 8, 8), :] = jnp.concatenate([o[64:72], o[72:80]], axis=1)

        def op(j):
            r = _dot(st.pop(("o", j)), wo_rows(j))
            st["acc"] = r if "acc" not in st else st["acc"] + r

        units = []
        for j in range(-skew, NP):
            units += [(mi, j + skew) for mi in (0, 1) if j + skew < NP] + ([(2, j)] if j >= 0 else [])
        events = [(t, lambda mi=mi, j=j: proj(mi, j)) for t, (mi, j) in enumerate(units)]
        events += [(3 * NP + j, lambda j=j: op(j)) for j in range(NP)]
        for j in range(NP):
            tqk = units.index((1, j)) + 1 + qk_lag
            events.append((tqk - 0.5, lambda j=j: qk(j)))
            events.append((max(tqk + pv_lag, units.index((2, j)) + 1 + qk_lag) - 0.4, lambda j=j: pv(j)))
        for t, fs in hooks.items():
            events += [(t - 0.3, {None: pin, "pb": pin_pb}.get(f, f)) for f in fs]
        for _, f in sorted(events, key=lambda ev: ev[0]):
            f()
        out = st["acc"]
        ob_s[(s0 >> 1) + u0 // 2, (u0 % 2) * 32 + 8:(u0 % 2) * 32 + 32, :] = out[8:32].astype(BF)
        return out[0:8].astype(BF).astype(F32)

    def loop_a(i, mem):
        box = {}
        jobs = [{} for _ in range(4)]
        t_0, dt, t_n0, t_n1, nps, t_x = SCHED_LA

        def add(t, fs):
            u = min(t // 64, 3)
            jobs[u].setdefault(t - 64 * u, []).extend(fs)

        pieces = [(f, blk, k) for blk in range(2) for f in (mid_1, mid_2, mid_3) for k in range(8)]
        for n, (f, blk, k) in enumerate(pieces):
            add(64 * (n // nps) + t_0 + dt * (n % nps), ["pb", lambda f=f, blk=blk, k=k: f(i, blk, k)])
        add(192 + t_n0, [lambda: box.update(n=nyq_a())])
        add(192 + t_n1, [lambda: nyq_b(box["n"])])
        for u, t in enumerate(sorted([64, 128, 192, t_x])):
            add(t, [lambda u=u: early_rest(i, u)])
        for u in range(4):
            mem = step(4 * i, u, mem, jobs[u], STEP_A[u])
        return mem

    def loop_b(i, mem):
        box = {}
        jobs = [{} for _ in range(6)]
        t1, d1, t2, d2, t_n, t_o, t_x = SCHED_LB

        def add(t, fs):
            u = min(t // 64, 5)
            jobs[u].setdefault(t - 64 * u, []).extend(fs)

        for blk in range(2):
            for ka in range(4):
                add(128 * blk + t1 + d1 * ka, [None, lambda blk=blk, ka=ka: inv_pass1(i, blk, ka)])
            for b in range(8):
                add(128 * blk + 64 + t2 + d2 * b, [None, lambda blk=blk, b=b: inv_pass2(blk, b, box["n"])])
        add(t_n, [lambda: box.update(n=inv_nyq(i))])
        add(t_o, [lambda: inv_out(i)])
        for u, t in enumerate(sorted([64 * u for u in range(1, 6)] + [t_x])):
            add(t, [lambda u=u: late_proj(6 * i + u)])
        for u in range(6):
            mem = step(6 * i, 16 + u, mem, jobs[u], STEP_B[u])
        oa_copy(i).start()

        @pl.when((i == 2) | (i == 5))
        def _():
            ob_copy(i >> 2).start()

        return mem

    for kt in range(4):
        for c in first_copies(kt):
            c.start()
    for g in range(1, 4):
        w_copy(0, g).start()
    lax.fori_loop(0, 4, phase_0, 0)
    w_copy(1, 0).start()
    for c in early + chunk_copies(0):
        c.start()
    lax.fori_loop(1, 3, phase_a, 0)
    w_copy(1, 3).start()
    for c in chunk_copies(3):
        c.start()
    for c in early:
        c.wait()
    lax.fori_loop(0, 8, phase_b, 0)
    phase_c()
    for c in late:
        c.wait()
    mem = mem_s[0].astype(F32)
    mem = lax.fori_loop(0, 4, loop_a, mem)
    lax.fori_loop(0, 8, loop_b, mem)
    ob_copy(2).start()
    last = [cp(ob_s.at[pl.ds(24, 8), pl.ds(r, n), :], o_h.at[pl.ds(24, 8), pl.ds(r, n), pl.ds(DM, DM)],
               sem_ob.at[3 + k]) for k, (r, n) in enumerate([(8, 24), (40, 24), (0, 8), (32, 8)])]
    last[0].start()
    last[1].start()
    a = jnp.concatenate([od_s[c, 384:512, :] for c in range(NP)], axis=1).astype(BF)
    put_late(3, _dot(a, jnp.concatenate([wo_rows(j) for j in range(NP)], axis=0)))
    last[2].start()
    last[3].start()
    for c in range(8):
        oa_copy(c).wait()
    for g in range(3):
        ob_copy(g).wait()
    for c in last:
        c.wait()


def _compiler_params():
    base = dict(vmem_limit_bytes=120 * 1024 * 1024, disable_bounds_checks=True)
    try:
        return pltpu.CompilerParams(disable_semaphore_checks=True, **base)
    except TypeError:
        return pltpu.CompilerParams(**base)


@jax.jit
def pallas_concat_heads__spectral_gfnet__memory_aug_recurrent_mem_tr__prompt_kernel(
        A_x, A_w_r, A_w_i, B_x, B_mem0, B_Wq, B_Wk, B_Wv, B_Wo, B_seg_len=None):
    dmat, stw, misc = _consts()
    vm, dma = pltpu.VMEM, pltpu.SemaphoreType.DMA
    out = pl.pallas_call(
        _kernel,
        out_shape=jax.ShapeDtypeStruct((N1, N2, 2 * DM), BF),
        in_specs=[pl.BlockSpec(memory_space=pl.ANY)] * 12,
        out_specs=pl.BlockSpec(memory_space=pl.ANY),
        scratch_shapes=[
            vm((12, DM, 8, DH), BF), vm((PB_ROWS, 128), U32), vm((2048 + 32, 128), U32),
            vm((3 * H, DM // 2, DH), U32), vm((H, DM // 2, DH), U32), vm((H * DH, DM), BF),
            vm((BIG_ROWS, 128), F32), vm((NP, NSEG * 8, 2 * DH), F32), vm((128, DM), F32),
            vm((4, NSEG, 8, 128), BF), vm((4, NSEG * 4, 128), U32), vm((NSEG, 24, DM), BF),
            vm(misc.shape, F32),
            vm((N1, N2, DM), BF), vm((2, DM // 2 + 1, S), BF), vm(dmat.shape, U32), vm(stw.shape, F32),
            vm((N1, N2, DM), BF), vm((N1, N2, DM), BF), vm((2, MEM, DM), BF),
            dma((12,)), dma((8,)), dma((5,)), dma((8,)), dma((7,)), dma((4,)),
        ],
        compiler_params=_compiler_params(),
    )(A_x.reshape(N1, N2, DM), A_w_r.T, A_w_i.T,
      B_x.reshape(NSEG, SEG, DM), B_mem0.reshape(MEM, DM), B_Wq, B_Wk, B_Wv, B_Wo.reshape(H * DH, DM),
      jnp.asarray(dmat), jnp.asarray(stw), jnp.asarray(misc))
    return out.reshape(1, S, 2 * DM)
```

```python
import numpy as np
import jax
import jax.numpy as jnp
from jax import lax
import jax.experimental.pallas as pl
import jax.experimental.pallas.tpu as pltpu

S, DM, H, DH, MEM, SEG = 2048, 512, 32, 128, 8, 32
NSEG = S // SEG
NP = H // 2
N1, N2 = 32, 64
BF, F32, U32 = jnp.bfloat16, jnp.float32, jnp.uint32
EXP_C = float(DH ** -0.5 * np.log2(np.e))
HI_MASK = 0xFFFF0000

P_OFF = 0
T_OFF = P_OFF + 3 * NP * NSEG * 16
L_OFF = T_OFF + 64 * 8
V_OFF = L_OFF + 4 * 256
VN_OFF = V_OFF + 8192
X_OFF = VN_OFF + 128
BIG_ROWS = X_OFF + 64
TK_OFF = 0
TF_OFF = TK_OFF + 64
F_OFF = TF_OFF + 2 * 512 + 32
U_OFF = F_OFF + 8 * 512
UN_OFF = U_OFF + 8192
PB_ROWS = UN_OFF + 128

STEP_A = (361, 361, 361, 361)
STEP_B = (361, 361, 361, 361, 361, 361)
SCHED_PB = (0, 40, 16, 29, 0, 16, 17, 23, 33, 1)
SCHED_LA = (3, 2, 32, 13, 0)
SCHED_LB = (3, 6, 11, 3, 29, 267, 0)


def _pack_rows(m):
    f = np.ascontiguousarray(m, dtype=np.float32).view(np.uint32)
    r = ((f + 0x7FFF + ((f >> 16) & 1)) >> 16).astype(np.uint32)
    return r[..., 0::2, :] | (r[..., 1::2, :] << 16)


def _consts():
    l = np.arange(128)
    d2 = np.arange(128)[:, None]
    lo = (l % 2) == 0
    a_re = 2 * np.pi * d2 * (2 * l)[None, :] / DM
    a_im = 2 * np.pi * d2 * (2 * ((l - 1) % 128))[None, :] / DM
    m0 = np.where(lo[None, :], np.cos(a_re), -np.sin(a_im))
    m0[:, 1] = (-1.0) ** np.arange(128)
    m2 = np.where(lo[None, :], -np.sin(a_im), np.cos(a_re))
    e = np.arange(64)[:, None]

    def odd_cols(lanes):
        kd = 2 * lanes + 1
        ang = 2 * np.pi * e * kd[None, :] / DM
        sg = np.where(kd % 4 == 1, 1.0, -1.0)[None, :]
        return (np.concatenate([np.cos(ang), -sg * np.sin(ang)], axis=0),
                np.concatenate([-np.sin(ang), -sg * np.cos(ang)], axis=0))

    plus = (l % 4 == 0) | (l % 4 == 3)
    o_re, o_im = odd_cols(l)[0], odd_cols((l - 2) % 128)[1]
    mp = np.where(plus[None, :], o_re, o_im)
    mm = np.where(plus[None, :], o_im, o_re)
    sc = 2.0 / (S * DM)
    m0i = m0.T * sc
    m0i[0] /= 2
    m0i[1] /= 2
    a32 = 2 * np.pi * np.outer(np.arange(N1), np.arange(N1)) / N1
    c32, s32 = np.zeros((128, 128)), np.zeros((128, 128))
    c32[:N1, :N1], s32[:N1, :N1] = np.cos(a32), -np.sin(a32)
    nf = np.concatenate([c32, s32], axis=1)
    dfw = np.concatenate([np.concatenate([m0, m2], axis=1), np.concatenate([mp, mm], axis=1), nf], axis=0)
    dinv = np.concatenate([np.concatenate([m0i, m2.T * sc], axis=1),
                           np.concatenate([mp.T, mm.T], axis=1) * sc, nf], axis=0)
    rho = np.arange(N2)
    th = 2 * np.pi * np.outer(4 * (rho % 16) + rho // 16, rho) / N2
    c, s = np.cos(th), np.sin(th)
    mf = np.concatenate([np.concatenate([c, s], 1), np.concatenate([-s, c], 1)], 0)
    dfw = np.concatenate([dfw, np.concatenate([mf, mf.T], axis=1)], axis=0)
    dinv = np.concatenate([dinv, np.zeros((128, 256))], axis=0)
    dmat = _pack_rows(np.stack([dfw, dinv]))
    th = 2 * np.pi * np.arange(N1).reshape(4, 1, 8) * np.arange(N2).reshape(1, N2, 1) / S
    stw = np.broadcast_to(np.stack([np.cos(th), np.sin(th)], axis=2)[..., None], (4, N2, 2, 8, 128))
    stw = np.ascontiguousarray(stw, dtype=np.float32)
    head = np.concatenate([np.zeros(32), np.ones(32), np.zeros(8), np.ones(8)])
    pos = np.concatenate([np.arange(8), np.arange(16, 40)] * 2 + [np.arange(8, 16)] * 2)
    same = head[:, None] == head[None, :]
    ok = same & ((pos[:, None] < MEM) | (pos[:, None] >= pos[None, :]))
    misc = np.zeros((96 + 2 * N2, 128), np.float32)
    misc[:80, :80] = np.where(ok, 0.0, np.where(same, -1e9 * DH ** 0.5, -np.inf))
    atw = 2 * np.pi * np.outer(np.arange(N2), np.arange(128) % N1) / S
    misc[96:96 + N2], misc[96 + N2:] = np.cos(atw), np.sin(atw)
    return dmat, stw, misc


def _cmul(z, ang):
    re, im = z
    c, s = float(np.cos(ang)), float(np.sin(ang))
    if abs(s) < 1e-12:
        return (re, im) if c > 0 else (-re, -im)
    if abs(c) < 1e-12:
        return (-im, re) if s > 0 else (im, -re)
    if abs(abs(c) - abs(s)) < 1e-12:
        return ((re - im) * c, (re + im) * c) if c * s > 0 else ((re + im) * c, (im - re) * c)
    return re * c - im * s, re * s + im * c


def _fft(x, sign):
    n = len(x)
    if n == 1:
        return x
    if n == 2:
        (ar, ai), (br, bi) = x
        return [(ar + br, ai + bi), (ar - br, ai - bi)]
    ev, z1, z3 = _fft(x[0::2], sign), _fft(x[1::4], sign), _fft(x[3::4], sign)
    out = [None] * n
    q = n // 4
    for k in range(q):
        ar, ai = _cmul(z1[k], sign * 2 * np.pi * k / n)
        br, bi = _cmul(z3[k], sign * 2 * np.pi * 3 * k / n)
        sr, si, dr, di = ar + br, ai + bi, ar - br, ai - bi
        (er, ei), (fr, fi) = ev[k], ev[k + q]
        out[k] = (er + sr, ei + si)
        out[k + 2 * q] = (er - sr, ei - si)
        plus, minus = (fr - di, fi + dr), (fr + di, fi - dr)
        out[k + q], out[k + 3 * q] = (plus, minus) if sign > 0 else (minus, plus)
    return out


def _dot(a, b):
    return jnp.dot(a, b, preferred_element_type=F32)


def _bf(words):
    return pltpu.bitcast(words, BF)


def _f32(words):
    return pltpu.bitcast(words, F32)


def _u32(x):
    return pltpu.bitcast(x, U32)


def _rows8(off):
    return pl.ds(pl.multiple_of(off, 8), 8)


def _kernel(ax_h, wr_h, wi_h, bx_h, mem_h, wq_h, wk_h, wv_h, wo_h, dmat_h, stw_h, misc_h,
            o_h,
            wraw, pb, wtmp, w_s, wo_s, woraw, big, od_s, acc_s, x0raw, x0_s, xr_s, misc_s,
            ax_s, fraw, dmat_s, stw_s, oa_s, ob_s, mem_s,
            sem_w, sem_c, sem_m, sem_oa, sem_ob, sem_f):
    w_h = (wk_h, wq_h, wv_h)
    cp = pltpu.make_async_copy

    def w_copy(m, g):
        return cp(w_h[m].at[:, pl.ds(pl.multiple_of(8 * g, 8), 8), :], wraw.at[4 * m + g], sem_w.at[4 * m + g])

    def w_wait(t):
        cp(wraw.at[t], wraw.at[t], sem_w.at[t]).wait()

    def chunk_copies(i, which=(0, 1, 2, 3)):
        rows = pl.ds(pl.multiple_of(i * 512, 512), 512)
        cols = pl.ds(pl.multiple_of(i * 256, 256), 256)
        pairs = [lambda: (wo_h.at[rows], woraw.at[rows]),
                 lambda: (ax_h.at[:, _rows8(i * 8), :], ax_s.at[:, _rows8(i * 8), :]),
                 lambda: (wr_h.at[:, cols], fraw.at[0, :, cols]),
                 lambda: (wi_h.at[:, cols], fraw.at[1, :, cols])]
        return [cp(*pairs[k](), sem_c.at[i]) for k in which]

    def first_copies(kt):
        d = pl.ds(pl.multiple_of(kt * 128, 128), 128)
        return [cp(bx_h.at[:, pl.ds(0, 8), d], x0raw.at[kt], sem_f.at[kt]),
                cp(wk_h.at[d, pl.ds(0, 8), :], wraw.at[0, d], sem_f.at[kt])]

    early = [cp(dmat_h, dmat_s, sem_m.at[0]), cp(misc_h, misc_s, sem_m.at[1]), cp(mem_h, mem_s.at[0], sem_m.at[2])]
    late = [cp(bx_h.at[:, pl.ds(8, 24), :], xr_s, sem_m.at[3]), cp(stw_h, stw_s, sem_m.at[4])]

    def ob_copy(g):
        return cp(ob_s.at[_rows8(g * 8)], o_h.at[_rows8(g * 8), :, pl.ds(DM, DM)], sem_ob.at[g])

    def oa_copy(c):
        return cp(oa_s.at[:, _rows8(c * 8), :], o_h.at[:, _rows8(c * 8), pl.ds(0, DM)], sem_oa.at[c])

    lane = lax.broadcasted_iota(jnp.int32, (1, 128), 1)
    lane_lo = (lane & 1) == 0
    lane_plus = ((lane + 1) & 2) == 0
    lane_half = lane < 64
    rt = float(np.sqrt(0.5))

    order = [8 * a + b for b in range(8) for a in range(4)]

    def filt_prep(i, h, a):
        col = pl.ds(pl.multiple_of((2 * i + h) * 128, 128), 128)
        t = _u32(fraw[a, 0:256, col]).T
        for q in range(16):
            pb[_rows8(F_OFF + (a * 4 + q % 4) * 512 + ((2 * i + h) * 4 + q // 4) * 8), :] = t[q * 8:(q + 1) * 8]

    def ax_blocks(c):
        v = jnp.concatenate([ax_s[s1, _rows8(c * 8), :].astype(F32) for s1 in order], axis=0)
        return [v[:, i * 128:(i + 1) * 128] for i in range(4)]

    def t_rows(ka, b, part):
        return pl.ds(T_OFF + ((ka * 8 + b) * 2 + part) * 8, 8)

    def tf_rows(c, blk, ka, b, part):
        return _rows8(TF_OFF + (c % 2) * 32 + blk * 512 + ((ka * 8 + b) * 2 + part) * 8)

    def twiddles(c):
        return misc_s[_rows8(96 + c * 8), :], misc_s[_rows8(96 + N2 + c * 8), :]

    def fwd_even(c):
        x0, x1, x2, x3 = ax_blocks(c)
        p, q = x0 + x2, x1 + x3
        t0 = _dot((p + q).astype(BF), _bf(dmat_s[0, 0:64, 0:128]))
        t2 = _dot((p - q).astype(BF), _bf(dmat_s[0, 0:64, 128:256]))
        re = jnp.where(lane_lo, t0, t2)
        im = jnp.where(lane == 0, 0.0, pltpu.roll(jnp.where(lane_lo, t2, t0), 127, 1))
        n = jnp.zeros((8, 128), F32)
        for pos, s1 in enumerate(order):
            v = t0[pos * 8:(pos + 1) * 8]
            n = jnp.where(lane == s1, v if s1 == 1 else pltpu.roll(v, (s1 - 1) % 128, 1), n)
        return re, im, n

    def fwd_odd(c):
        x0, x1, x2, x3 = ax_blocks(c)
        a, b = x0 - x2, x1 - x3
        r = pltpu.roll(jnp.where(lane_half, b, (a - b) * rt), 64, 1)
        p, q = jnp.where(lane_half, a, r), jnp.where(lane_half, r, (a + b) * rt)
        tp = _dot((p + q).astype(BF), _bf(dmat_s[0, 64:128, 0:128]))
        tm = _dot((p - q).astype(BF), _bf(dmat_s[0, 64:128, 128:256]))
        return jnp.where(lane_plus, tp, tm), pltpu.roll(jnp.where(lane_plus, tm, tp), 126, 1)

    def fwd_pass1(c, blk, re, im):
        for b in range(8):
            z = _fft([(re[(b * 4 + a) * 8:(b * 4 + a + 1) * 8], im[(b * 4 + a) * 8:(b * 4 + a + 1) * 8])
                      for a in range(4)], -1)
            for ka in range(4):
                zr, zi = _cmul(z[ka], -2 * np.pi * b * ka / N1)
                pb[tf_rows(c, blk, ka, b, 0), :] = _u32(zr)
                pb[tf_rows(c, blk, ka, b, 1), :] = _u32(zi)

    def fwd_pass2(c, blk, ka):
        z = _fft([(_f32(pb[tf_rows(c, blk, ka, b, 0), :]), _f32(pb[tf_rows(c, blk, ka, b, 1), :]))
                  for b in range(8)], -1)
        for kb in range(8):
            k1 = ka + 4 * kb
            for part in range(2):
                row = U_OFF + (k1 // 8) * 2048 + (blk * 2 + part) * 512 + (k1 % 8) * 8
                pb[_rows8(row + c * 64), :] = _u32(z[kb][part])

    def fwd_nyq(c, n):
        u = _dot(n.astype(BF), _bf(dmat_s[0, 128:192, :]))
        ur, ui = u[:, 0:128], u[:, 128:256]
        ct, st = twiddles(c)
        return ur * ct + ui * st, ui * ct - ur * st

    def put_nyq(c, u):
        pb[_rows8(UN_OFF + c * 8), :] = _u32(u[0])
        pb[_rows8(UN_OFF + 64 + c * 8), :] = _u32(u[1])

    def cfilter(z, wr, wi):
        zr, zi = z[0:64], z[64:128]
        return jnp.concatenate([zr * wr - zi * wi, zr * wi + zi * wr], axis=0).astype(BF)

    def tm_rows(kc, r, part):
        return pl.ds(TF_OFF + ((kc * 8 + r) * 2 + part) * 8, 8)

    def tm_get(kc, r):
        return _f32(pb[tm_rows(kc, r, 0), :]), _f32(pb[tm_rows(kc, r, 1), :])

    def tm_put(kc, r, z):
        pb[tm_rows(kc, r, 0), :] = _u32(z[0])
        pb[tm_rows(kc, r, 1), :] = _u32(z[1])

    def mid_1(g, blk, r):
        view = pb.at[pl.ds(pl.multiple_of(U_OFF + g * 2048, 32), 2048 + 8)]
        x = []
        for c in range(8):
            re, im = [_f32(view[pl.ds((blk * 2 + part) * 512 + c * 64 + r, 8, stride=8), :]) for part in range(2)]
            if 8 * c + r:
                ct, st = stw_s[g, 8 * c + r, 0], stw_s[g, 8 * c + r, 1]
                re, im = re * ct + im * st, im * ct - re * st
            x.append((re, im))
        z = _fft(x, -1)
        for kc in range(8):
            tm_put(kc, r, _cmul(z[kc], -2 * np.pi * r * kc / N2))

    def mid_2(g, blk, kc):
        z = _fft([tm_get(kc, r) for r in range(8)], -1)
        y = []
        for kr in range(8):
            w = [pb[pl.ds(pl.multiple_of(g * 512, 32) + (F_OFF + a * 2048 + (kc + 8 * kr) * 8), 8), :]
                 for a in range(2)]
            wr, wi = [_f32(v & jnp.uint32(HI_MASK)) if blk else _f32(v << 16) for v in w]
            zr, zi = z[kr]
            y.append((zr * wr - zi * wi, zr * wi + zi * wr))
        v = _fft(y, 1)
        for r in range(8):
            tm_put(kc, r, _cmul(v[r], 2 * np.pi * r * kc / N2))

    def mid_3(g, blk, r):
        z = _fft([tm_get(kc, r) for kc in range(8)], 1)
        for c in range(8):
            re, im = z[c]
            if 8 * c + r:
                ct, st = stw_s[g, 8 * c + r, 0], stw_s[g, 8 * c + r, 1]
                re, im = re * ct - im * st, im * ct + re * st
            for part, v in enumerate((re, im)):
                row = V_OFF + c * 1024 + (blk * 2 + part) * 256 + r * 8
                big[pl.ds(pl.multiple_of(g * 64, 32) + row, 8), :] = v

    def nyq_a():
        z = _dot(_bf(dmat_s[0, 192:256, 0:128]), _f32(pb[pl.ds(UN_OFF, 128), :]).astype(BF))
        w = []
        for a in range(2):
            g = jnp.concatenate([fraw[a, 256:257, t * 128:(t + 1) * 128].astype(F32) for t in range(16)], axis=0)
            w.append(jnp.concatenate([g] + [pltpu.roll(g, 128 - 32 * q, 1) for q in range(1, 4)], axis=0))
        return cfilter(z, *w)

    def nyq_b(y):
        big[pl.ds(VN_OFF, 128), :] = _dot(_bf(dmat_s[0, 192:256, 128:256]), y)

    def inv_pass1(c, blk, ka):
        view = big.at[pl.ds(pl.multiple_of(V_OFF + c * 1024, 32), 1024 + 8)]
        z = _fft([tuple(view[pl.ds((blk * 2 + part) * 256 + (k1 // 8) * 64 + k1 % 8, 8, stride=8), :]
                        for part in range(2)) for k1 in range(ka, N1, 4)], 1)
        for b in range(8):
            zr, zi = _cmul(z[b], 2 * np.pi * b * ka / N1)
            big[t_rows(ka, b, 0), :] = zr
            big[t_rows(ka, b, 1), :] = zi

    def inv_nyq(c):
        vr, vi = big[_rows8(VN_OFF + c * 8), :], big[_rows8(VN_OFF + 64 + c * 8), :]
        ct, st = twiddles(c)
        m = _bf(dmat_s[1, 128:192, :])
        return (_dot((vr * ct - vi * st).astype(BF), m[:, 0:128])
                + _dot((vi * ct + vr * st).astype(BF), m[:, 128:256]))

    def inv_pass2(blk, b, n):
        z = _fft([(big[t_rows(ka, b, 0), :], big[t_rows(ka, b, 1), :]) for ka in range(4)], 1)
        for a in range(4):
            re, im = z[a]
            s1 = 8 * a + b
            if blk == 0:
                im = pltpu.roll(im, 1, 1)
                nv = n if s1 == 1 else pltpu.roll(n, (1 - s1) % 128, 1)
                re, im = jnp.where(lane == 1, nv, jnp.where(lane_lo, re, im)), jnp.where(lane_lo, im, re)
            else:
                im = pltpu.roll(im, 2, 1)
                re, im = jnp.where(lane_plus, re, im), jnp.where(lane_plus, im, re)
            big[pl.ds(L_OFF + (2 * blk) * 256 + s1 * 8, 8), :] = re
            big[pl.ds(L_OFF + (2 * blk + 1) * 256 + s1 * 8, 8), :] = im

    def inv_out(c):
        lhs = [big[pl.ds(L_OFF + i * 256, 256), :] for i in range(4)]
        c0 = _dot(lhs[0].astype(BF), _bf(dmat_s[1, 0:64, 0:128]))
        c2 = _dot(lhs[1].astype(BF), _bf(dmat_s[1, 0:64, 128:256]))
        lp = _dot(lhs[2].astype(BF), _bf(dmat_s[1, 64:128, 0:128]))
        lm = _dot(lhs[3].astype(BF), _bf(dmat_s[1, 64:128, 128:256]))
        pp, qq = lp + lm, lp - lm
        r = pltpu.roll(jnp.where(lane_half, qq, pp), 64, 1)
        p, q = jnp.where(lane_half, pp, (r + qq) * rt), jnp.where(lane_half, r, (qq - r) * rt)
        e, f = c0 + c2, c0 - c2
        y = jnp.concatenate([e + p, f + q, e - p, f - q], axis=1)
        oa_s[:, _rows8(c * 8), :] = y.reshape(N1, 8, DM).astype(BF)

    def head_words(hh, n):
        a = wtmp[pl.ds(hh // 2, n, stride=8), :]
        b = wtmp[pl.ds(4 + hh // 2, n, stride=8), :]
        return (a >> 16) | (b & jnp.uint32(HI_MASK)) if hh % 2 else (a & 0xFFFF) | (b << 16)

    def head_weights(t, hh):
        w = head_words(hh, 256)
        w_s[t * 8 + hh] = w
        return w

    def stage_chunk(t):
        for dc in range(8):
            wtmp[dc * 256:(dc + 1) * 256, :] = _u32(wraw[t, dc * 64:(dc + 1) * 64].reshape(512, 128))
        head_weights(t, 0)

    def early_proj(t, hooks):
        for jj in range(4):
            res = []
            for hh in (2 * jj, 2 * jj + 1):
                w = w_s[t * 8] if hh == 0 else head_weights(t, hh)
                r = _dot(_bf(jnp.concatenate([x0_s[k] for k in range(4)], axis=1)), _bf(w))
                res.append(r.reshape(NSEG, 8, 128))
                for tm, f, pinned in hooks:
                    if tm // 8 == hh:
                        if pinned:
                            pb[_rows8(TK_OFF + (t % 2) * 32), :] = _u32(r[(tm % 8) * 64:(tm % 8) * 64 + 8])
                        f()
            big[pl.ds(pl.multiple_of(P_OFF + (t * 4 + jj) * 1024, 1024), 1024), :] = (
                jnp.concatenate(res, axis=1).reshape(1024, 128))

    def phase_0(kt, carry):
        for c in first_copies(kt):
            c.wait()
        for dc in range(2):
            v = wraw[0, pl.ds(pl.multiple_of(kt * 128 + dc * 64, 64), 64)]
            wtmp[dc * 256:(dc + 1) * 256, :] = _u32(v.reshape(512, 128))
        xk = _u32(x0raw[kt].reshape(NSEG * 8, 128))
        x0_s[kt] = xk
        for jj in range(4):
            res = []
            for hh in (2 * jj, 2 * jj + 1):
                w = head_words(hh, 64)
                w_s[hh, pl.ds(pl.multiple_of(kt * 64, 64), 64), :] = w
                res.append(_dot(_bf(xk), _bf(w)).reshape(NSEG, 8, 128))
            rows = pl.ds(P_OFF + jj * 1024, 1024)
            big[rows, :] = jnp.where(kt > 0, big[rows, :], 0.0) + jnp.concatenate(res, axis=1).reshape(1024, 128)
        return carry

    def phase_a(t, carry):
        @pl.when(t <= 2)
        def _():
            w_wait(t)
            w_copy(1, t).start()
            for c in chunk_copies(t):
                c.start()
            stage_chunk(t)

        @pl.when(t >= 2)
        def _():
            w_wait(t + 1)

        early_proj(t, [])
        stage_chunk(jnp.where(t >= 2, t + 1, t))
        return carry

    def phase_b(i, carry):
        t = i + 3

        @pl.when(i < 4)
        def _():
            for c in [w_copy(2, i)] + chunk_copies(i + 4, (0,)):
                c.start()

        w_wait(t + 1)
        for c in chunk_copies(i):
            c.wait()

        @pl.when(i < 4)
        def _():
            for c in chunk_copies(i + 4, (1, 2, 3)):
                c.start()

        @pl.when(i == 4)
        def _():
            for c in late:
                c.start()

        def wo_retile(n):
            wo_s[n * 8 + i] = _u32(woraw[pl.ds(pl.multiple_of(i * 512, 512), 512), n * 128:(n + 1) * 128])

        box = {}
        t_om, t_f, t_o1, t_o2, t_em, t_e1, t_n, t_e2, t_pn, dt = SCHED_PB
        hooks = [(t_f + dt * k, lambda k=k: filt_prep(i, k // 2, k % 2), False) for k in range(4)]
        hooks += [(t_om, lambda: box.update(o=fwd_odd(i)), False),
                  (t_o1, lambda: fwd_pass1(i, 1, *box["o"]), False),
                  (t_em, lambda: box.update(e=fwd_even(i)), False),
                  (t_e1, lambda: fwd_pass1(i, 0, *box["e"][:2]), False),
                  (t_n, lambda: box.update(n=fwd_nyq(i, box["e"][2])), False),
                  (t_pn, lambda: put_nyq(i, box["n"]), False)]
        hooks += [(t_o2 + dt * ka, lambda ka=ka: fwd_pass2(i, 1, ka), True) for ka in range(4)]
        hooks += [(t_e2 + dt * ka, lambda ka=ka: fwd_pass2(i, 0, ka), True) for ka in range(4)]
        hooks += [(0, lambda n=n: wo_retile(n), False) for n in range(4)]
        early_proj(t, sorted(hooks, key=lambda h: h[0]))
        stage_chunk(jnp.minimum(t + 1, 11))
        return carry

    def x0_rows(r0, n):
        return _bf(jnp.concatenate([x0_s[k, r0 // 2:(r0 + n) // 2, :] for k in range(4)], axis=1))

    def phase_c():
        pb[TK_OFF:TK_OFF + 64, :] = jnp.zeros((64, 128), U32)
        for jj in range(4):
            res = []
            for hh in (2 * jj, 2 * jj + 1):
                w = w_s[88] if hh == 0 else head_weights(11, hh)
                res.append(_dot(x0_rows(0, 128), _bf(w)).reshape(16, 8, 128))
                if hh == 0:
                    y = nyq_a()
                if hh == 5:
                    nyq_b(y)
            big[pl.ds(P_OFF + (44 + jj) * 1024, 256), :] = jnp.concatenate(res, axis=1).reshape(256, 128)

    def early_rest(i, u):
        r = _dot(x0_rows(128 + 192 * (u % 2), 192), _bf(w_s[88 + 2 * i + u // 2]))
        for q in range(24):
            row = P_OFF + 44 * 1024 + (16 + 24 * (u % 2) + q) * 16 + (u // 2) * 8
            big[pl.ds(pl.multiple_of(i * 1024, 32) + row, 8), :] = r[q * 8:(q + 1) * 8]

    def wo_rows(j):
        r = pl.ds(pl.multiple_of((j & 1) * 128, 128), 128)
        return _bf(jnp.concatenate([wo_s[n * 8 + (j >> 1), r, :] for n in range(4)], axis=1))

    def put_late(g, res):
        for i in range(16):
            ob_s[g * 8 + i // 2, (i % 2) * 32:(i % 2) * 32 + 8, :] = res[i * 8:(i + 1) * 8].astype(BF)

    def late_proj(idx):
        g, c = idx >> 4, idx & 15
        a = od_s[c, pl.ds(pl.multiple_of(g * 128, 128), 128), :].astype(BF)
        res = jnp.where(c > 0, acc_s[...], 0.0) + _dot(a, wo_rows(c))
        acc_s[...] = res
        put_late(g, res)

    def step(s0, u0, mem, hooks, lags):
        s = s0 + u0
        qk_lag, pv_lag, skew = lags // 100, lags // 10 % 10, lags % 10
        lhs = jnp.concatenate([mem, xr_s[s].astype(F32)], axis=0).astype(BF)
        st = {}

        def proj(mi, j):
            w1 = w_s[mi * H + 2 * j]
            if "gate" in st:
                w1 = jnp.concatenate([w1[0:248], w1[248:256] | st.pop("gate")], axis=0)
            y1 = _dot(lhs, _bf(w1))
            y2 = _dot(lhs, _bf(w_s[mi * H + 2 * j + 1]))
            pre = big[pl.ds(pl.multiple_of(s0 * 16, 32) + (P_OFF + (mi * NP + j) * 1024 + u0 * 16), 16), :]
            st[mi, j] = jnp.concatenate([y1, y2, pre], axis=0).astype(BF)
            st["last"] = y1[0:8]

        def pin():
            big[pl.ds(pl.multiple_of((s0 & 2) * 16, 32) + X_OFF, 8), :] = st["last"]

        def gate():
            st["gate"] = pb[pl.ds(pl.multiple_of((s0 % 8) * 8, 32) + (TK_OFF + 8), 8), :]

        def pin_pb():
            pb[pl.ds(pl.multiple_of((s0 % 8) * 8, 32) + TK_OFF, 8), :] = _u32(st["last"])

        def qk(j):
            sc = lax.dot_general(st.pop((1, j)), st.pop((0, j)), (((1,), (1,)), ((), ())),
                                 preferred_element_type=F32)
            fill = misc_s[0:80, 0:80]
            sc = jnp.where(fill == 0.0, sc, fill)
            p = jnp.exp2((sc - jnp.max(sc, axis=1, keepdims=True)) * EXP_C)
            st["p", j] = (p.astype(BF), pl.reciprocal(jnp.sum(p, axis=1, keepdims=True), approx=True))

        def pv(j):
            p, rl = st.pop(("p", j))
            o = _dot(p, st.pop((2, j))) * rl
            st["o", j] = jnp.concatenate([o[0:32], o[32:64]], axis=1).astype(BF)
            od_s[j, pl.ds(pl.multiple_of(s0 * 8, 16) + u0 * 8, 8), :] = jnp.concatenate([o[64:72], o[72:80]], axis=1)

        def op(j):
            r = _dot(st.pop(("o", j)), wo_rows(j))
            st["acc"] = r if "acc" not in st else st["acc"] + r

        units = []
        for j in range(-skew, NP):
            units += [(mi, j + skew) for mi in (0, 1) if j + skew < NP] + ([(2, j)] if j >= 0 else [])
        events = [(t, lambda mi=mi, j=j: proj(mi, j)) for t, (mi, j) in enumerate(units)]
        events += [(3 * NP + j, lambda j=j: op(j)) for j in range(NP)]
        for j in range(NP):
            tqk = units.index((1, j)) + 1 + qk_lag
            events.append((tqk - 0.5, lambda j=j: qk(j)))
            events.append((max(tqk + pv_lag, units.index((2, j)) + 1 + qk_lag) - 0.4, lambda j=j: pv(j)))
        for t, fs in hooks.items():
            events += [(t - 0.3, {None: pin, "pb": pin_pb, "gate": gate}.get(f, f)) for f in fs]
        for _, f in sorted(events, key=lambda ev: ev[0]):
            f()
        out = st["acc"]
        ob_s[(s0 >> 1) + u0 // 2, (u0 % 2) * 32 + 8:(u0 % 2) * 32 + 32, :] = out[8:32].astype(BF)
        return out[0:8].astype(BF).astype(F32)

    def loop_a(i, mem):
        jobs = [{} for _ in range(4)]
        t_0, dt, t_g, nps, t_x = SCHED_LA

        def add(t, fs):
            u = min(t // 64, 3)
            jobs[u].setdefault(t - 64 * u, []).extend(fs)

        pieces = [(f, blk, k) for blk in range(2) for f in (mid_1, mid_2, mid_3) for k in range(8)]
        for n, (f, blk, k) in enumerate(pieces):
            add(64 * (n // nps) + t_0 + dt * (n % nps), ["pb", lambda f=f, blk=blk, k=k: f(i, blk, k)])
        add(192 + t_g, ["gate"])
        for u, t in enumerate(sorted([64, 128, 192, t_x])):
            add(t, [lambda u=u: early_rest(i, u)])
        for u in range(4):
            mem = step(4 * i, u, mem, jobs[u], STEP_A[u])
        return mem

    def loop_b(i, mem):
        box = {}
        jobs = [{} for _ in range(6)]
        t1, d1, t2, d2, t_n, t_o, t_x = SCHED_LB

        def add(t, fs):
            u = min(t // 64, 5)
            jobs[u].setdefault(t - 64 * u, []).extend(fs)

        for blk in range(2):
            for ka in range(4):
                add(128 * blk + t1 + d1 * ka, [None, lambda blk=blk, ka=ka: inv_pass1(i, blk, ka)])
            for b in range(8):
                add(128 * blk + 64 + t2 + d2 * b, [None, lambda blk=blk, b=b: inv_pass2(blk, b, box["n"])])
        add(t_n, [lambda: box.update(n=inv_nyq(i))])
        add(t_o, [lambda: inv_out(i)])
        for u, t in enumerate(sorted([64 * u for u in range(1, 6)] + [t_x])):
            add(t, [lambda u=u: late_proj(6 * i + u)])
        for u in range(6):
            mem = step(6 * i, 16 + u, mem, jobs[u], STEP_B[u])
        oa_copy(i).start()

        @pl.when((i == 2) | (i == 5))
        def _():
            ob_copy(i >> 2).start()

        return mem

    for kt in range(4):
        for c in first_copies(kt):
            c.start()
    for g in range(1, 4):
        w_copy(0, g).start()
    lax.fori_loop(0, 4, phase_0, 0)
    w_copy(1, 0).start()
    for c in early + chunk_copies(0):
        c.start()
    lax.fori_loop(1, 3, phase_a, 0)
    w_copy(1, 3).start()
    for c in chunk_copies(3):
        c.start()
    for c in early:
        c.wait()
    lax.fori_loop(0, 8, phase_b, 0)
    phase_c()
    for c in late:
        c.wait()
    mem = mem_s[0].astype(F32)
    mem = lax.fori_loop(0, 4, loop_a, mem)
    lax.fori_loop(0, 8, loop_b, mem)
    ob_copy(2).start()
    last = [cp(ob_s.at[pl.ds(24, 8), pl.ds(r, n), :], o_h.at[pl.ds(24, 8), pl.ds(r, n), pl.ds(DM, DM)],
               sem_ob.at[3 + k]) for k, (r, n) in enumerate([(8, 24), (40, 24), (0, 8), (32, 8)])]
    last[0].start()
    last[1].start()
    a = jnp.concatenate([od_s[c, 384:512, :] for c in range(NP)], axis=1).astype(BF)
    put_late(3, _dot(a, jnp.concatenate([wo_rows(j) for j in range(NP)], axis=0)))
    last[2].start()
    last[3].start()
    for c in range(8):
        oa_copy(c).wait()
    for g in range(3):
        ob_copy(g).wait()
    for c in last:
        c.wait()


def _compiler_params():
    base = dict(vmem_limit_bytes=120 * 1024 * 1024, disable_bounds_checks=True)
    try:
        return pltpu.CompilerParams(disable_semaphore_checks=True, **base)
    except TypeError:
        return pltpu.CompilerParams(**base)


@jax.jit
def pallas_concat_heads__spectral_gfnet__memory_aug_recurrent_mem_tr__prompt_kernel(
        A_x, A_w_r, A_w_i, B_x, B_mem0, B_Wq, B_Wk, B_Wv, B_Wo, B_seg_len=None):
    dmat, stw, misc = _consts()
    vm, dma = pltpu.VMEM, pltpu.SemaphoreType.DMA
    out = pl.pallas_call(
        _kernel,
        out_shape=jax.ShapeDtypeStruct((N1, N2, 2 * DM), BF),
        in_specs=[pl.BlockSpec(memory_space=pl.ANY)] * 12,
        out_specs=pl.BlockSpec(memory_space=pl.ANY),
        scratch_shapes=[
            vm((12, DM, 8, DH), BF), vm((PB_ROWS, 128), U32), vm((2048 + 32, 128), U32),
            vm((3 * H, DM // 2, DH), U32), vm((H, DM // 2, DH), U32), vm((H * DH, DM), BF),
            vm((BIG_ROWS, 128), F32), vm((NP, NSEG * 8, 2 * DH), F32), vm((128, DM), F32),
            vm((4, NSEG, 8, 128), BF), vm((4, NSEG * 4, 128), U32), vm((NSEG, 24, DM), BF),
            vm(misc.shape, F32),
            vm((N1, N2, DM), BF), vm((2, DM // 2 + 1, S), BF), vm(dmat.shape, U32), vm(stw.shape, F32),
            vm((N1, N2, DM), BF), vm((N1, N2, DM), BF), vm((2, MEM, DM), BF),
            dma((12,)), dma((8,)), dma((5,)), dma((8,)), dma((7,)), dma((4,)),
        ],
        compiler_params=_compiler_params(),
    )(A_x.reshape(N1, N2, DM), A_w_r.T, A_w_i.T,
      B_x.reshape(NSEG, SEG, DM), B_mem0.reshape(MEM, DM), B_Wq, B_Wk, B_Wv, B_Wo.reshape(H * DH, DM),
      jnp.asarray(dmat), jnp.asarray(stw), jnp.asarray(misc))
    return out.reshape(1, S, 2 * DM)
```

```python
import numpy as np
import jax
import jax.numpy as jnp
from jax import lax
import jax.experimental.pallas as pl
import jax.experimental.pallas.tpu as pltpu

S, DM, H, DH, MEM, SEG = 2048, 512, 32, 128, 8, 32
NSEG = S // SEG
NP = H // 2
N1, N2 = 32, 64
BF, F32, U32 = jnp.bfloat16, jnp.float32, jnp.uint32
EXP_C = float(DH ** -0.5 * np.log2(np.e))
HI_MASK = 0xFFFF0000

P_OFF = 0
T_OFF = P_OFF + 3 * NP * NSEG * 16
L_OFF = T_OFF + 64 * 8
V_OFF = L_OFF + 4 * 256
VN_OFF = V_OFF + 8192
X_OFF = VN_OFF + 128
BIG_ROWS = X_OFF + 64
TK_OFF = 0
TF_OFF = TK_OFF + 64
F_OFF = TF_OFF + 2 * 512 + 32
U_OFF = F_OFF + 8 * 512
UN_OFF = U_OFF + 8192
PB_ROWS = UN_OFF + 128

STEP_A = (361, 361, 361, 361)
STEP_B = (361, 361, 361, 361, 361, 361)
SCHED_PB = (0, 40, 16, 29, 0, 16, 17, 23, 33, 1)
SCHED_LA = (3, 2, 32, 13, 0)
SCHED_LB = (3, 6, 11, 3, 29, 267, 0)


def _pack_rows(m):
    f = np.ascontiguousarray(m, dtype=np.float32).view(np.uint32)
    r = ((f + 0x7FFF + ((f >> 16) & 1)) >> 16).astype(np.uint32)
    return r[..., 0::2, :] | (r[..., 1::2, :] << 16)


def _consts():
    l = np.arange(128)
    d2 = np.arange(128)[:, None]
    lo = (l % 2) == 0
    a_re = 2 * np.pi * d2 * (2 * l)[None, :] / DM
    a_im = 2 * np.pi * d2 * (2 * ((l - 1) % 128))[None, :] / DM
    m0 = np.where(lo[None, :], np.cos(a_re), -np.sin(a_im))
    m0[:, 1] = (-1.0) ** np.arange(128)
    m2 = np.where(lo[None, :], -np.sin(a_im), np.cos(a_re))
    e = np.arange(64)[:, None]

    def odd_cols(lanes):
        kd = 2 * lanes + 1
        ang = 2 * np.pi * e * kd[None, :] / DM
        sg = np.where(kd % 4 == 1, 1.0, -1.0)[None, :]
        return (np.concatenate([np.cos(ang), -sg * np.sin(ang)], axis=0),
                np.concatenate([-np.sin(ang), -sg * np.cos(ang)], axis=0))

    plus = (l % 4 == 0) | (l % 4 == 3)
    o_re, o_im = odd_cols(l)[0], odd_cols((l - 2) % 128)[1]
    mp = np.where(plus[None, :], o_re, o_im)
    mm = np.where(plus[None, :], o_im, o_re)
    sc = 2.0 / (S * DM)
    m0i = m0.T * sc
    m0i[0] /= 2
    m0i[1] /= 2
    a32 = 2 * np.pi * np.outer(np.arange(N1), np.arange(N1)) / N1
    c32, s32 = np.zeros((128, 128)), np.zeros((128, 128))
    c32[:N1, :N1], s32[:N1, :N1] = np.cos(a32), -np.sin(a32)
    nf = np.concatenate([c32, s32], axis=1)
    dfw = np.concatenate([np.concatenate([m0, m2], axis=1), np.concatenate([mp, mm], axis=1), nf], axis=0)
    dinv = np.concatenate([np.concatenate([m0i, m2.T * sc], axis=1),
                           np.concatenate([mp.T, mm.T], axis=1) * sc, nf], axis=0)
    rho = np.arange(N2)
    th = 2 * np.pi * np.outer(4 * (rho % 16) + rho // 16, rho) / N2
    c, s = np.cos(th), np.sin(th)
    mf = np.concatenate([np.concatenate([c, s], 1), np.concatenate([-s, c], 1)], 0)
    dfw = np.concatenate([dfw, np.concatenate([mf, mf.T], axis=1)], axis=0)
    dinv = np.concatenate([dinv, np.zeros((128, 256))], axis=0)
    dmat = _pack_rows(np.stack([dfw, dinv]))
    th = 2 * np.pi * np.arange(N1).reshape(4, 1, 8) * np.arange(N2).reshape(1, N2, 1) / S
    stw = np.broadcast_to(np.stack([np.cos(th), np.sin(th)], axis=2)[..., None], (4, N2, 2, 8, 128))
    stw = np.ascontiguousarray(stw, dtype=np.float32)
    head = np.concatenate([np.zeros(32), np.ones(32), np.zeros(8), np.ones(8)])
    pos = np.concatenate([np.arange(8), np.arange(16, 40)] * 2 + [np.arange(8, 16)] * 2)
    same = head[:, None] == head[None, :]
    ok = same & ((pos[:, None] < MEM) | (pos[:, None] >= pos[None, :]))
    misc = np.zeros((96 + 2 * N2, 128), np.float32)
    misc[:80, :80] = np.where(ok, 0.0, np.where(same, -1e9 * DH ** 0.5, -np.inf))
    atw = 2 * np.pi * np.outer(np.arange(N2), np.arange(128) % N1) / S
    misc[96:96 + N2], misc[96 + N2:] = np.cos(atw), np.sin(atw)
    return dmat, stw, misc


def _cmul(z, ang):
    re, im = z
    c, s = float(np.cos(ang)), float(np.sin(ang))
    if abs(s) < 1e-12:
        return (re, im) if c > 0 else (-re, -im)
    if abs(c) < 1e-12:
        return (-im, re) if s > 0 else (im, -re)
    if abs(abs(c) - abs(s)) < 1e-12:
        return ((re - im) * c, (re + im) * c) if c * s > 0 else ((re + im) * c, (im - re) * c)
    return re * c - im * s, re * s + im * c


def _fft(x, sign):
    n = len(x)
    if n == 1:
        return x
    if n == 2:
        (ar, ai), (br, bi) = x
        return [(ar + br, ai + bi), (ar - br, ai - bi)]
    ev, z1, z3 = _fft(x[0::2], sign), _fft(x[1::4], sign), _fft(x[3::4], sign)
    out = [None] * n
    q = n // 4
    for k in range(q):
        ar, ai = _cmul(z1[k], sign * 2 * np.pi * k / n)
        br, bi = _cmul(z3[k], sign * 2 * np.pi * 3 * k / n)
        sr, si, dr, di = ar + br, ai + bi, ar - br, ai - bi
        (er, ei), (fr, fi) = ev[k], ev[k + q]
        out[k] = (er + sr, ei + si)
        out[k + 2 * q] = (er - sr, ei - si)
        plus, minus = (fr - di, fi + dr), (fr + di, fi - dr)
        out[k + q], out[k + 3 * q] = (plus, minus) if sign > 0 else (minus, plus)
    return out


def _dot(a, b):
    return jnp.dot(a, b, preferred_element_type=F32)


def _bf(words):
    return pltpu.bitcast(words, BF)


def _f32(words):
    return pltpu.bitcast(words, F32)


def _u32(x):
    return pltpu.bitcast(x, U32)


def _rows8(off):
    return pl.ds(pl.multiple_of(off, 8), 8)


def _kernel(ax_h, wr_h, wi_h, bx_h, mem_h, wq_h, wk_h, wv_h, wo_h, dmat_h, stw_h, misc_h,
            o_h,
            wraw, pb, wtmp, w_s, wo_s, woraw, big, od_s, acc_s, x0raw, x0_s, xr_s, misc_s,
            ax_s, fraw, dmat_s, stw_s, oa_s, ob_s, mem_s,
            sem_w, sem_c, sem_m, sem_oa, sem_ob, sem_f):
    w_h = (wk_h, wq_h, wv_h)
    cp = pltpu.make_async_copy

    def w_copy(m, g):
        return cp(w_h[m].at[:, pl.ds(pl.multiple_of(8 * g, 8), 8), :], wraw.at[4 * m + g], sem_w.at[4 * m + g])

    def w_wait(t):
        cp(wraw.at[t], wraw.at[t], sem_w.at[t]).wait()

    def chunk_copies(i, which=(0, 1, 2, 3)):
        rows = pl.ds(pl.multiple_of(i * 512, 512), 512)
        cols = pl.ds(pl.multiple_of(i * 256, 256), 256)
        pairs = [lambda: (wo_h.at[rows], woraw.at[rows]),
                 lambda: (ax_h.at[:, _rows8(i * 8), :], ax_s.at[:, _rows8(i * 8), :]),
                 lambda: (wr_h.at[:, cols], fraw.at[0, :, cols]),
                 lambda: (wi_h.at[:, cols], fraw.at[1, :, cols])]
        return [cp(*pairs[k](), sem_c.at[i]) for k in which]

    def first_copies(kt):
        d = pl.ds(pl.multiple_of(kt * 128, 128), 128)
        return [cp(bx_h.at[:, pl.ds(0, 8), d], x0raw.at[kt], sem_f.at[kt]),
                cp(wk_h.at[d, pl.ds(0, 8), :], wraw.at[0, d], sem_f.at[kt])]

    early = [cp(dmat_h, dmat_s, sem_m.at[0]), cp(misc_h, misc_s, sem_m.at[1]), cp(mem_h, mem_s.at[0], sem_m.at[2])]
    late = [cp(bx_h.at[:, pl.ds(8, 24), :], xr_s, sem_m.at[3]), cp(stw_h, stw_s, sem_m.at[4])]

    def ob_copy(g):
        return cp(ob_s.at[_rows8(g * 8)], o_h.at[_rows8(g * 8), :, pl.ds(DM, DM)], sem_ob.at[g])

    def oa_copy(c):
        return cp(oa_s.at[:, _rows8(c * 8), :], o_h.at[:, _rows8(c * 8), pl.ds(0, DM)], sem_oa.at[c])

    lane = lax.broadcasted_iota(jnp.int32, (1, 128), 1)
    lane_lo = (lane & 1) == 0
    lane_plus = ((lane + 1) & 2) == 0
    lane_half = lane < 64
    rt = float(np.sqrt(0.5))

    order = [8 * a + b for b in range(8) for a in range(4)]

    def filt_prep(i, h, a):
        col = pl.ds(pl.multiple_of((2 * i + h) * 128, 128), 128)
        t = _u32(fraw[a, 0:256, col]).T
        for q in range(16):
            pb[_rows8(F_OFF + (a * 4 + q % 4) * 512 + ((2 * i + h) * 4 + q // 4) * 8), :] = t[q * 8:(q + 1) * 8]

    def ax_blocks(c):
        v = jnp.concatenate([ax_s[s1, _rows8(c * 8), :].astype(F32) for s1 in order], axis=0)
        return [v[:, i * 128:(i + 1) * 128] for i in range(4)]

    def t_rows(ka, b, part):
        return pl.ds(T_OFF + ((ka * 8 + b) * 2 + part) * 8, 8)

    def tf_rows(c, blk, ka, b, part):
        return _rows8(TF_OFF + (c % 2) * 32 + blk * 512 + ((ka * 8 + b) * 2 + part) * 8)

    def twiddles(c):
        return misc_s[_rows8(96 + c * 8), :], misc_s[_rows8(96 + N2 + c * 8), :]

    def fwd_even(c):
        x0, x1, x2, x3 = ax_blocks(c)
        p, q = x0 + x2, x1 + x3
        t0 = _dot((p + q).astype(BF), _bf(dmat_s[0, 0:64, 0:128]))
        t2 = _dot((p - q).astype(BF), _bf(dmat_s[0, 0:64, 128:256]))
        re = jnp.where(lane_lo, t0, t2)
        im = jnp.where(lane == 0, 0.0, pltpu.roll(jnp.where(lane_lo, t2, t0), 127, 1))
        n = jnp.zeros((8, 128), F32)
        for pos, s1 in enumerate(order):
            v = t0[pos * 8:(pos + 1) * 8]
            n = jnp.where(lane == s1, v if s1 == 1 else pltpu.roll(v, (s1 - 1) % 128, 1), n)
        return re, im, n

    def fwd_odd(c):
        x0, x1, x2, x3 = ax_blocks(c)
        a, b = x0 - x2, x1 - x3
        r = pltpu.roll(jnp.where(lane_half, b, (a - b) * rt), 64, 1)
        p, q = jnp.where(lane_half, a, r), jnp.where(lane_half, r, (a + b) * rt)
        tp = _dot((p + q).astype(BF), _bf(dmat_s[0, 64:128, 0:128]))
        tm = _dot((p - q).astype(BF), _bf(dmat_s[0, 64:128, 128:256]))
        return jnp.where(lane_plus, tp, tm), pltpu.roll(jnp.where(lane_plus, tm, tp), 126, 1)

    def fwd_pass1(c, blk, re, im):
        for b in range(8):
            z = _fft([(re[(b * 4 + a) * 8:(b * 4 + a + 1) * 8], im[(b * 4 + a) * 8:(b * 4 + a + 1) * 8])
                      for a in range(4)], -1)
            for ka in range(4):
                zr, zi = _cmul(z[ka], -2 * np.pi * b * ka / N1)
                pb[tf_rows(c, blk, ka, b, 0), :] = _u32(zr)
                pb[tf_rows(c, blk, ka, b, 1), :] = _u32(zi)

    def fwd_pass2(c, blk, ka):
        z = _fft([(_f32(pb[tf_rows(c, blk, ka, b, 0), :]), _f32(pb[tf_rows(c, blk, ka, b, 1), :]))
                  for b in range(8)], -1)
        for kb in range(8):
            k1 = ka + 4 * kb
            for part in range(2):
                row = U_OFF + (k1 // 8) * 2048 + (blk * 2 + part) * 512 + (k1 % 8) * 8
                pb[_rows8(row + c * 64), :] = _u32(z[kb][part])

    def fwd_nyq(c, n):
        u = _dot(n.astype(BF), _bf(dmat_s[0, 128:192, :]))
        ur, ui = u[:, 0:128], u[:, 128:256]
        ct, st = twiddles(c)
        return ur * ct + ui * st, ui * ct - ur * st

    def put_nyq(c, u):
        pb[_rows8(UN_OFF + c * 8), :] = _u32(u[0])
        pb[_rows8(UN_OFF + 64 + c * 8), :] = _u32(u[1])

    def cfilter(z, wr, wi):
        zr, zi = z[0:64], z[64:128]
        return jnp.concatenate([zr * wr - zi * wi, zr * wi + zi * wr], axis=0).astype(BF)

    def tm_rows(kc, r, part):
        return pl.ds(TF_OFF + ((kc * 8 + r) * 2 + part) * 8, 8)

    def tm_get(kc, r):
        return _f32(pb[tm_rows(kc, r, 0), :]), _f32(pb[tm_rows(kc, r, 1), :])

    def tm_put(kc, r, z):
        pb[tm_rows(kc, r, 0), :] = _u32(z[0])
        pb[tm_rows(kc, r, 1), :] = _u32(z[1])

    def mid_1(g, blk, r):
        view = pb.at[pl.ds(pl.multiple_of(U_OFF + g * 2048, 32), 2048 + 8)]
        x = []
        for c in range(8):
            re, im = [_f32(view[pl.ds((blk * 2 + part) * 512 + c * 64 + r, 8, stride=8), :]) for part in range(2)]
            if 8 * c + r:
                ct, st = stw_s[g, 8 * c + r, 0], stw_s[g, 8 * c + r, 1]
                re, im = re * ct + im * st, im * ct - re * st
            x.append((re, im))
        z = _fft(x, -1)
        for kc in range(8):
            tm_put(kc, r, _cmul(z[kc], -2 * np.pi * r * kc / N2))

    def mid_2(g, blk, kc):
        z = _fft([tm_get(kc, r) for r in range(8)], -1)
        y = []
        for kr in range(8):
            w = [pb[pl.ds(pl.multiple_of(g * 512, 32) + (F_OFF + a * 2048 + (kc + 8 * kr) * 8), 8), :]
                 for a in range(2)]
            wr, wi = [_f32(v & jnp.uint32(HI_MASK)) if blk else _f32(v << 16) for v in w]
            zr, zi = z[kr]
            y.append((zr * wr - zi * wi, zr * wi + zi * wr))
        v = _fft(y, 1)
        for r in range(8):
            tm_put(kc, r, _cmul(v[r], 2 * np.pi * r * kc / N2))

    def mid_3(g, blk, r):
        z = _fft([tm_get(kc, r) for kc in range(8)], 1)
        for c in range(8):
            re, im = z[c]
            if 8 * c + r:
                ct, st = stw_s[g, 8 * c + r, 0], stw_s[g, 8 * c + r, 1]
                re, im = re * ct - im * st, im * ct + re * st
            for part, v in enumerate((re, im)):
                row = V_OFF + c * 1024 + (blk * 2 + part) * 256 + r * 8
                big[pl.ds(pl.multiple_of(g * 64, 32) + row, 8), :] = v

    def nyq_a():
        z = _dot(_bf(dmat_s[0, 192:256, 0:128]), _f32(pb[pl.ds(UN_OFF, 128), :]).astype(BF))
        w = []
        for a in range(2):
            g = jnp.concatenate([fraw[a, 256:257, t * 128:(t + 1) * 128].astype(F32) for t in range(16)], axis=0)
            w.append(jnp.concatenate([g] + [pltpu.roll(g, 128 - 32 * q, 1) for q in range(1, 4)], axis=0))
        return cfilter(z, *w)

    def nyq_b(y):
        big[pl.ds(VN_OFF, 128), :] = _dot(_bf(dmat_s[0, 192:256, 128:256]), y)

    def inv_pass1(c, blk, ka):
        view = big.at[pl.ds(pl.multiple_of(V_OFF + c * 1024, 32), 1024 + 8)]
        z = _fft([tuple(view[pl.ds((blk * 2 + part) * 256 + (k1 // 8) * 64 + k1 % 8, 8, stride=8), :]
                        for part in range(2)) for k1 in range(ka, N1, 4)], 1)
        for b in range(8):
            zr, zi = _cmul(z[b], 2 * np.pi * b * ka / N1)
            big[t_rows(ka, b, 0), :] = zr
            big[t_rows(ka, b, 1), :] = zi

    def inv_nyq(c):
        vr, vi = big[_rows8(VN_OFF + c * 8), :], big[_rows8(VN_OFF + 64 + c * 8), :]
        ct, st = twiddles(c)
        m = _bf(dmat_s[1, 128:192, :])
        return (_dot((vr * ct - vi * st).astype(BF), m[:, 0:128])
                + _dot((vi * ct + vr * st).astype(BF), m[:, 128:256]))

    def inv_pass2(blk, b, n):
        z = _fft([(big[t_rows(ka, b, 0), :], big[t_rows(ka, b, 1), :]) for ka in range(4)], 1)
        for a in range(4):
            re, im = z[a]
            s1 = 8 * a + b
            if blk == 0:
                im = pltpu.roll(im, 1, 1)
                nv = n if s1 == 1 else pltpu.roll(n, (1 - s1) % 128, 1)
                re, im = jnp.where(lane == 1, nv, jnp.where(lane_lo, re, im)), jnp.where(lane_lo, im, re)
            else:
                im = pltpu.roll(im, 2, 1)
                re, im = jnp.where(lane_plus, re, im), jnp.where(lane_plus, im, re)
            big[pl.ds(L_OFF + (2 * blk) * 256 + s1 * 8, 8), :] = re
            big[pl.ds(L_OFF + (2 * blk + 1) * 256 + s1 * 8, 8), :] = im

    def inv_out(c):
        lhs = [big[pl.ds(L_OFF + i * 256, 256), :] for i in range(4)]
        c0 = _dot(lhs[0].astype(BF), _bf(dmat_s[1, 0:64, 0:128]))
        c2 = _dot(lhs[1].astype(BF), _bf(dmat_s[1, 0:64, 128:256]))
        lp = _dot(lhs[2].astype(BF), _bf(dmat_s[1, 64:128, 0:128]))
        lm = _dot(lhs[3].astype(BF), _bf(dmat_s[1, 64:128, 128:256]))
        pp, qq = lp + lm, lp - lm
        r = pltpu.roll(jnp.where(lane_half, qq, pp), 64, 1)
        p, q = jnp.where(lane_half, pp, (r + qq) * rt), jnp.where(lane_half, r, (qq - r) * rt)
        e, f = c0 + c2, c0 - c2
        y = jnp.concatenate([e + p, f + q, e - p, f - q], axis=1)
        oa_s[:, _rows8(c * 8), :] = y.reshape(N1, 8, DM).astype(BF)

    def head_words(hh, n):
        a = wtmp[pl.ds(hh // 2, n, stride=8), :]
        b = wtmp[pl.ds(4 + hh // 2, n, stride=8), :]
        return (a >> 16) | (b & jnp.uint32(HI_MASK)) if hh % 2 else (a & 0xFFFF) | (b << 16)

    def head_weights(t, hh):
        w = head_words(hh, 256)
        w_s[t * 8 + hh] = w
        return w

    def stage_chunk(t, first_head=True):
        for dc in range(8):
            wtmp[dc * 256:(dc + 1) * 256, :] = _u32(wraw[t, dc * 64:(dc + 1) * 64].reshape(512, 128))
        if first_head:
            head_weights(t, 0)

    def early_proj(t, hooks, first_ready=True):
        for jj in range(4):
            res = []
            for hh in (2 * jj, 2 * jj + 1):
                w = w_s[t * 8] if hh == 0 and first_ready else head_weights(t, hh)
                r = _dot(_bf(jnp.concatenate([x0_s[k] for k in range(4)], axis=1)), _bf(w))
                res.append(r.reshape(NSEG, 8, 128))
                for tm, f, pinned in hooks:
                    if tm // 8 == hh:
                        if pinned:
                            pb[_rows8(TK_OFF + (t % 2) * 32), :] = _u32(r[(tm % 8) * 64:(tm % 8) * 64 + 8])
                        f()
            big[pl.ds(pl.multiple_of(P_OFF + (t * 4 + jj) * 1024, 1024), 1024), :] = (
                jnp.concatenate(res, axis=1).reshape(1024, 128))

    def phase_0(kt, carry):
        for c in first_copies(kt):
            c.wait()
        for dc in range(2):
            v = wraw[0, pl.ds(pl.multiple_of(kt * 128 + dc * 64, 64), 64)]
            wtmp[dc * 256:(dc + 1) * 256, :] = _u32(v.reshape(512, 128))
        xk = _u32(x0raw[kt].reshape(NSEG * 8, 128))
        x0_s[kt] = xk
        for jj in range(4):
            res = []
            a = wtmp[pl.ds(jj, 64, stride=8), :]
            b = wtmp[pl.ds(4 + jj, 64, stride=8), :]
            for hh, w in ((2 * jj, (a & 0xFFFF) | (b << 16)), (2 * jj + 1, (a >> 16) | (b & jnp.uint32(HI_MASK)))):
                w_s[hh, pl.ds(pl.multiple_of(kt * 64, 64), 64), :] = w
                res.append(_dot(_bf(xk), _bf(w)).reshape(NSEG, 8, 128))
            rows = pl.ds(P_OFF + jj * 1024, 1024)
            big[rows, :] = jnp.where(kt > 0, big[rows, :], 0.0) + jnp.concatenate(res, axis=1).reshape(1024, 128)
        return carry

    def phase_a(t, carry):
        @pl.when(t <= 2)
        def _():
            w_wait(t)
            w_copy(1, t).start()
            for c in chunk_copies(t):
                c.start()
            stage_chunk(t, False)

        @pl.when(t >= 2)
        def _():
            w_wait(t + 1)

        early_proj(t, [], False)
        stage_chunk(jnp.where(t >= 2, t + 1, t))
        return carry

    def phase_b(i, carry):
        t = i + 3

        @pl.when(i < 4)
        def _():
            for c in [w_copy(2, i)] + chunk_copies(i + 4, (0,)):
                c.start()

        w_wait(t + 1)
        for c in chunk_copies(i):
            c.wait()

        @pl.when(i < 4)
        def _():
            for c in chunk_copies(i + 4, (1, 2, 3)):
                c.start()

        @pl.when(i == 4)
        def _():
            for c in late:
                c.start()

        def wo_retile(n):
            wo_s[n * 8 + i] = _u32(woraw[pl.ds(pl.multiple_of(i * 512, 512), 512), n * 128:(n + 1) * 128])

        box = {}
        t_om, t_f, t_o1, t_o2, t_em, t_e1, t_n, t_e2, t_pn, dt = SCHED_PB
        hooks = [(t_f + dt * k, lambda k=k: filt_prep(i, k // 2, k % 2), False) for k in range(4)]
        hooks += [(t_om, lambda: box.update(o=fwd_odd(i)), False),
                  (t_o1, lambda: fwd_pass1(i, 1, *box["o"]), False),
                  (t_em, lambda: box.update(e=fwd_even(i)), False),
                  (t_e1, lambda: fwd_pass1(i, 0, *box["e"][:2]), False),
                  (t_n, lambda: box.update(n=fwd_nyq(i, box["e"][2])), False),
                  (t_pn, lambda: put_nyq(i, box["n"]), False)]
        hooks += [(t_o2 + dt * ka, lambda ka=ka: fwd_pass2(i, 1, ka), True) for ka in range(4)]
        hooks += [(t_e2 + dt * ka, lambda ka=ka: fwd_pass2(i, 0, ka), True) for ka in range(4)]
        hooks += [(0, lambda n=n: wo_retile(n), False) for n in range(4)]
        early_proj(t, sorted(hooks, key=lambda h: h[0]))
        stage_chunk(jnp.minimum(t + 1, 11))
        return carry

    def x0_rows(r0, n):
        return _bf(jnp.concatenate([x0_s[k, r0 // 2:(r0 + n) // 2, :] for k in range(4)], axis=1))

    def phase_c():
        pb[TK_OFF:TK_OFF + 64, :] = jnp.zeros((64, 128), U32)
        for jj in range(4):
            res = []
            for hh in (2 * jj, 2 * jj + 1):
                w = w_s[88] if hh == 0 else head_weights(11, hh)
                res.append(_dot(x0_rows(0, 128), _bf(w)).reshape(16, 8, 128))
                if hh == 0:
                    y = nyq_a()
                if hh == 5:
                    nyq_b(y)
            big[pl.ds(P_OFF + (44 + jj) * 1024, 256), :] = jnp.concatenate(res, axis=1).reshape(256, 128)

    def early_rest(i, u):
        r = _dot(x0_rows(128 + 192 * (u % 2), 192), _bf(w_s[88 + 2 * i + u // 2]))
        for q in range(24):
            row = P_OFF + 44 * 1024 + (16 + 24 * (u % 2) + q) * 16 + (u // 2) * 8
            big[pl.ds(pl.multiple_of(i * 1024, 32) + row, 8), :] = r[q * 8:(q + 1) * 8]

    def wo_rows(j):
        r = pl.ds(pl.multiple_of((j & 1) * 128, 128), 128)
        return _bf(jnp.concatenate([wo_s[n * 8 + (j >> 1), r, :] for n in range(4)], axis=1))

    def put_late(g, res):
        for i in range(16):
            ob_s[g * 8 + i // 2, (i % 2) * 32:(i % 2) * 32 + 8, :] = res[i * 8:(i + 1) * 8].astype(BF)

    def late_proj(idx):
        g, c = idx >> 4, idx & 15
        a = od_s[c, pl.ds(pl.multiple_of(g * 128, 128), 128), :].astype(BF)
        res = jnp.where(c > 0, acc_s[...], 0.0) + _dot(a, wo_rows(c))
        acc_s[...] = res
        put_late(g, res)

    def step(s0, u0, mem, hooks, lags):
        s = s0 + u0
        qk_lag, pv_lag, skew = lags // 100, lags // 10 % 10, lags % 10
        lhs = jnp.concatenate([mem, xr_s[s].astype(F32)], axis=0).astype(BF)
        st = {}

        def proj(mi, j):
            w1 = w_s[mi * H + 2 * j]
            if "gate" in st:
                w1 = jnp.concatenate([w1[0:248], w1[248:256] | st.pop("gate")], axis=0)
            y1 = _dot(lhs, _bf(w1))
            y2 = _dot(lhs, _bf(w_s[mi * H + 2 * j + 1]))
            pre = big[pl.ds(pl.multiple_of(s0 * 16, 32) + (P_OFF + (mi * NP + j) * 1024 + u0 * 16), 16), :]
            st[mi, j] = jnp.concatenate([y1, y2, pre], axis=0).astype(BF)
            st["last"] = y1[0:8]

        def pin():
            big[pl.ds(pl.multiple_of((s0 & 2) * 16, 32) + X_OFF, 8), :] = st["last"]

        def gate():
            st["gate"] = pb[pl.ds(pl.multiple_of((s0 % 8) * 8, 32) + (TK_OFF + 8), 8), :]

        def pin_pb():
            pb[pl.ds(pl.multiple_of((s0 % 8) * 8, 32) + TK_OFF, 8), :] = _u32(st["last"])

        def qk(j):
            sc = lax.dot_general(st.pop((1, j)), st.pop((0, j)), (((1,), (1,)), ((), ())),
                                 preferred_element_type=F32)
            fill = misc_s[0:80, 0:80]
            sc = jnp.where(fill == 0.0, sc, fill)
            p = jnp.exp2((sc - jnp.max(sc, axis=1, keepdims=True)) * EXP_C)
            st["p", j] = (p.astype(BF), pl.reciprocal(jnp.sum(p, axis=1, keepdims=True), approx=True))

        def pv(j):
            p, rl = st.pop(("p", j))
            o = _dot(p, st.pop((2, j))) * rl
            st["o", j] = jnp.concatenate([o[0:32], o[32:64]], axis=1).astype(BF)
            od_s[j, pl.ds(pl.multiple_of(s0 * 8, 16) + u0 * 8, 8), :] = jnp.concatenate([o[64:72], o[72:80]], axis=1)

        def op(j):
            r = _dot(st.pop(("o", j)), wo_rows(j))
            st["acc"] = r if "acc" not in st else st["acc"] + r

        units = []
        for j in range(-skew, NP):
            units += [(mi, j + skew) for mi in (0, 1) if j + skew < NP] + ([(2, j)] if j >= 0 else [])
        events = [(t, lambda mi=mi, j=j: proj(mi, j)) for t, (mi, j) in enumerate(units)]
        events += [(3 * NP + j, lambda j=j: op(j)) for j in range(NP)]
        for j in range(NP):
            tqk = units.index((1, j)) + 1 + qk_lag
            events.append((tqk - 0.5, lambda j=j: qk(j)))
            events.append((max(tqk + pv_lag, units.index((2, j)) + 1 + qk_lag) - 0.4, lambda j=j: pv(j)))
        for t, fs in hooks.items():
            events += [(t - 0.3, {None: pin, "pb": pin_pb, "gate": gate}.get(f, f)) for f in fs]
        for _, f in sorted(events, key=lambda ev: ev[0]):
            f()
        out = st["acc"]
        ob_s[(s0 >> 1) + u0 // 2, (u0 % 2) * 32 + 8:(u0 % 2) * 32 + 32, :] = out[8:32].astype(BF)
        return out[0:8].astype(BF).astype(F32)

    def loop_a(i, mem):
        jobs = [{} for _ in range(4)]
        t_0, dt, t_g, nps, t_x = SCHED_LA

        def add(t, fs):
            u = min(t // 64, 3)
            jobs[u].setdefault(t - 64 * u, []).extend(fs)

        pieces = [(f, blk, k) for blk in range(2) for f in (mid_1, mid_2, mid_3) for k in range(8)]
        for n, (f, blk, k) in enumerate(pieces):
            add(64 * (n // nps) + t_0 + dt * (n % nps), ["pb", lambda f=f, blk=blk, k=k: f(i, blk, k)])
        add(192 + t_g, ["gate"])
        for u, t in enumerate(sorted([64, 128, 192, t_x])):
            add(t, [lambda u=u: early_rest(i, u)])
        for u in range(4):
            mem = step(4 * i, u, mem, jobs[u], STEP_A[u])
        return mem

    def loop_b(i, mem):
        box = {}
        jobs = [{} for _ in range(6)]
        t1, d1, t2, d2, t_n, t_o, t_x = SCHED_LB

        def add(t, fs):
            u = min(t // 64, 5)
            jobs[u].setdefault(t - 64 * u, []).extend(fs)

        for blk in range(2):
            for ka in range(4):
                add(128 * blk + t1 + d1 * ka, [None, lambda blk=blk, ka=ka: inv_pass1(i, blk, ka)])
            for b in range(8):
                add(128 * blk + 64 + t2 + d2 * b, [None, lambda blk=blk, b=b: inv_pass2(blk, b, box["n"])])
        add(t_n, [lambda: box.update(n=inv_nyq(i))])
        add(t_o, [lambda: inv_out(i)])
        for u, t in enumerate(sorted([64 * u for u in range(1, 6)] + [t_x])):
            add(t, [lambda u=u: late_proj(6 * i + u)])
        for u in range(6):
            mem = step(6 * i, 16 + u, mem, jobs[u], STEP_B[u])
        oa_copy(i).start()

        @pl.when((i == 2) | (i == 5))
        def _():
            ob_copy(i >> 2).start()

        return mem

    for kt in range(4):
        for c in first_copies(kt):
            c.start()
    for g in range(1, 4):
        w_copy(0, g).start()
    lax.fori_loop(0, 4, phase_0, 0)
    w_copy(1, 0).start()
    for c in early + chunk_copies(0):
        c.start()
    lax.fori_loop(1, 3, phase_a, 0)
    w_copy(1, 3).start()
    for c in chunk_copies(3):
        c.start()
    for c in early:
        c.wait()
    lax.fori_loop(0, 8, phase_b, 0)
    phase_c()
    for c in late:
        c.wait()
    mem = mem_s[0].astype(F32)
    mem = lax.fori_loop(0, 4, loop_a, mem)
    lax.fori_loop(0, 8, loop_b, mem)
    ob_copy(2).start()
    parts = [(8, 24, 0, DM), (40, 24, 0, DM), (0, 8, 0, 384), (32, 8, 0, 384), (0, 8, 384, 128), (32, 8, 384, 128)]
    last = [cp(ob_s.at[pl.ds(24, 8), pl.ds(r, n), pl.ds(c0, nc)],
               o_h.at[pl.ds(24, 8), pl.ds(r, n), pl.ds(DM + c0, nc)], sem_ob.at[3 + k])
            for k, (r, n, c0, nc) in enumerate(parts)]
    last[0].start()
    last[1].start()
    a = jnp.concatenate([od_s[c, 384:512, :] for c in range(NP)], axis=1).astype(BF)
    w = jnp.concatenate([wo_rows(j) for j in range(NP)], axis=0)
    for k, (c0, nc) in enumerate([(0, 384), (384, 128)]):
        res = _dot(a, w[:, c0:c0 + nc])
        for i in range(16):
            ob_s[24 + i // 2, (i % 2) * 32:(i % 2) * 32 + 8, c0:c0 + nc] = res[i * 8:(i + 1) * 8].astype(BF)
        last[2 + 2 * k].start()
        last[3 + 2 * k].start()
    for c in range(8):
        oa_copy(c).wait()
    for g in range(3):
        ob_copy(g).wait()
    for c in last:
        c.wait()


def _compiler_params():
    base = dict(vmem_limit_bytes=120 * 1024 * 1024, disable_bounds_checks=True)
    try:
        return pltpu.CompilerParams(disable_semaphore_checks=True, **base)
    except TypeError:
        return pltpu.CompilerParams(**base)


@jax.jit
def pallas_concat_heads__spectral_gfnet__memory_aug_recurrent_mem_tr__prompt_kernel(
        A_x, A_w_r, A_w_i, B_x, B_mem0, B_Wq, B_Wk, B_Wv, B_Wo, B_seg_len=None):
    dmat, stw, misc = _consts()
    vm, dma = pltpu.VMEM, pltpu.SemaphoreType.DMA
    out = pl.pallas_call(
        _kernel,
        out_shape=jax.ShapeDtypeStruct((N1, N2, 2 * DM), BF),
        in_specs=[pl.BlockSpec(memory_space=pl.ANY)] * 12,
        out_specs=pl.BlockSpec(memory_space=pl.ANY),
        scratch_shapes=[
            vm((12, DM, 8, DH), BF), vm((PB_ROWS, 128), U32), vm((2048 + 32, 128), U32),
            vm((3 * H, DM // 2, DH), U32), vm((H, DM // 2, DH), U32), vm((H * DH, DM), BF),
            vm((BIG_ROWS, 128), F32), vm((NP, NSEG * 8, 2 * DH), F32), vm((128, DM), F32),
            vm((4, NSEG, 8, 128), BF), vm((4, NSEG * 4, 128), U32), vm((NSEG, 24, DM), BF),
            vm(misc.shape, F32),
            vm((N1, N2, DM), BF), vm((2, DM // 2 + 1, S), BF), vm(dmat.shape, U32), vm(stw.shape, F32),
            vm((N1, N2, DM), BF), vm((N1, N2, DM), BF), vm((2, MEM, DM), BF),
            dma((12,)), dma((8,)), dma((5,)), dma((8,)), dma((9,)), dma((4,)),
        ],
        compiler_params=_compiler_params(),
    )(A_x.reshape(N1, N2, DM), A_w_r.T, A_w_i.T,
      B_x.reshape(NSEG, SEG, DM), B_mem0.reshape(MEM, DM), B_Wq, B_Wk, B_Wv, B_Wo.reshape(H * DH, DM),
      jnp.asarray(dmat), jnp.asarray(stw), jnp.asarray(misc))
    return out.reshape(1, S, 2 * DM)
```
